```python
import jax
import jax.numpy as jnp

def _softmax(x, axis=-1):
    return jax.nn.softmax(x, axis=axis)
def _gelu(x):
    return jax.nn.gelu(x, approximate=True)
def _silu(x):
    return jax.nn.silu(x)
def _sigmoid(x):
    return jax.nn.sigmoid(x)
def _layernorm(x, axis=-1, eps=1e-5):
    m = jnp.mean(x, axis=axis, keepdims=True)
    v = jnp.var(x, axis=axis, keepdims=True)
    return (x - m) / jnp.sqrt(v + eps)
def _scatter_add(tgt, idx, src, axis=0):
    return tgt.at[idx].add(src)
def _segment_sum(src, seg, n):
    return jax.ops.segment_sum(src, seg, n)
class _Rng:
    def __init__(self, key):
        self._k = key
    def _next(self):
        self._k, sub = jax.random.split(self._k)
        return sub
    def normal(self, shape):
        return jax.random.normal(self._next(), shape, dtype=jnp.bfloat16)
    def randint(self, lo, hi, shape):
        return jax.random.randint(self._next(), shape, lo, hi, dtype=jnp.int32)
    def uniform(self, shape, lo=0.0, hi=1.0):
        return jax.random.uniform(self._next(), shape, jnp.bfloat16, lo, hi)
    def permutation(self, n):
        return jax.random.permutation(self._next(), n)


kernel_name = 'gated_mix__sliding_local_dilated__ssm_conv_s4__prompt'

def setup_inputs():
    _rng = _Rng(jax.random.key(int.from_bytes(__import__("os").urandom(4), "little")))
    _w = (lambda a: (lambda t: t.astype(jnp.bfloat16) if jnp.issubdtype(t.dtype, jnp.floating) else t)(jnp.asarray(a)))
    def _A_setup():
        B, S, D = 1, 2048, 640
        return {
            "x": _w((lambda *s: _rng.normal(s) * 0.05)(B, S, D)),
            "wqkv": _w((lambda *s: _rng.normal(s) * 0.05)(D, 3 * D)),
            "wo": _w((lambda *s: _rng.normal(s) * 0.05)(D, D)),
        }
    _A_in = _A_setup()

    def _B_setup():
        B, L, D, N = 1, 2048, 640, 192
        A_re = -jnp.exp((lambda *s: _rng.normal(s) * 0.05)(D, N))
        A_im = jnp.pi * (lambda *s: _rng.normal(s) * 0.05)(D, N)
        B_re = (lambda *s: _rng.normal(s) * 0.05)(D, N)
        B_im = (lambda *s: _rng.normal(s) * 0.05)(D, N)
        C_re = (lambda *s: _rng.normal(s) * 0.05)(D, N)
        C_im = (lambda *s: _rng.normal(s) * 0.05)(D, N)
        log_dt = (lambda *s: _rng.normal(s) * 0.05)(D) * 0.5 - 4.0
        Dskip = (lambda *s: _rng.normal(s) * 0.05)(D)
        return {
            "u": _w((lambda *s: _rng.normal(s) * 0.05)(B, L, D)),
            "A_re": _w(A_re),
            "A_im": _w(A_im),
            "B_re": _w(B_re),
            "B_im": _w(B_im),
            "C_re": _w(C_re),
            "C_im": _w(C_im),
            "log_dt": _w(log_dt),
            "Dskip": _w(Dskip),
        }
    _B_in = _B_setup()

    return {
        "A_x": _A_in["x"],
        "A_wqkv": _A_in["wqkv"],
        "A_wo": _A_in["wo"],
        "B_u": _B_in["u"],
        "B_A_re": _B_in["A_re"],
        "B_A_im": _B_in["A_im"],
        "B_B_re": _B_in["B_re"],
        "B_B_im": _B_in["B_im"],
        "B_C_re": _B_in["C_re"],
        "B_C_im": _B_in["C_im"],
        "B_log_dt": _B_in["log_dt"],
        "B_Dskip": _B_in["Dskip"],
        "gate_w": _w((lambda *s: _rng.normal(s) * 0.05)(640)),
    }

def reference(A_x, A_wqkv, A_wo, B_u, B_A_re, B_A_im, B_B_re, B_B_im, B_C_re, B_C_im, B_log_dt, B_Dskip, gate_w):
    def _A_ref(x, wqkv, wo):
        B, S, D = x.shape
        H = 32; Dh = D // H
        W, dil = 8, 2
        qkv = (lambda x, *d: x.transpose(*d))((x @ wqkv).reshape(B, S, 3, H, Dh), 2, 0, 3, 1, 4)
        q, k, v = qkv[0], qkv[1], qkv[2]
        scale = Dh ** -0.5
        pos = jnp.arange(S)
        off = jnp.arange(W) * dil
        idx = pos[:, None] - off[None, :]
        mask = idx >= 0
        idx_c = jnp.where(mask, idx, 0).reshape(-1)
        kg = k[:, :, idx_c, :].reshape(B, H, S, W, Dh)
        vg = v[:, :, idx_c, :].reshape(B, H, S, W, Dh)
        logits = jnp.einsum("bhsd,bhswd->bhsw", q, kg) * scale
        logits = jnp.where(mask[None, None, :, :], logits, -1e9)
        attn = _softmax(logits, axis=-1)
        o = jnp.einsum("bhsw,bhswd->bhsd", attn, vg)
        return (lambda x, *d: x.transpose(*d))(o, 0, 2, 1, 3).reshape(B, S, D) @ wo

    def _B_ref(u, A_re, A_im, B_re, B_im, C_re, C_im, log_dt, Dskip):
        Bsz, L, D = u.shape
        dt = jnp.exp(log_dt)[:, None]
        A = A_re + 1j * A_im
        Bc = B_re + 1j * B_im
        Cc = C_re + 1j * C_im
        logdA = dt * A
        dB = dt * Bc
        l = (lambda x, dt: x.astype(dt))(jnp.arange(L), A_re.dtype)
        P = jnp.exp(logdA[:, :, None] * l[None, None, :])
        K = jnp.einsum("dn,dnl,dn->dl", Cc, P, dB).real
        L2 = 2 * L
        Kp = jnp.pad(K, ((0, 0), (0, L)))
        up = (lambda x, *d: x.transpose(*d))(u, 0, 2, 1)
        up = jnp.pad(up, ((0, 0), (0, 0), (0, L)))
        Kf = (lambda x, axes=(-2,-1): jnp.fft.rfft2(x.astype(jnp.float32), axes=axes))(Kp[:, None, :], axes=(-2, -1))
        Uf = (lambda x, axes=(-2,-1): jnp.fft.rfft2(x.astype(jnp.float32), axes=axes))(up[:, :, None, :], axes=(-2, -1))
        Yf = Uf * Kf[None, :, :, :]
        y = (lambda x, s, axes=(-2,-1): jnp.fft.irfft2(x, s=s, axes=axes).astype(jnp.bfloat16))(Yf, (1, L2), axes=(-2, -1))[:, :, 0, :L]
        y = (lambda x, *d: x.transpose(*d))(y, 0, 2, 1) + u * Dskip[None, None, :]
        return y

    x = A_x
    g = _sigmoid((x * gate_w).sum(-1, keepdims=True))
    a = _A_ref(x, A_wqkv, A_wo)
    b = _B_ref(x, B_A_re, B_A_im, B_B_re, B_B_im, B_C_re, B_C_im, B_log_dt, B_Dskip)
    return g * a + (1 - g) * b
```

```python
import ml_dtypes
import numpy as np

import jax
import jax.numpy as jnp
import jax.experimental.pallas as pl
import jax.experimental.pallas.tpu as pltpu

F32 = jnp.float32
BF16 = jnp.bfloat16

S = 2048
D = 640
NS = 192
H = 32
DH = D // H
WIN, DIL = 8, 2
T = 128
NB = S // T
NT = D // 128
PAD = 16
CH = 32
M2 = 256
M3 = 128

_BASE = (0, 4, 256, 512, 1024, 2048)
_OFF = ((0, 1, 2, 3), (0, 1, 2, 3), (0, 2, 4, 6), (0, 4, 256, 260), (0, 256, 512, 768), (0, 0, 0, 0))


def _dft_constants():
    k = np.concatenate([np.arange(0, T, 2), np.arange(1, T, 2)])
    theta = 2.0 * np.pi * (k + 0.5) / (2 * T)
    ang = theta[:, None] * np.arange(T)[None, :]
    fwd = np.concatenate([np.cos(ang), -np.sin(ang)], axis=0)
    inv = np.stack([np.cos(ang).reshape(T // 8, 8, T), -np.sin(ang).reshape(T // 8, 8, T)], axis=1)
    inv = inv.reshape(2 * T, T).T / T
    slot = {}
    for t in range(len(_BASE)):
        for lane in range(128):
            i, a, p = lane // 8, (lane % 8) // 2, lane % 2
            slot.setdefault(_BASE[t] + _OFF[t][a] + 8 * (2 * i + p), (t, lane))
    lag = np.arange(S).astype(np.float32).astype(ml_dtypes.bfloat16).astype(np.float64).astype(np.int64)
    mats, passes = [], []
    for m in range(NB):
        per_tile = {}
        for n in range(T):
            t, lane = slot[int(lag[m * T + n])]
            per_tile.setdefault(t, np.zeros((2 * T, 128)))[:, lane] += fwd[:, n]
        passes.append(tuple((t, len(mats) + j) for j, t in enumerate(sorted(per_tile))))
        mats.extend(per_tile[t] for t in sorted(per_tile))
    to_bf16 = lambda a: np.asarray(a, np.float32).astype(ml_dtypes.bfloat16)
    return to_bf16(fwd), to_bf16(inv), to_bf16(np.stack(mats)), tuple(passes)


_FWD, _INV, _KMATS, _KPASSES = _dft_constants()

(_Q_V0, _Q_Z16, _Q_Z32, _Q_Z64, _Q_Z128, _Q_W0, _Q_W1, _Q_W2,
 _Q_G01, _Q_G02, _Q_G11, _Q_G12, _Q_G21, _Q_G22) = range(14)
_NQ = 14

_NT_DIMS = (((1,), (1,)), ((), ()))


def _csq(z):
    x, y, p, q = z
    return ((x - y) * (x + y), (x + x) * y, (p - q) * (p + q), (p + p) * q)


def _cmul(a, b):
    ax, ay, ap, aq = a
    bx, by, bp, bq = b
    return (ax * bx - ay * by, ax * by + ay * bx, ap * bp - aq * bq, ap * bq + aq * bp)


def _vmul(v, m, swapped):
    x, y, t, u = v
    mx, my, mp, mq = m
    tn = t * mp + u * mq
    return (x * mx - y * my, x * my + y * mx, tn, (u * mp - t * mq) if swapped else None)


def _kernel(x_hbm, wqkv_hbm, wo_hbm, kmat_hbm,
            are_ref, aim_ref, bre_ref, bim_ref, cre_ref, cim_ref,
            ldt_ref, dskip_ref, gw_ref, fwd_ref, inv_ref,
            out_hbm,
            xs, wraw, woraw, kmat, wt, wop, tmp, dts, tab, rs, xf, kf, zs, qs, ks, vs, os_, outs,
            in_sem, out_sem):
    cp_x = pltpu.make_async_copy(x_hbm, xs, in_sem.at[0])
    cp_w = pltpu.make_async_copy(wqkv_hbm, wraw, in_sem.at[1])
    cp_wo = pltpu.make_async_copy(wo_hbm, woraw, in_sem.at[2])
    cp_km = pltpu.make_async_copy(kmat_hbm, kmat, in_sem.at[3])
    cp_x.start()
    cp_km.start()
    cp_w.start()
    cp_wo.start()

    lane = jax.lax.broadcasted_iota(jnp.int32, (8, 128), 1)
    row = jax.lax.broadcasted_iota(jnp.int32, (8, 128), 0)
    low = lane < 64

    dt_row = jnp.exp(ldt_ref[...].astype(F32)).astype(BF16).astype(F32)
    for c in range(NT):
        dts[c * 128:(c + 1) * 128, :] = jnp.broadcast_to(dt_row[:, c * 128:(c + 1) * 128], (128, 128)).T

    def put(tile, slot, even, odd):
        for comp in range(4):
            base = ((tile * _NQ + slot) * 4 + comp) * 16
            tab[pl.ds(base, 8, stride=2), :] = even[comp]
            tab[pl.ds(base + 1, 8, stride=2), :] = odd[comp]

    def get(group, slot):
        tile, half = divmod(group, 2)
        return tuple(tab[pl.ds(((tile * _NQ + slot) * 4 + comp) * 16 + 8 * half, 8), :] for comp in range(4))

    def running(z, conj):
        x, y, p, q = z
        if conj:
            return (x, -y, jnp.where(low, p, -q), jnp.where(low, q, p))
        return (x, y, jnp.where(low, p, q), jnp.where(low, -q, p))

    def conj(z):
        return (z[0], -z[1], z[2], -z[3])

    def tables(r0, pair):
        rows = pl.ds(r0, 16)
        dt = dts[rows, :]

        def split(ref):
            v = ref[rows, :].astype(F32)
            hi = v[:, 128:NS]
            return v[:, :128], jnp.concatenate([hi, hi], axis=1)

        a_re, a_im = split(are_ref), split(aim_ref)
        b_re, b_im = split(bre_ref), split(bim_ref)
        c_re, c_im = split(cre_ref), split(cim_ref)
        mag_lo = jnp.exp(dt * a_re[0])
        ang_lo = dt * a_im[0]
        zr_lo, zi_lo = mag_lo * jnp.cos(ang_lo), mag_lo * jnp.sin(ang_lo)
        pick = lambda v: jnp.where(low, v[0:8], v[8:16])
        mag_hi = jnp.exp(pick(dt * a_re[1]))
        ang_hi = pick(dt * a_im[1])
        zr_hi, zi_hi = mag_hi * jnp.cos(ang_hi), mag_hi * jnp.sin(ang_hi)
        zr_sw, zi_sw = pltpu.roll(zr_hi, 64, 1), pltpu.roll(zi_hi, 64, 1)
        w_re = [c_re[i] * (dt * b_re[i]) - c_im[i] * (dt * b_im[i]) for i in range(2)]
        w_im = [c_re[i] * (dt * b_im[i]) + c_im[i] * (dt * b_re[i]) for i in range(2)]
        one = (jnp.ones((8, 128), F32), jnp.zeros((8, 128), F32)) * 2
        for half in range(2):
            sl = slice(8 * half, 8 * half + 8)
            if half == 0:
                p, q = jnp.where(low, zr_hi, zr_sw), jnp.where(low, -zi_hi, zi_sw)
            else:
                p, q = jnp.where(low, zr_sw, zr_hi), jnp.where(low, -zi_sw, zi_hi)
            pw = {1: (zr_lo[sl], zi_lo[sl], p, q)}
            e = 1
            while e < S:
                pw[2 * e] = _csq(pw[e])
                e *= 2
            w = (w_re[0][sl], w_im[0][sl], w_re[1][sl], jnp.where(low, -w_im[1][sl], w_im[1][sl]))
            tile = 2 * pair + half
            put(tile, _Q_V0, running(one, True), running(pw[8], True))
            for slot, e in ((_Q_Z16, 16), (_Q_Z32, 32), (_Q_Z64, 64), (_Q_Z128, 128)):
                zc = conj(pw[e])
                put(tile, slot, zc, zc)
            put(tile, _Q_W0, running(w, False), running(_cmul(w, pw[4]), False))
            put(tile, _Q_W1, running(_cmul(w, pw[256]), False), running(_cmul(w, pw[512]), False))
            put(tile, _Q_W2, running(_cmul(w, pw[1024]), False), running(_cmul(w, pw[2048]), False))
            put(tile, _Q_G01, pw[1], pw[1])
            put(tile, _Q_G02, pw[2], pw[2])
            put(tile, _Q_G11, pw[2], pw[4])
            put(tile, _Q_G12, pw[4], pw[256])
            put(tile, _Q_G21, pw[256], one)
            put(tile, _Q_G22, pw[512], one)

    chan = row // 2
    slot_of_lane = ((lane // 2) - chan) % 4

    def generate(group, out_row):
        v = [get(group, _Q_V0)]
        for slot in (_Q_Z16, _Q_Z32, _Q_Z64, _Q_Z128):
            m = get(group, slot)
            v = v + [_vmul(u, m, slot != _Q_Z128) for u in v]
        rhs = jnp.concatenate([jnp.concatenate(u[:3], axis=1) for u in v], axis=0).astype(BF16)
        u_rows = []
        for sw, s1, s2 in ((_Q_W0, _Q_G01, _Q_G02), (_Q_W1, _Q_G11, _Q_G12), (_Q_W2, _Q_G21, _Q_G22)):
            w0, g1, g2 = get(group, sw), get(group, s1), get(group, s2)
            w1 = _vmul(w0, g1, True)
            u_rows += [w0, w1, _vmul(w0, g2, False), _vmul(w1, g2, False)]
        lhs = jnp.concatenate([jnp.concatenate(u[:3], axis=1) for u in u_rows], axis=0).astype(BF16)
        res = jax.lax.dot_general(lhs, rhs, _NT_DIMS, preferred_element_type=F32)
        for i in range(3):
            blk = [res[(4 * i + a) * 8:(4 * i + a + 1) * 8] for a in range(4)]
            r = blk[0]
            for a in range(1, 4):
                r = jnp.where(slot_of_lane == a, pltpu.roll(blk[a], 2 * a, 1), r)
            r = jnp.where((chan & 1) == 1, pltpu.roll(r, 128 - 2, 1), r)
            r = jnp.where((chan & 2) == 2, pltpu.roll(r, 128 - 4, 1), r)
            rs[i, pl.ds(out_row, 8), :] = r

    def gen_step(it, carry):
        r0 = pl.multiple_of(it * CH, CH)
        for pair in range(CH // 16):
            tables(pl.multiple_of(r0 + 16 * pair, 16), pair)
        for group in range(CH // 4):
            generate(group, pl.multiple_of(2 * r0 + 8 * group, 8))
        return carry

    jax.lax.fori_loop(0, D // CH, gen_step, 0)

    cp_x.wait()
    cp_km.wait()
    cp_w.wait()
    cp_wo.wait()

    def dft_step(c, carry):
        col = pl.ds(pl.multiple_of(c * 128, 128), 128)
        tiles = [rs[t // 2, pl.ds(c * 256 + t % 2, 128, stride=2), :].astype(BF16) for t in range(len(_BASE))]
        for m in range(NB):
            acc = None
            for t, idx in _KPASSES[m]:
                part = jax.lax.dot_general(kmat[idx], tiles[t], _NT_DIMS, preferred_element_type=F32)
                acc = part if acc is None else acc + part
            kf[m, :, col] = acc
            xf[m, :, col] = jnp.dot(fwd_ref[...], xs[m * T:(m + 1) * T, col], preferred_element_type=F32)
        for n in range(3 * NT):
            tmp[n * 128:(n + 1) * 128, :] = wraw[col, n * 128:(n + 1) * 128].astype(F32).T
        for part in range(3):
            for j in range(DH):
                wt[part * D + j * H:part * D + (j + 1) * H, col] = (
                    tmp[pl.ds(part * D + j, H, stride=DH), :].astype(BF16))
        tmp[0:D, :] = woraw[:, col].astype(F32)
        for j in range(DH):
            wop[j * H:(j + 1) * H, col] = tmp[pl.ds(j, H, stride=DH), :].astype(BF16)
        return carry

    jax.lax.fori_loop(0, NT, dft_step, 0)

    for c in range(NT):
        ks[c, 0:PAD, :] = jnp.zeros((PAD, 128), F32)
        vs[c, 0:PAD, :] = jnp.zeros((PAD, 128), F32)
    q_scale = float(DH ** -0.5 * np.log2(np.e))

    def causal(a, b):
        out = []
        for j in range(NB):
            acc = a[0] * b[j]
            for i in range(1, j + 1):
                acc = acc + a[i] * b[j - i]
            out.append(acc)
        return out

    def conv(ft, c, sign):
        re = pl.ds(pl.multiple_of(ft * 8, 8), 8)
        im = pl.ds(pl.multiple_of(T + ft * 8, 8), 8)
        col = slice(c * 128, (c + 1) * 128)
        k_re = [kf[m, re, col] for m in range(NB)]
        k_im = [kf[m, im, col] for m in range(NB)]
        kc = [k_re[0]] + [k_re[m] - sign * k_im[m - 1] for m in range(1, NB)]
        kd = [k_im[0]] + [k_im[m] + sign * k_re[m - 1] for m in range(1, NB)]
        x_re = [xf[m, re, col] for m in range(NB)]
        x_im = [xf[m, im, col] for m in range(NB)]
        s1 = causal([a + b for a, b in zip(x_re, x_im)], kc)
        s2 = causal(x_re, [d - c_ for c_, d in zip(kc, kd)])
        s3 = causal(x_im, [d + c_ for c_, d in zip(kc, kd)])
        dst = pl.ds(pl.multiple_of(ft * 16, 16), 16)
        for j in range(NB):
            zs[j, dst, col] = jnp.concatenate([s1[j] - s3[j], s1[j] + s2[j]], axis=0).astype(BF16)

    n2 = S // M2
    ft_per_step = (T // 8) // n2

    def proj_step(it, carry):
        r0 = pl.multiple_of(it * M2, M2)
        sign = jnp.where(it < n2 // 2, 1.0, -1.0).astype(F32)
        xb = xs[pl.ds(r0, M2), :]
        for part, dst in enumerate((qs, ks, vs)):
            res = jax.lax.dot_general(xb, wt[part * D:(part + 1) * D, :], _NT_DIMS, preferred_element_type=F32)
            for c in range(NT):
                blk = res[:, c * 128:(c + 1) * 128]
                if part == 0:
                    dst[c, pl.ds(r0, M2), :] = blk * q_scale
                else:
                    dst[c, pl.ds(r0 + PAD, M2), :] = blk
        for f in range(ft_per_step):
            for c in range(NT):
                conv(it * ft_per_step + f, c, sign)
        return carry

    jax.lax.fori_loop(0, n2, proj_step, 0)

    def attend(r0, first):
        for pair in range(M3 // 16):
            halves = []
            for half in range(2):
                t0 = 16 * pair + 8 * half
                q = [qs[c, pl.ds(r0 + t0, 8), :] for c in range(NT)]
                logit = []
                for w in range(WIN):
                    src = pl.ds(r0 + (t0 + PAD - DIL * w), 8)
                    acc = q[0] * ks[0, src, :]
                    for c in range(1, NT):
                        acc = acc + q[c] * ks[c, src, :]
                    acc = acc + pltpu.roll(acc, 64, 1)
                    acc = acc + pltpu.roll(acc, 32, 1)
                    if first and t0 < DIL * w:
                        acc = jnp.where(row + t0 >= DIL * w, acc, -1e9)
                    logit.append(acc)
                top = logit[0]
                for w in range(1, WIN):
                    top = jnp.maximum(top, logit[w])
                e = [jnp.exp2(l - top) for l in logit]
                den = e[0]
                for w in range(1, WIN):
                    den = den + e[w]
                inv = 1.0 / den
                o = []
                for c in range(NT):
                    acc = e[0] * vs[c, pl.ds(r0 + (t0 + PAD), 8), :]
                    for w in range(1, WIN):
                        acc = acc + e[w] * vs[c, pl.ds(r0 + (t0 + PAD - DIL * w), 8), :]
                    o.append(acc * inv)
                halves.append(jnp.concatenate(o, axis=1))
            os_[pl.ds(r0 + 16 * pair, 16), :] = jnp.concatenate(halves, axis=0).astype(BF16)

    def out_copy(blk):
        rows = pl.ds(pl.multiple_of(blk * M3, M3), M3)
        return pltpu.make_async_copy(outs.at[rows], out_hbm.at[rows], out_sem.at[blk])

    def finish(blk):
        r0 = pl.multiple_of(blk * M3, M3)
        rows = pl.ds(r0, M3)
        att = jnp.dot(os_[rows, :], wop[...], preferred_element_type=F32)
        y = jnp.dot(inv_ref[...], zs[blk], preferred_element_type=F32)
        xb = xs[rows, :].astype(F32)
        gate = jax.nn.sigmoid(jnp.sum(xb * gw_ref[...].astype(F32), axis=1, keepdims=True))
        ssm = y + xb * dskip_ref[...].astype(F32)
        outs[rows, :] = (ssm + gate * (att - ssm)).astype(BF16)

    attend(0, True)

    def out_step(it, carry):
        finish(it)
        attend(pl.multiple_of((it + 1) * M3, M3), False)
        out_copy(it).start()
        return carry

    n3 = S // M3
    jax.lax.fori_loop(0, n3 - 1, out_step, 0)
    finish(n3 - 1)
    out_copy(n3 - 1).start()
    for blk in range(n3):
        out_copy(blk).wait()


@jax.jit
def pallas_gated_mix__sliding_local_dilated__ssm_conv_s4__prompt_kernel(
    A_x: jax.Array,
    A_wqkv: jax.Array,
    A_wo: jax.Array,
    B_u: jax.Array,
    B_A_re: jax.Array,
    B_A_im: jax.Array,
    B_B_re: jax.Array,
    B_B_im: jax.Array,
    B_C_re: jax.Array,
    B_C_im: jax.Array,
    B_log_dt: jax.Array,
    B_Dskip: jax.Array,
    gate_w: jax.Array,
):
    del B_u
    assert A_x.shape == (1, S, D) and B_A_re.shape == (D, NS) and B_A_re.dtype == BF16
    hbm = pl.BlockSpec(memory_space=pl.ANY)
    vmem = pl.BlockSpec(memory_space=pltpu.VMEM)
    out = pl.pallas_call(
        _kernel,
        out_shape=jax.ShapeDtypeStruct((S, D), BF16),
        in_specs=[hbm] * 4 + [vmem] * 11,
        out_specs=hbm,
        scratch_shapes=[
            pltpu.VMEM((S, D), BF16),
            pltpu.VMEM((D, 3 * D), BF16),
            pltpu.VMEM((D, D), BF16),
            pltpu.VMEM(_KMATS.shape, BF16),
            pltpu.VMEM((3 * D, D), BF16),
            pltpu.VMEM((D, D), BF16),
            pltpu.VMEM((3 * D, 128), F32),
            pltpu.VMEM((D, 128), F32),
            pltpu.VMEM((CH // 8 * _NQ * 4 * 16, 128), F32),
            pltpu.VMEM((3, 2 * D, 128), F32),
            pltpu.VMEM((NB, 2 * T, D), F32),
            pltpu.VMEM((NB, 2 * T, D), F32),
            pltpu.VMEM((NB, 2 * T, D), BF16),
            pltpu.VMEM((NT, S, 128), F32),
            pltpu.VMEM((NT, S + PAD, 128), F32),
            pltpu.VMEM((NT, S + PAD, 128), F32),
            pltpu.VMEM((S, D), BF16),
            pltpu.VMEM((S, D), BF16),
            pltpu.SemaphoreType.DMA((4,)),
            pltpu.SemaphoreType.DMA((S // M3,)),
        ],
        compiler_params=pltpu.CompilerParams(vmem_limit_bytes=100 * 1024 * 1024),
    )(
        A_x.reshape(S, D), A_wqkv, A_wo, _KMATS,
        B_A_re, B_A_im, B_B_re, B_B_im, B_C_re, B_C_im,
        B_log_dt.reshape(1, D), B_Dskip.reshape(1, D), gate_w.reshape(1, D), _FWD, _INV,
    )
    return out.reshape(1, S, D)
```

```python
import itertools

import ml_dtypes
import numpy as np

import jax
import jax.numpy as jnp
import jax.experimental.pallas as pl
import jax.experimental.pallas.tpu as pltpu

F32 = jnp.float32
BF16 = jnp.bfloat16

S = 2048
D = 640
NS = 192
H = 32
DH = D // H
WIN, DIL = 8, 2
T = 128
NB = S // T
NT = D // 128
PAD = 16
M2 = 256
LEAD = 5
EARLY = 15
M3 = 256

_BASE = (0, 4, 256, 512, 1024, 2048)
_OFF = ((0, 1, 2, 3), (0, 1, 2, 3), (0, 2, 4, 6), (0, 4, 256, 260), (0, 256, 512, 768), (0, 0, 0, 0))


def _dft_constants():
    k = np.concatenate([np.arange(0, T, 2), np.arange(1, T, 2)])
    theta = 2.0 * np.pi * (k + 0.5) / (2 * T)
    ang = theta[:, None] * np.arange(T)[None, :]
    fwd = np.concatenate([np.cos(ang), -np.sin(ang)], axis=0)
    inv = np.stack([np.cos(ang).reshape(T // 8, 8, T), -np.sin(ang).reshape(T // 8, 8, T)], axis=1)
    inv = inv.reshape(2 * T, T).T / T
    slot = {}
    for t in range(len(_BASE)):
        for lane in range(128):
            i, a, p = lane // 8, (lane % 8) // 2, lane % 2
            slot.setdefault(_BASE[t] + _OFF[t][a] + 8 * (2 * i + p), (t, lane))
    lag = np.arange(S).astype(np.float32).astype(ml_dtypes.bfloat16).astype(np.float64).astype(np.int64)
    mats, passes = [], []
    for m in range(NB):
        per_tile = {}
        for n in range(T):
            t, lane = slot[int(lag[m * T + n])]
            per_tile.setdefault(t, np.zeros((2 * T, 128)))[:, lane] += fwd[:, n]
        passes.append(tuple((t, len(mats) + j) for j, t in enumerate(sorted(per_tile))))
        mats.extend(per_tile[t] for t in sorted(per_tile))

    def to_bf16(a):
        bits = np.asarray(a, np.float32).astype(ml_dtypes.bfloat16).view(np.uint16).astype(np.uint32)
        return (bits[..., 0::2, :] | (bits[..., 1::2, :] << 16)).view(np.int32)

    inv = inv.reshape(T, 2, T).transpose(1, 0, 2)
    return to_bf16(fwd), to_bf16(inv), to_bf16(np.stack(mats)), tuple(passes)


_FWD, _INV, _KMATS, _KPASSES = _dft_constants()

_Q_W, _Q_G, _Q_V, _Q_REC, _NQ = 0, 6, 9, 11, 12

_NT_DIMS = (((1,), (1,)), ((), ()))


def _csq(z):
    x, y, p, q = z
    return ((x - y) * (x + y), (x + x) * y, (p - q) * (p + q), (p + p) * q)


def _cmul(a, b):
    ax, ay, ap, aq = a
    bx, by, bp, bq = b
    return (ax * bx - ay * by, ax * by + ay * bx, ap * bp - aq * bq, ap * bq + aq * bp)


def _words(v):
    return pltpu.bitcast(v, jnp.int32)


def _halves(v):
    return pltpu.bitcast(v, BF16)


def _take(gen, n):
    out = []
    for _ in range(n):
        out += next(gen, [])
    return out


def _kernel(x_hbm, wqkv_hbm, wo_hbm, kmat_hbm, are_hbm, aim_hbm, bre_hbm, bim_hbm, cre_hbm, cim_hbm,
            ldt_ref, dskip_ref, gw_ref, fwd_ref, inv_ref, zero_ref, origin_ref,
            out_hbm,
            xs, xw, wraw, woraw, kmat, par, wt, wop, tmp, dts, zw, tab, rs, spec, zs, qs, ks, vs, ps, os_, oc, gs, att, ys, outs,
            x_sem, w_sem, wo_sem, km_sem, par_sem, out_sem):
    def lanes(c):
        return pl.ds(c * 128, 128) if isinstance(c, int) else pl.ds(pl.multiple_of(c * 128, 128), 128)

    def par_copies(c):
        return [pltpu.make_async_copy(src.at[:, lanes(c)], par.at[c, i], par_sem.at[c, i])
                for i, src in enumerate((are_hbm, aim_hbm, bre_hbm, bim_hbm, cre_hbm, cim_hbm))]

    def tile_copies(c):
        return [pltpu.make_async_copy(x_hbm.at[:, lanes(c)], xs.at[c], x_sem.at[c]),
                pltpu.make_async_copy(wqkv_hbm.at[lanes(c), :], wraw.at[c], w_sem.at[c]),
                pltpu.make_async_copy(wo_hbm.at[:, lanes(c)], woraw.at[c], wo_sem.at[c])]

    km_copy = pltpu.make_async_copy(kmat_hbm, kmat, km_sem.at[0])

    lane = jax.lax.broadcasted_iota(jnp.int32, (8, 128), 1)
    row = jax.lax.broadcasted_iota(jnp.int32, (8, 128), 0)
    low = lane < 64
    never = zero_ref[...] != 0

    def paced(panels, rows, values):
        groups = rows // 16
        regs = [[panel(g) for panel in panels] for g in range(groups)]
        order = [(g, c) for g in range(groups) for c in range(len(panels))]
        for n, val in enumerate(values):
            g, c = order[n * len(order) // len(values)]
            regs[g][c] = jnp.where(never, _words(val), regs[g][c])
        return _halves(jnp.concatenate([jnp.concatenate(r, axis=1) for r in regs], axis=0))

    dt_row = jnp.exp(ldt_ref[...].astype(F32).reshape(1, D)).astype(BF16).astype(F32)
    for c in range(NT):
        dts[c] = jnp.broadcast_to(dt_row[:, c * 128:(c + 1) * 128], (8, 128))

    def discretize(c):
        dt = dts[c][0:1, :]
        cols = [[] for _ in range(4)]
        raw = [par[c, i].astype(F32) for i in range(6)]
        for r in range(NS // 16):
            a_re, a_im, b_re, b_im, c_re, c_im = (v[16 * r:16 * r + 16] for v in raw)
            mag, ang = jnp.exp(dt * a_re), dt * a_im
            db_re, db_im = dt * b_re, dt * b_im
            vals = (mag * jnp.cos(ang), mag * jnp.sin(ang),
                    c_re * db_re - c_im * db_im, c_re * db_im + c_im * db_re)
            for col, val in zip(cols, vals):
                col.append(val)
            yield [vals[0][:8], vals[1][:8]]
            yield [vals[0][8:], vals[1][8:]]
        for i in range(2):
            re, im = jnp.concatenate(cols[2 * i], axis=0), jnp.concatenate(cols[2 * i + 1], axis=0)
            zw[c % 2, 4 * i + 0] = re[:128].T
            zw[c % 2, 4 * i + 1] = im[:128].T
            zw[c % 2, 4 * i + 2] = jnp.concatenate([re[128:], re[128:]], axis=0).T
            zw[c % 2, 4 * i + 3] = jnp.concatenate([-im[128:], im[128:]], axis=0).T

    def put(tile, slot, even, odd):
        for comp in range(len(even)):
            tab[tile % 2, comp, pl.ds(16 * slot, 8, stride=2), :] = even[comp]
            tab[tile % 2, comp, pl.ds(16 * slot + 1, 8, stride=2), :] = odd[comp]

    def get(group, slot, comps):
        tile, half = divmod(group, 2)
        return tuple(tab[tile % 2, comp, pl.ds(16 * slot + 8 * half, 8), :] for comp in range(comps))

    def running(z, conj=False):
        x, y, p, q = z
        if conj:
            return (x, -y, jnp.where(low, p, -q))
        return (x, y, jnp.where(low, p, q), jnp.where(low, -q, p))

    def tables(c, tile):
        rows = slice(8 * tile, 8 * tile + 8)
        one = (jnp.ones((8, 128), F32), jnp.zeros((8, 128), F32)) * 2
        pw = {1: tuple(zw[c % 2, i, rows, :] for i in range(4))}
        w = tuple(zw[c % 2, 4 + i, rows, :] for i in range(4))
        e = 1
        while e < S:
            pw[2 * e] = _csq(pw[e])
            e *= 2
        z24 = _cmul(pw[16], pw[8])
        put(tile, _Q_V, running(one, True), running(pw[8], True))
        put(tile, _Q_V + 1, running(pw[16], True), running(z24, True))
        x, y, p, q = pw[16]
        rec = (x + x, x * x + y * y, p + p, p * p + q * q)
        put(tile, _Q_REC, rec, rec)
        yield list(z24 + rec)
        first = [w] + [_cmul(w, pw[e]) for e in _BASE[1:]]
        second = [_cmul(f, pw[off[1]]) if off[1] else f for f, off in zip(first, _OFF)]
        step = [pw[off[2]] if off[2] else one for off in _OFF]
        for i in range(3):
            put(tile, _Q_W + i, running(first[2 * i]), running(first[2 * i + 1]))
            put(tile, _Q_W + 3 + i, running(second[2 * i]), running(second[2 * i + 1]))
            put(tile, _Q_G + i, step[2 * i], step[2 * i + 1])
        yield [v for f in second for v in f]

    def operand(rows):
        return jnp.concatenate([jnp.concatenate(parts, axis=1) for parts in rows], axis=0).astype(BF16)

    chan = row // 2
    slot_of_lane = ((lane // 2) - chan) % 4

    def generate(c, riders, extra):
        base = c % 2 * 256 if isinstance(c, int) else pl.multiple_of(c % 2 * 256, 256)
        _take(tables(c, 0), 2)
        res, stage2, stage3 = None, [], []
        for group in range(32 + 3):
            for i, r in enumerate(stage3):
                rs[i, pl.ds(base + 8 * (group - 3), 8), :] = jnp.where(
                    (chan & 2) == 2, pltpu.roll(r, 128 - 4, 1), r)
            stage3 = [jnp.where((chan & 1) == 1, pltpu.roll(r, 128 - 2, 1), r) for r in stage2]
            stage2 = []
            for i in range(3 if res is not None else 0):
                r = res[8 * i:8 * i + 8]
                for a in range(1, 4):
                    blk = res[24 * a + 8 * i:24 * a + 8 * i + 8]
                    r = jnp.where(slot_of_lane == a, pltpu.roll(blk, 2 * a, 1), r)
                stage2.append(r)
            res = None
            if group < 32:
                if group % 2 == 0:
                    ahead = tables(c, group // 2 + 1) if group + 2 < 32 else iter(())
                pace = _take(extra, 1) + _take(ahead, 1)
                ride = riders[group * len(riders) // 32:(group + 1) * len(riders) // 32]
                for n, rider in enumerate(ride):
                    rider(pace[n * len(pace) // len(ride):(n + 1) * len(pace) // len(ride)])
                v = [get(group, _Q_V, 3), get(group, _Q_V + 1, 3)]
                a_lo, b_lo, a_hi, b_hi = get(group, _Q_REC, 4)
                for i in range(2, 16):
                    v.append(tuple(al * v1 - be * v0 for al, be, v1, v0 in
                                   zip((a_lo, a_lo, a_hi), (b_lo, b_lo, b_hi), v[i - 1], v[i - 2])))
                u = [get(group, _Q_W + n, 4) for n in range(6)]
                m = [get(group, _Q_G + i, 4) for i in range(3)] * 2
                lhs = [part[:3] for part in u] + [
                    (x * mx - y * my, y * mx + x * my, t * mp + s * mq)
                    for (x, y, t, s), (mx, my, mp, mq) in zip(u, m)]
                res = jax.lax.dot_general(operand(lhs), operand(v), _NT_DIMS, preferred_element_type=F32)
        _take(extra, NS)

    def dft_passes(c):
        base = c % 2 * 256 if isinstance(c, int) else pl.multiple_of(c % 2 * 256, 256)
        tiles, partial = {}, {}

        def kernel_pass(m, t, idx, last):
            def run(values):
                if t not in tiles:
                    tiles[t] = rs[t // 2, pl.ds(base + t % 2, 128, stride=2), :].astype(BF16)
                lhs = paced([lambda g: kmat[idx, 8 * g:8 * g + 8, :]], 2 * T, values)
                part = jax.lax.dot_general(lhs, tiles[t], _NT_DIMS, preferred_element_type=F32)
                partial[m] = part if m not in partial else partial[m] + part
                if last:
                    spec[NT + c, m] = partial[m]
            return run

        def signal_pass(m):
            def run(values):
                lhs = paced([lambda g: fwd_ref[8 * g:8 * g + 8, :]], 2 * T, values)
                block = xs[c, m * T:(m + 1) * T, :]
                xw[c, m * T // 2:(m + 1) * T // 2, :] = _words(block)
                spec[c, m] = jnp.dot(lhs, block, preferred_element_type=F32)
            return run

        runs = []
        for m in range(NB):
            runs += [kernel_pass(m, t, idx, n + 1 == len(_KPASSES[m])) for n, (t, idx) in enumerate(_KPASSES[m])]
            runs.append(signal_pass(m))
        return runs

    def permute_weights(c):
        for part in range(3):
            for n in range(NT):
                col = part * D + n * 128
                tmp[part, n * 128:(n + 1) * 128, :] = wraw[c, :, col:col + 128].astype(F32).T
            for j in range(DH):
                wt[c, pl.ds((part * D + j * H) // 2, H // 2), :] = _words(
                    tmp[part, pl.ds(j, H, stride=DH), :].astype(BF16))
        tmp[3] = woraw[c].astype(F32)
        for j in range(DH):
            wop[c, pl.ds(j * H // 2, H // 2), :] = _words(tmp[3, pl.ds(j, H, stride=DH), :].astype(BF16))

    with jax.named_scope("P0"):
        for cp in par_copies(0) + par_copies(1):
            cp.start()
        for cp in par_copies(0):
            cp.wait()
        km_copy.start()
        for cp in tile_copies(0):
            cp.start()
        for c in range(2, NT):
            for cp in par_copies(c):
                cp.start()
        _take(discretize(0), NS)
        for cp in par_copies(1):
            cp.wait()
        generate(0, [], discretize(1))
        for c in range(1, NT):
            for cp in tile_copies(c):
                cp.start()
        km_copy.wait()
        for c in range(2, NT):
            for cp in par_copies(c):
                cp.wait()

    def ssm_step(c, carry):
        for cp in tile_copies(c - 1):
            cp.wait()
        permute_weights(c - 1)
        generate(c, dft_passes(c - 1), discretize(c + 1))
        return carry

    with jax.named_scope("P1"):
        jax.lax.fori_loop(1, NT - 1, ssm_step, 0)
    with jax.named_scope("P1b"):
        for cp in tile_copies(NT - 2) + tile_copies(NT - 1):
            cp.wait()
        permute_weights(NT - 2)
        generate(NT - 1, dft_passes(NT - 2), iter(()))
        permute_weights(NT - 1)
        for run in dft_passes(NT - 1):
            run([])

    for c in range(NT):
        ks[c, 0:PAD, :] = jnp.zeros((PAD, 128), F32)
        vs[c, 0:PAD, :] = jnp.zeros((PAD, 128), F32)
    q_scale = float(DH ** -0.5 * np.log2(np.e))
    n2 = S // M2
    ft_per_step = (T // 8) // n2

    def causal(a, b, j):
        acc = a[0] * b[j]
        for i in range(1, j + 1):
            acc = acc + a[i] * b[j - i]
        return acc

    even_order = [j for i in range(NB // 2) for j in (i, NB - 1 - i)]

    def convolve(it):
        for f in range(ft_per_step):
            ft = (it * ft_per_step + f) // 2 + f % 2 * (T // 16)
            plus, minus = (jnp.subtract, jnp.add) if f % 2 else (jnp.add, jnp.subtract)
            for c in range(NT):
                def load(slab, part, phase):
                    rows = pl.ds(pl.multiple_of(origin_ref[phase] + part * T + ft * 8, 8), 8)
                    return [spec[slab, m, rows, :] for m in range(NB)]

                k_re, k_im = load(NT + c, 0, 0), load(NT + c, 1, 0)
                a = [u + v for u, v in zip(load(c, 0, 0), load(c, 1, 0))]
                b = [k_re[0]] + [minus(k_re[m], k_im[m - 1]) for m in range(1, NB)]
                s1, s2 = {}, {}
                for j in even_order:
                    s1[j] = causal(a, b, j)
                    yield s1[j]
                k_re, k_im = load(NT + c, 0, 1), load(NT + c, 1, 1)
                a = load(c, 0, 1)
                b = [k_im[0] - k_re[0]] + [plus(k_im[m] - k_re[m], k_im[m - 1] + k_re[m - 1]) for m in range(1, NB)]
                for j in even_order:
                    s2[j] = causal(a, b, j)
                    yield s2[j]
                k_re, k_im = load(NT + c, 0, 2), load(NT + c, 1, 2)
                a = load(c, 1, 2)
                b = [-k_im[0] - k_re[0]] + [
                    (k_re[m - 1] - k_im[m - 1] if f % 2 else k_im[m - 1] - k_re[m - 1]) - (k_im[m] + k_re[m])
                    for m in range(1, NB)]
                for j in even_order:
                    z = jnp.concatenate([s1[j], s1[j]], axis=0) + jnp.concatenate([causal(a, b, j), s2[j]], axis=0)
                    z = _words(z.astype(BF16))
                    zs[j, c, pl.ds(pl.multiple_of(ft * 8, 8), 8), :] = z
                    yield z

    def scores(r0):
        for tile in range(M2 // 8):
            t0 = 8 * tile
            q = [qs[c, t0:t0 + 8, :] for c in range(NT)]
            for w in range(WIN):
                src = pl.ds(r0 + (t0 + PAD - DIL * w), 8)
                acc = q[0] * ks[0, src, :]
                for c in range(1, NT):
                    acc = acc + q[c] * ks[c, src, :]
                ps[w, pl.ds(r0 + t0, 8), :] = acc
                yield acc

    def proj_step(it, carry):
        r0 = pl.multiple_of(it * M2, M2)
        conv, dots = convolve(it), scores(r0)
        x_panel = lambda c: lambda g: xw[c, pl.ds(pl.multiple_of(it * (M2 // 2), 8) + 8 * g, 8), :]
        place = lambda n, base: ((qs, ks, vs)[n // NT], (n % NT, pl.ds(base + (r0 + PAD if n >= NT else 0), M2)))
        todo, slots = 3 * NB * NT * ft_per_step, 0
        for n in range(3 * NT):
            if n % 4 == 0:
                hi = min(n + 4, 3 * NT)
                count = EARLY * todo * (slots + 1) // 260 - EARLY * todo * slots // 260 if slots < 13 else 0
                slots += 1
                xb = paced([x_panel(NT - 1)], M2, list(itertools.islice(conv, count)))
                tail = jax.lax.dot_general(xb, _halves(wt[NT - 1, n * 64:hi * 64, :]), _NT_DIMS,
                                           preferred_element_type=F32)
                for i in range(n, hi):
                    ref, idx = place(i, 0)
                    ref[idx] = tail[:, (i - n) * 128:(i - n + 1) * 128]
            if n < 2 * NT:
                count = EARLY * todo * (slots + 1) // 260 - EARLY * todo * slots // 260
                values = list(itertools.islice(conv, count))
            else:
                left = 3 * NT - n
                values = list(itertools.islice(conv, -(-(todo - EARLY * todo // 20) // NT)))
                values += list(itertools.islice(dots, M2 * (NT - left + 1) // NT - M2 * (NT - left) // NT))
            slots += 1
            xb = paced([x_panel(c) for c in range(NT - 1)], M2, values)
            w = _halves(jnp.concatenate([wt[c, n * 64:(n + 1) * 64, :] for c in range(NT - 1)], axis=1))
            ref, idx = place(n, pl.multiple_of(origin_ref[0], 8))
            res = jax.lax.dot_general(xb, w, _NT_DIMS, preferred_element_type=F32) + ref[idx]
            ref, idx = place(n, 0)
            ref[idx] = res if n >= NT else res * q_scale
        assert next(conv, None) is None and next(dots, None) is None
        return carry

    with jax.named_scope("P2"):
        jax.lax.fori_loop(0, n2, proj_step, 0)

    def attend(blk, first):
        r0 = 0 if first else pl.multiple_of(blk * M3, M3)
        stage1 = stage2 = None
        for pair in range(M3 // 16 + 2):
            logit = None if stage2 is None else [a + pltpu.roll(a, 32, 1) for a in stage2]
            stage2 = None if stage1 is None else [a + pltpu.roll(a, 64, 1) for a in stage1]
            stage1 = [ps[w, pl.ds(r0 + 16 * pair, 16), :] for w in range(WIN)] if pair < M3 // 16 else None
            if logit is None:
                continue
            t0 = 16 * (pair - 2)
            if first and t0 == 0:
                pos = jax.lax.broadcasted_iota(jnp.int32, (16, 128), 0)
                logit = [jnp.where(pos >= DIL * w, l, -1e9) if w else l for w, l in enumerate(logit)]
            top = logit[0]
            for w in range(1, WIN):
                top = jnp.maximum(top, logit[w])
            e = [jnp.exp2(l - top) for l in logit]
            den = e[0]
            for w in range(1, WIN):
                den = den + e[w]
            inv = pl.reciprocal(den, approx=True)
            inv = inv * (2.0 - den * inv)
            yield inv[0:8]
            yield inv[8:16]
            for c in range(NT):
                acc = e[0] * vs[c, pl.ds(r0 + (t0 + PAD), 16), :]
                for w in range(1, WIN):
                    acc = acc + e[w] * vs[c, pl.ds(r0 + (t0 + PAD - DIL * w), 16), :]
                o = _words((acc * inv).astype(BF16))
                os_[blk % 2, c, t0 // 2:t0 // 2 + 8, :] = o
                yield o

    def out_copy(blk, c):
        rows = pl.ds(pl.multiple_of(blk * M3, M3), M3)
        return pltpu.make_async_copy(outs.at[c, rows], out_hbm.at[rows, lanes(c)], out_sem.at[blk, c])

    def gates(blk):
        r0 = 0 if isinstance(blk, int) else pl.multiple_of(blk * (M3 // 2), 8)
        gw_row = gw_ref[...].astype(F32).reshape(1, D)
        for g in range(M3 // 16):
            rows = pl.ds(r0 + 8 * g, 8)
            score = _halves(xw[0, rows, :]).astype(F32) * gw_row[:, 0:128]
            for c in range(1, NT):
                score = score + _halves(xw[c, rows, :]).astype(F32) * gw_row[:, c * 128:(c + 1) * 128]
            gate = jnp.broadcast_to(jax.nn.sigmoid(jnp.sum(score, axis=1, keepdims=True)), (16, 128))
            gs[blk % 2, 16 * g:16 * g + 16, :] = gate
            yield gate[8:16]

    def finish(blk, work, total):
        rows = pl.ds(pl.multiple_of(blk * M3, M3), M3)
        word_rows = pl.ds(pl.multiple_of(blk * (M3 // 2), 8), M3 // 2)
        dskip_row = dskip_ref[...].astype(F32).reshape(1, D)
        spent = [0]

        def pull(cost):
            lo, spent[0] = spent[0], spent[0] + cost
            share = lambda t: total * max(t - LEAD, 0) // (35 - LEAD)
            return list(itertools.islice(work, share(spent[0]) - share(lo)))

        o_panel = lambda c: lambda g: oc[c, 8 * g:8 * g + 8, :]
        inv_panels = [lambda g, k=k: inv_ref[k, 8 * g:8 * g + 8, :] for k in range(2)]
        oc[...] = os_[blk % 2]
        for lo, hi in ((0, 4), (4, 5)):
            w = _halves(jnp.concatenate([wop[c, 256:320, :] for c in range(lo, hi)], axis=1))
            tail = jnp.dot(paced([o_panel(NT - 1)], M3, pull(hi - lo)), w, preferred_element_type=F32)
            for c in range(lo, hi):
                att[c] = tail[:, (c - lo) * 128:(c - lo + 1) * 128]
        for lo, hi in ((0, 2), (2, 4), (4, 5)):
            for i in range(M3 // T):
                z = _halves(jnp.concatenate([zs[blk * (M3 // T) + i, c] for c in range(lo, hi)], axis=1))
                y = jnp.dot(paced(inv_panels, T, pull(hi - lo)), z, preferred_element_type=F32)
                for c in range(lo, hi):
                    ys[c, i * T:(i + 1) * T, :] = y[:, (c - lo) * 128:(c - lo + 1) * 128]
        back = pl.ds(pl.multiple_of(origin_ref[0], 8), M3)
        for c in range(NT):
            mixed = jnp.dot(paced([o_panel(k) for k in range(NT - 1)], M3, pull(4)), _halves(wop[c, 0:256, :]),
                            preferred_element_type=F32) + att[c, back, :]
            ssm = ys[c, back, :] + _halves(xw[c, word_rows, :]).astype(F32) * dskip_row[:, c * 128:(c + 1) * 128]
            outs[c, rows, :] = (ssm + gs[blk % 2] * (mixed - ssm)).astype(BF16)
        assert next(work, None) is None

    for _ in itertools.chain(attend(0, True), gates(0)):
        pass

    def out_step(it, carry):
        finish(it, itertools.chain(attend(it + 1, False), gates(it + 1)), M3 // 16 * (NT + 3))
        for c in range(NT):
            out_copy(it, c).start()
        return carry

    n3 = S // M3
    with jax.named_scope("P3"):
        jax.lax.fori_loop(0, n3 - 1, out_step, 0)
    with jax.named_scope("P4"):
        finish(n3 - 1, iter(()), 0)
        for c in range(NT):
            out_copy(n3 - 1, c).start()
        for blk in range(n3):
            for c in range(NT):
                out_copy(blk, c).wait()


@jax.jit
def pallas_gated_mix__sliding_local_dilated__ssm_conv_s4__prompt_kernel(
    A_x: jax.Array,
    A_wqkv: jax.Array,
    A_wo: jax.Array,
    B_u: jax.Array,
    B_A_re: jax.Array,
    B_A_im: jax.Array,
    B_B_re: jax.Array,
    B_B_im: jax.Array,
    B_C_re: jax.Array,
    B_C_im: jax.Array,
    B_log_dt: jax.Array,
    B_Dskip: jax.Array,
    gate_w: jax.Array,
):
    del B_u
    assert A_x.shape == (1, S, D) and B_A_re.shape == (D, NS) and B_A_re.dtype == BF16
    hbm = pl.BlockSpec(memory_space=pl.ANY)
    vmem = pl.BlockSpec(memory_space=pltpu.VMEM)
    out = pl.pallas_call(
        _kernel,
        out_shape=jax.ShapeDtypeStruct((S, D), BF16),
        in_specs=[hbm] * 10 + [vmem] * 6 + [pl.BlockSpec(memory_space=pltpu.SMEM)],
        out_specs=hbm,
        scratch_shapes=[
            pltpu.VMEM((NT, S, 128), BF16),
            pltpu.VMEM((NT, S // 2, 128), jnp.int32),
            pltpu.VMEM((NT, 128, 3 * D), BF16),
            pltpu.VMEM((NT, D, 128), BF16),
            pltpu.VMEM(_KMATS.shape, jnp.int32),
            pltpu.VMEM((NT, 6, NS, 128), BF16),
            pltpu.VMEM((NT, 3 * D // 2, 128), jnp.int32),
            pltpu.VMEM((NT, D // 2, 128), jnp.int32),
            pltpu.VMEM((4, D, 128), F32),
            pltpu.VMEM((NT, 8, 128), F32),
            pltpu.VMEM((2, 8, 128, 128), F32),
            pltpu.VMEM((2, 4, 16 * _NQ, 128), F32),
            pltpu.VMEM((3, 512, 128), F32),
            pltpu.VMEM((2 * NT, NB, 2 * T, 128), F32),
            pltpu.VMEM((NB, NT, T, 128), jnp.int32),
            pltpu.VMEM((NT, M2, 128), F32),
            pltpu.VMEM((NT, S + PAD, 128), F32),
            pltpu.VMEM((NT, S + PAD, 128), F32),
            pltpu.VMEM((WIN, S, 128), F32),
            pltpu.VMEM((2, NT, M3 // 2, 128), jnp.int32),
            pltpu.VMEM((NT, M3 // 2, 128), jnp.int32),
            pltpu.VMEM((2, M3, 128), F32),
            pltpu.VMEM((NT, M3, 128), F32),
            pltpu.VMEM((NT, M3, 128), F32),
            pltpu.VMEM((NT, S, 128), BF16),
            pltpu.SemaphoreType.DMA((NT,)),
            pltpu.SemaphoreType.DMA((NT,)),
            pltpu.SemaphoreType.DMA((NT,)),
            pltpu.SemaphoreType.DMA((1,)),
            pltpu.SemaphoreType.DMA((NT, 6)),
            pltpu.SemaphoreType.DMA((S // M3, NT)),
        ],
        compiler_params=pltpu.CompilerParams(vmem_limit_bytes=100 * 1024 * 1024),
    )(
        A_x.reshape(S, D), A_wqkv, A_wo, _KMATS,
        B_A_re.T, B_A_im.T, B_B_re.T, B_B_im.T, B_C_re.T, B_C_im.T,
        B_log_dt, B_Dskip, gate_w, _FWD, _INV, np.zeros((8, 128), np.int32), np.zeros((4,), np.int32),
    )
    return out.reshape(1, S, D)
```

```python
import itertools

import ml_dtypes
import numpy as np

import jax
import jax.numpy as jnp
import jax.experimental.pallas as pl
import jax.experimental.pallas.tpu as pltpu

F32 = jnp.float32
BF16 = jnp.bfloat16

S = 2048
D = 640
NS = 192
H = 32
DH = D // H
WIN, DIL = 8, 2
T = 128
NB = S // T
NT = D // 128
PAD = 16
M2 = 256
RELEASE = 11
LAG_S = 8
LEAD = 0
LAG_D = 4
LAG_T = 4
LAG_V = 4
LAG_U = 4
EARLY = 20
M3 = 256

_BASE = (0, 4, 256, 512, 1024, 2048)
_OFF = ((0, 1, 2, 3), (0, 1, 2, 3), (0, 2, 4, 6), (0, 4, 256, 260), (0, 256, 512, 768), (0, 0, 0, 0))


def _dft_constants():
    k = np.concatenate([np.arange(0, T, 2), np.arange(1, T, 2)])
    theta = 2.0 * np.pi * (k + 0.5) / (2 * T)
    ang = theta[:, None] * np.arange(T)[None, :]
    fwd = np.concatenate([np.cos(ang), -np.sin(ang)], axis=0)
    inv = np.stack([np.cos(ang).reshape(T // 8, 8, T), -np.sin(ang).reshape(T // 8, 8, T)], axis=1)
    inv = inv.reshape(2 * T, T).T / T
    slot = {}
    for t in range(len(_BASE)):
        for lane in range(128):
            i, a, p = lane // 8, (lane % 8) // 2, lane % 2
            slot.setdefault(_BASE[t] + _OFF[t][a] + 8 * (2 * i + p), (t, lane))
    lag = np.arange(S).astype(np.float32).astype(ml_dtypes.bfloat16).astype(np.float64).astype(np.int64)
    mats, passes = [], []
    for m in range(NB):
        per_tile = {}
        for n in range(T):
            t, lane = slot[int(lag[m * T + n])]
            per_tile.setdefault(t, np.zeros((2 * T, 128)))[:, lane] += fwd[:, n]
        passes.append(tuple((t, len(mats) + j) for j, t in enumerate(sorted(per_tile))))
        mats.extend(per_tile[t] for t in sorted(per_tile))

    def to_bf16(a):
        bits = np.asarray(a, np.float32).astype(ml_dtypes.bfloat16).view(np.uint16).astype(np.uint32)
        return (bits[..., 0::2, :] | (bits[..., 1::2, :] << 16)).view(np.int32)

    inv = inv.reshape(T, 2, T).transpose(1, 0, 2)
    return to_bf16(fwd), to_bf16(inv), to_bf16(np.stack(mats)), tuple(passes)


_FWD, _INV, _KMATS, _KPASSES = _dft_constants()

_Q_W, _Q_G, _Q_V, _Q_REC, _NQ = 0, 6, 9, 11, 12

_NT_DIMS = (((1,), (1,)), ((), ()))


def _csq(z):
    x, y, p, q = z
    return ((x - y) * (x + y), (x + x) * y, (p - q) * (p + q), (p + p) * q)


def _cmul(a, b):
    ax, ay, ap, aq = a
    bx, by, bp, bq = b
    return (ax * bx - ay * by, ax * by + ay * bx, ap * bp - aq * bq, ap * bq + aq * bp)


def _words(v):
    return pltpu.bitcast(v, jnp.int32)


def _halves(v):
    return pltpu.bitcast(v, BF16)


def _take(gen, n):
    out = []
    for _ in range(n):
        out += next(gen, [])
    return out


def _kernel(x_hbm, wqkv_hbm, wo_hbm, kmat_hbm, are_hbm, aim_hbm, bre_hbm, bim_hbm, cre_hbm, cim_hbm,
            ldt_ref, dskip_ref, gw_ref, fwd_ref, inv_ref, zero_ref, origin_ref,
            out_hbm,
            xs, xw, wraw, woraw, kmat, par, wt, wop, tmp, dts, disc, zw, tab, rs, kt, spec, zs, qs, ks, vs, ps, ls, os_, oc, gs, att, ys, outs,
            x_sem, w_sem, wo_sem, km_sem, par_sem, out_sem):
    def lanes(c):
        return pl.ds(c * 128, 128) if isinstance(c, int) else pl.ds(pl.multiple_of(c * 128, 128), 128)

    def par_copies(c):
        return [pltpu.make_async_copy(src.at[:, lanes(c)], par.at[c, i], par_sem.at[c, i])
                for i, src in enumerate((are_hbm, aim_hbm, bre_hbm, bim_hbm, cre_hbm, cim_hbm))]

    def tile_copies(c):
        return [pltpu.make_async_copy(x_hbm.at[:, lanes(c)], xs.at[c], x_sem.at[c]),
                pltpu.make_async_copy(wqkv_hbm.at[lanes(c), :], wraw.at[c], w_sem.at[c]),
                pltpu.make_async_copy(wo_hbm.at[:, lanes(c)], woraw.at[c], wo_sem.at[c])]

    km_copy = pltpu.make_async_copy(kmat_hbm, kmat, km_sem.at[0])

    lane = jax.lax.broadcasted_iota(jnp.int32, (8, 128), 1)
    row = jax.lax.broadcasted_iota(jnp.int32, (8, 128), 0)
    low = lane < 64
    never = zero_ref[...] != 0

    def behind(val, earlier):
        return val if earlier is None else jnp.where(never, earlier, val)

    def paced(panels, rows, values):
        groups = rows // 16
        regs = [[panel(g) for panel in panels] for g in range(groups)]
        order = [(g, c) for g in range(groups) for c in range(len(panels))]
        for n, val in enumerate(values):
            g, c = order[n * len(order) // len(values)]
            regs[g][c] = jnp.where(never, _words(val), regs[g][c])
        return _halves(jnp.concatenate([jnp.concatenate(r, axis=1) for r in regs], axis=0))

    dt_row = jnp.exp(ldt_ref[...].astype(F32).reshape(1, D)).astype(BF16).astype(F32)
    for c in range(NT):
        dts[c] = jnp.broadcast_to(dt_row[:, c * 128:(c + 1) * 128], (8, 128))

    def discretize(c, past):
        dt = dts[c][0:1, :]
        for r in range(NS // 32):
            raw = [par[c, i, 32 * r:32 * r + 32, :].astype(F32) for i in range(6)]
            for n in range(4):
                a_re, a_im, b_re, b_im, c_re, c_im = (v[8 * n:8 * n + 8] for v in raw)
                mag, ang = jnp.exp(dt * a_re), behind(dt * a_im, past[-LAG_D])
                db_re, db_im = dt * b_re, dt * b_im
                vals = (mag * jnp.cos(ang), mag * jnp.sin(ang),
                        c_re * db_re - c_im * db_im, c_re * db_im + c_im * db_re)
                for i, val in enumerate(vals):
                    disc[i, 32 * r + 8 * n:32 * r + 8 * n + 8, :] = val
                yield list(vals[:2])
        for i in range(2):
            zw[c % 2, 4 * i + 0] = disc[2 * i, 0:128, :].T
            zw[c % 2, 4 * i + 1] = disc[2 * i + 1, 0:128, :].T
            yield []
            re, im = disc[2 * i, 128:NS, :], disc[2 * i + 1, 128:NS, :]
            zw[c % 2, 4 * i + 2] = jnp.concatenate([re, re], axis=0).T
            zw[c % 2, 4 * i + 3] = jnp.concatenate([-im, im], axis=0).T
            yield []

    def put(tile, slot, even, odd):
        for comp in range(len(even)):
            tab[tile % 2, comp, pl.ds(16 * slot, 8, stride=2), :] = even[comp]
            tab[tile % 2, comp, pl.ds(16 * slot + 1, 8, stride=2), :] = odd[comp]

    def get(group, slot, comps):
        tile, half = divmod(group, 2)
        return tuple(tab[tile % 2, comp, pl.ds(16 * slot + 8 * half, 8), :] for comp in range(comps))

    def running(z, conj=False):
        x, y, p, q = z
        if conj:
            return (x, -y, jnp.where(low, p, -q))
        return (x, y, jnp.where(low, p, q), jnp.where(low, -q, p))

    def tables(c, tile, earlier):
        rows = slice(8 * tile, 8 * tile + 8)
        one = (jnp.ones((8, 128), F32), jnp.zeros((8, 128), F32)) * 2
        pw = {1: tuple(behind(zw[c % 2, i, rows, :], earlier if i % 2 == 0 else None) for i in range(4))}
        w = tuple(zw[c % 2, 4 + i, rows, :] for i in range(4))
        e = 1
        while e < S:
            pw[2 * e] = _csq(pw[e])
            e *= 2
        z24 = _cmul(pw[16], pw[8])
        put(tile, _Q_V, running(one, True), running(pw[8], True))
        put(tile, _Q_V + 1, running(pw[16], True), running(z24, True))
        x, y, p, q = pw[16]
        rec = (x + x, x * x + y * y, p + p, p * p + q * q)
        put(tile, _Q_REC, rec, rec)
        yield list(z24 + rec)
        first = [w] + [_cmul(w, pw[e]) for e in _BASE[1:]]
        second = [_cmul(f, pw[off[1]]) if off[1] else f for f, off in zip(first, _OFF)]
        step = [pw[off[2]] if off[2] else one for off in _OFF]
        for i in range(3):
            put(tile, _Q_W + i, running(first[2 * i]), running(first[2 * i + 1]))
            put(tile, _Q_W + 3 + i, running(second[2 * i]), running(second[2 * i + 1]))
            put(tile, _Q_G + i, step[2 * i], step[2 * i + 1])
        yield [v for f in second for v in f]

    def operand(panels):
        return jnp.concatenate([jnp.concatenate(parts, axis=0) for parts in panels], axis=1).astype(BF16)

    chan = row // 2
    slot_of_lane = ((lane // 2) - chan) % 4

    def generate(c, riders, upcoming, chores):
        base = c % 2 * 256 if isinstance(c, int) else pl.multiple_of(c % 2 * 256, 256)
        _take(tables(c, 0, None), 2)
        res, stage2, stage3, past = None, [], [], [None] * 8
        extra = discretize(c + 1, past) if upcoming else iter(())
        for group in range(32 + 3):
            for i, r in enumerate(stage3):
                rs[i, pl.ds(base + 8 * (group - 3), 8), :] = jnp.where(
                    (chan & 2) == 2, pltpu.roll(r, 128 - 4, 1), r)
            stage3 = [jnp.where((chan & 1) == 1, pltpu.roll(r, 128 - 2, 1), r) for r in stage2]
            stage2 = []
            for i in range(3 if res is not None else 0):
                r = res[8 * i:8 * i + 8]
                for a in range(1, 4):
                    blk = res[24 * a + 8 * i:24 * a + 8 * i + 8]
                    r = jnp.where(slot_of_lane == a, pltpu.roll(blk, 2 * a, 1), r)
                stage2.append(r)
            res = None
            if group < 32:
                if group % 2 == 0:
                    ahead = tables(c, group // 2 + 1, past[-LAG_T]) if group + 2 < 32 else iter(())
                _take(chores, 1)
                pace = _take(extra, 1) + _take(ahead, 1)
                ride = riders[group * len(riders) // 32:(group + 1) * len(riders) // 32]
                for n, rider in enumerate(ride):
                    rider(pace[n * len(pace) // len(ride):(n + 1) * len(pace) // len(ride)])
                a_lo, b_lo, a_hi, b_hi = get(group, _Q_REC, 4)
                rhs = []
                for al, be, v in zip((a_lo, a_lo, a_hi), (b_lo, b_lo, b_hi),
                                     zip(get(group, _Q_V, 3), get(group, _Q_V + 1, 3))):
                    v = [v[0], behind(v[1], past[-LAG_V])]
                    for i in range(2, 16):
                        v.append(al * v[i - 1] - be * v[i - 2])
                    rhs.append(v)
                u = [get(group, _Q_W + n, 4) for n in range(6)]
                m = [tuple(behind(g, past[-LAG_U]) for g in get(group, _Q_G + i, 4)) for i in range(3)] * 2
                lhs = [[v[0] for v in u] + [v[0] * g[0] - v[1] * g[1] for v, g in zip(u, m)],
                       [v[1] for v in u] + [v[1] * g[0] + v[0] * g[1] for v, g in zip(u, m)],
                       [v[2] for v in u] + [v[2] * g[2] + v[3] * g[3] for v, g in zip(u, m)]]
                res = jax.lax.dot_general(operand(lhs), operand(rhs), _NT_DIMS, preferred_element_type=F32)
                past.append(res[0:8] if riders else None)
        _take(extra, NS)
        _take(chores, NS)

    def dft_passes(c):
        base = c % 2 * 256 if isinstance(c, int) else pl.multiple_of(c % 2 * 256, 256)
        for t in range(len(_BASE)):
            kt[t] = _words(rs[t // 2, pl.ds(base + t % 2, 128, stride=2), :].astype(BF16))

        def kernel_pass(m):
            def run(values):
                lhs = paced([lambda g, idx=idx: kmat[idx, 8 * g:8 * g + 8, :] for _, idx in _KPASSES[m]],
                            2 * T, values)
                rhs = _halves(jnp.concatenate([kt[t] for t, _ in _KPASSES[m]], axis=1))
                spec[NT + c, m] = jax.lax.dot_general(lhs, rhs, _NT_DIMS, preferred_element_type=F32)
            return run

        def signal_pass(m):
            def run(values):
                lhs = paced([lambda g: fwd_ref[8 * g:8 * g + 8, :]], 2 * T, values)
                block = xs[c, m * T:(m + 1) * T, :]
                xw[c, m * T // 2:(m + 1) * T // 2, :] = _words(block)
                spec[c, m] = jnp.dot(lhs, block, preferred_element_type=F32)
            return run

        return [make(m) for m in range(NB) for make in (signal_pass, kernel_pass)]

    def permute_weights(c):
        for part in range(3):
            for n in range(NT):
                col = part * D + n * 128
                tmp[part, n * 128:(n + 1) * 128, :] = wraw[c, :, col:col + 128].astype(F32).T
                yield []
            for j in range(DH):
                wt[c, pl.ds((part * D + j * H) // 2, H // 2), :] = _words(
                    tmp[part, pl.ds(j, H, stride=DH), :].astype(BF16))
                if j % 7 == 6:
                    yield []
        tmp[3] = woraw[c].astype(F32)
        yield []
        for j in range(DH):
            wop[c, pl.ds(j * H // 2, H // 2), :] = _words(tmp[3, pl.ds(j, H, stride=DH), :].astype(BF16))
            if j % 7 == 6:
                yield []

    with jax.named_scope("P0"):
        for cp in par_copies(0) + par_copies(1):
            cp.start()
        for cp in par_copies(0):
            cp.wait()
        km_copy.start()
        for cp in tile_copies(0):
            cp.start()
        for c in range(2, NT):
            for cp in par_copies(c):
                cp.start()
        _take(discretize(0, [None] * 8), NS)
        for cp in par_copies(1):
            cp.wait()
        generate(0, [], True, iter(()))
        for c in range(1, NT):
            for cp in tile_copies(c):
                cp.start()
        km_copy.wait()
        for c in range(2, NT):
            for cp in par_copies(c):
                cp.wait()

    def ssm_step(c, carry):
        for cp in tile_copies(c - 1):
            cp.wait()
        generate(c, dft_passes(c - 1), True, permute_weights(c - 1))
        return carry

    with jax.named_scope("P1"):
        jax.lax.fori_loop(1, NT - 1, ssm_step, 0)
    with jax.named_scope("P1b"):
        for cp in tile_copies(NT - 2) + tile_copies(NT - 1):
            cp.wait()
        generate(NT - 1, dft_passes(NT - 2), False, permute_weights(NT - 2))
        chores = permute_weights(NT - 1)
        for run in dft_passes(NT - 1):
            _take(chores, 1)
            run([])
        _take(chores, NS)

    for c in range(NT):
        ks[c, 0:PAD, :] = jnp.zeros((PAD, 128), F32)
        vs[c, 0:PAD, :] = jnp.zeros((PAD, 128), F32)
    q_scale = float(DH ** -0.5 * np.log2(np.e))
    n2 = S // M2
    ft_per_step = (T // 8) // n2

    def causal(a, b, j):
        acc = a[0] * b[j]
        for i in range(1, j + 1):
            acc = acc + a[i] * b[j - i]
        return acc

    even_order = [j for i in range(NB // 2) for j in (i, NB - 1 - i)]

    def convolve(it):
        def tile_of(f):
            return (it * ft_per_step + f) // 2 + f % 2 * (T // 16)

        def operands(f, c, phase):
            def load(slab, part):
                rows = pl.ds(pl.multiple_of(origin_ref[phase] + part * T + tile_of(f) * 8, 8), 8)
                return [spec[slab, m, rows, :] for m in range(NB)]

            plus, minus = (jnp.subtract, jnp.add) if f % 2 else (jnp.add, jnp.subtract)
            k_re, k_im = load(NT + c, 0), load(NT + c, 1)
            if phase == 0:
                return ([u + v for u, v in zip(load(c, 0), load(c, 1))],
                        [k_re[0]] + [minus(k_re[m], k_im[m - 1]) for m in range(1, NB)])
            if phase == 1:
                return load(c, 0), [k_im[0] - k_re[0]] + [
                    plus(k_im[m] - k_re[m], k_im[m - 1] + k_re[m - 1]) for m in range(1, NB)]
            return load(c, 1), [-k_im[0] - k_re[0]] + [
                (k_re[m - 1] - k_im[m - 1] if f % 2 else k_im[m - 1] - k_re[m - 1]) - (k_im[m] + k_re[m])
                for m in range(1, NB)]

        jobs = [(f, c, phase) for f in range(ft_per_step) for c in range(NT) for phase in range(3)]
        ahead, sums = operands(*jobs[0]), [{}, {}, {}]
        for n, (f, c, phase) in enumerate(jobs):
            a, b = ahead
            for i, j in enumerate(even_order):
                val = sums[phase][j] = causal(a, b, j)
                if i == RELEASE and n + 1 < len(jobs):
                    spec[2 * NT, 0, pl.ds(pl.multiple_of(origin_ref[3], 8), 8), :] = val
                    ahead = operands(*jobs[n + 1])
                if phase == 2:
                    z = jnp.concatenate([sums[0][j]] * 2, axis=0) + jnp.concatenate([val, sums[1][j]], axis=0)
                    val = _words(z.astype(BF16))
                    zs[j, c, pl.ds(pl.multiple_of(tile_of(f) * 8, 8), 8), :] = val
                yield val

    def logits(r0):
        past = [None] * LAG_S
        for t0 in range(0, M2, 8):
            q = [qs[c, t0:t0 + 8, :] for c in range(NT)]
            q[0] = behind(q[0], past[-LAG_S])
            for w in range(WIN):
                src = pl.ds(r0 + (t0 + PAD - DIL * w), 8)
                acc = q[0] * ks[0, src, :]
                for c in range(1, NT):
                    acc = acc + q[c] * ks[c, src, :]
                acc = acc + pltpu.roll(acc, 64, 1)
                acc = acc + pltpu.roll(acc, 32, 1)
                ps[w, pl.ds(r0 + t0, 8), :] = acc
            past.append(acc)
            yield

    def proj_step(it, carry):
        r0 = pl.multiple_of(it * M2, M2)
        conv, dots = convolve(it), logits(r0)
        x_panel = lambda c: lambda g: xw[c, pl.ds(pl.multiple_of(it * (M2 // 2), 8) + 8 * g, 8), :]
        place = lambda n, base: ((qs, ks, vs)[n // NT], (n % NT, pl.ds(base + (r0 + PAD if n >= NT else 0), M2)))
        todo, slots = 3 * NB * NT * ft_per_step, 0
        for n in range(3 * NT):
            if n % 4 == 0:
                hi = min(n + 4, 3 * NT)
                count = EARLY * todo * (slots + 1) // 260 - EARLY * todo * slots // 260 if slots < 13 else 0
                slots += 1
                xb = paced([x_panel(NT - 1)], M2, list(itertools.islice(conv, count)))
                tail = jax.lax.dot_general(xb, _halves(wt[NT - 1, n * 64:hi * 64, :]), _NT_DIMS,
                                           preferred_element_type=F32)
                for i in range(n, hi):
                    ref, idx = place(i, 0)
                    ref[idx] = tail[:, (i - n) * 128:(i - n + 1) * 128]
            if n < 2 * NT:
                count = EARLY * todo * (slots + 1) // 260 - EARLY * todo * slots // 260
                values = list(itertools.islice(conv, count))
            else:
                values = list(itertools.islice(conv, -(-(todo - EARLY * todo // 20) // NT)))
                for _ in itertools.islice(dots, -(-(M2 // 8) // NT)):
                    pass
            slots += 1
            xb = paced([x_panel(c) for c in range(NT - 1)], M2, values)
            w = _halves(jnp.concatenate([wt[c, n * 64:(n + 1) * 64, :] for c in range(NT - 1)], axis=1))
            ref, idx = place(n, pl.multiple_of(origin_ref[0], 8))
            res = jax.lax.dot_general(xb, w, _NT_DIMS, preferred_element_type=F32) + ref[idx]
            ref, idx = place(n, 0)
            ref[idx] = res if n >= NT else res * q_scale
        assert next(conv, None) is None and next(dots, 0) == 0
        return carry

    with jax.named_scope("P2"):
        jax.lax.fori_loop(0, n2, proj_step, 0)

    def attend(blk):
        r0 = 0 if isinstance(blk, int) else pl.multiple_of(blk * M3, M3)
        for t0 in range(0, M3, 16):
            logit = [ps[w, pl.ds(r0 + t0, 16), :] for w in range(WIN)]
            if isinstance(blk, int) and t0 == 0:
                pos = jax.lax.broadcasted_iota(jnp.int32, (16, 128), 0)
                logit = [jnp.where(pos >= DIL * w, l, -1e9) if w else l for w, l in enumerate(logit)]
            top = logit[0]
            for w in range(1, WIN):
                top = jnp.maximum(top, logit[w])
            e = [jnp.exp2(l - top) for l in logit]
            den = e[0]
            for w in range(1, WIN):
                den = den + e[w]
            inv = pl.reciprocal(den, approx=True)
            inv = inv * (2.0 - den * inv)
            for c in range(NT):
                acc = e[0] * vs[c, pl.ds(r0 + (t0 + PAD), 16), :]
                for w in range(1, WIN):
                    acc = acc + e[w] * vs[c, pl.ds(r0 + (t0 + PAD - DIL * w), 16), :]
                o = _words((acc * inv).astype(BF16))
                os_[blk % 2, c, t0 // 2:t0 // 2 + 8, :] = o
                yield o

    def out_copy(blk, c):
        rows = pl.ds(pl.multiple_of(blk * M3, M3), M3)
        return pltpu.make_async_copy(outs.at[c, rows], out_hbm.at[rows, lanes(c)], out_sem.at[blk, c])

    def gates(blk):
        r0 = 0 if isinstance(blk, int) else pl.multiple_of(blk * (M3 // 2), 8)
        gw_row = gw_ref[...].astype(F32).reshape(1, D)
        for g in range(M3 // 16):
            rows = pl.ds(r0 + 8 * g, 8)
            score = _halves(xw[0, rows, :]).astype(F32) * gw_row[:, 0:128]
            for c in range(1, NT):
                score = score + _halves(xw[c, rows, :]).astype(F32) * gw_row[:, c * 128:(c + 1) * 128]
            gate = jnp.broadcast_to(jax.nn.sigmoid(jnp.sum(score, axis=1, keepdims=True)), (16, 128))
            gs[blk % 2, 16 * g:16 * g + 16, :] = gate
            yield

    def finish(blk, work, total):
        rows = pl.ds(pl.multiple_of(blk * M3, M3), M3)
        word_rows = pl.ds(pl.multiple_of(blk * (M3 // 2), 8), M3 // 2)
        dskip_row = dskip_ref[...].astype(F32).reshape(1, D)
        spent = [0]

        def pull(cost):
            lo, spent[0] = spent[0], spent[0] + cost
            share = lambda t: total * max(t - LEAD, 0) // (35 - LEAD)
            return list(itertools.islice(work, share(spent[0]) - share(lo)))

        o_panel = lambda c: lambda g: oc[c, 8 * g:8 * g + 8, :]
        inv_panels = [lambda g, k=k: inv_ref[k, 8 * g:8 * g + 8, :] for k in range(2)]
        oc[...] = os_[blk % 2]
        for lo, hi in ((0, 4), (4, 5)):
            w = _halves(jnp.concatenate([wop[c, 256:320, :] for c in range(lo, hi)], axis=1))
            tail = jnp.dot(paced([o_panel(NT - 1)], M3, pull(hi - lo)), w, preferred_element_type=F32)
            for c in range(lo, hi):
                att[c] = tail[:, (c - lo) * 128:(c - lo + 1) * 128]
        for lo, hi in ((0, 2), (2, 4), (4, 5)):
            for i in range(M3 // T):
                z = _halves(jnp.concatenate([zs[blk * (M3 // T) + i, c] for c in range(lo, hi)], axis=1))
                y = jnp.dot(paced(inv_panels, T, pull(hi - lo)), z, preferred_element_type=F32)
                for c in range(lo, hi):
                    ys[c, i * T:(i + 1) * T, :] = y[:, (c - lo) * 128:(c - lo + 1) * 128]
        back = pl.ds(pl.multiple_of(origin_ref[0], 8), M3)
        for c in range(NT):
            mixed = jnp.dot(paced([o_panel(k) for k in range(NT - 1)], M3, pull(4)), _halves(wop[c, 0:256, :]),
                            preferred_element_type=F32) + att[c, back, :]
            ssm = ys[c, back, :] + _halves(xw[c, word_rows, :]).astype(F32) * dskip_row[:, c * 128:(c + 1) * 128]
            outs[c, rows, :] = (ssm + gs[blk % 2] * (mixed - ssm)).astype(BF16)
        assert next(work, None) is None

    def prepare(blk):
        now, mix = attend(blk), gates(blk)
        for _ in range(M3 // 16):
            next(mix)
            yield from itertools.islice(now, NT)

    for _ in prepare(0):
        pass
    n3 = S // M3

    def out_step(it, carry):
        finish(it, prepare(it + 1), M3 // 16 * NT)
        for c in range(NT):
            out_copy(it, c).start()
        return carry

    with jax.named_scope("P3"):
        jax.lax.fori_loop(0, n3 - 1, out_step, 0)
    with jax.named_scope("P4"):
        finish(n3 - 1, iter(()), 0)
        for c in range(NT):
            out_copy(n3 - 1, c).start()
        for blk in range(n3):
            for c in range(NT):
                out_copy(blk, c).wait()


@jax.jit
def pallas_gated_mix__sliding_local_dilated__ssm_conv_s4__prompt_kernel(
    A_x: jax.Array,
    A_wqkv: jax.Array,
    A_wo: jax.Array,
    B_u: jax.Array,
    B_A_re: jax.Array,
    B_A_im: jax.Array,
    B_B_re: jax.Array,
    B_B_im: jax.Array,
    B_C_re: jax.Array,
    B_C_im: jax.Array,
    B_log_dt: jax.Array,
    B_Dskip: jax.Array,
    gate_w: jax.Array,
):
    del B_u
    assert A_x.shape == (1, S, D) and B_A_re.shape == (D, NS) and B_A_re.dtype == BF16
    hbm = pl.BlockSpec(memory_space=pl.ANY)
    vmem = pl.BlockSpec(memory_space=pltpu.VMEM)
    out = pl.pallas_call(
        _kernel,
        out_shape=jax.ShapeDtypeStruct((S, D), BF16),
        in_specs=[hbm] * 10 + [vmem] * 6 + [pl.BlockSpec(memory_space=pltpu.SMEM)],
        out_specs=hbm,
        scratch_shapes=[
            pltpu.VMEM((NT, S, 128), BF16),
            pltpu.VMEM((NT, S // 2, 128), jnp.int32),
            pltpu.VMEM((NT, 128, 3 * D), BF16),
            pltpu.VMEM((NT, D, 128), BF16),
            pltpu.VMEM(_KMATS.shape, jnp.int32),
            pltpu.VMEM((NT, 6, NS, 128), BF16),
            pltpu.VMEM((NT, 3 * D // 2, 128), jnp.int32),
            pltpu.VMEM((NT, D // 2, 128), jnp.int32),
            pltpu.VMEM((4, D, 128), F32),
            pltpu.VMEM((NT, 8, 128), F32),
            pltpu.VMEM((4, NS, 128), F32),
            pltpu.VMEM((2, 8, 128, 128), F32),
            pltpu.VMEM((2, 4, 16 * _NQ, 128), F32),
            pltpu.VMEM((3, 512, 128), F32),
            pltpu.VMEM((len(_BASE), 64, 128), jnp.int32),
            pltpu.VMEM((2 * NT + 1, NB, 2 * T, 128), F32),
            pltpu.VMEM((NB, NT, T, 128), jnp.int32),
            pltpu.VMEM((NT, M2, 128), F32),
            pltpu.VMEM((NT, S + PAD, 128), F32),
            pltpu.VMEM((NT, S + PAD, 128), F32),
            pltpu.VMEM((WIN, S, 128), F32),
            pltpu.VMEM((WIN, M3, 128), F32),
            pltpu.VMEM((2, NT, M3 // 2, 128), jnp.int32),
            pltpu.VMEM((NT, M3 // 2, 128), jnp.int32),
            pltpu.VMEM((2, M3, 128), F32),
            pltpu.VMEM((NT, M3, 128), F32),
            pltpu.VMEM((NT, M3, 128), F32),
            pltpu.VMEM((NT, S, 128), BF16),
            pltpu.SemaphoreType.DMA((NT,)),
            pltpu.SemaphoreType.DMA((NT,)),
            pltpu.SemaphoreType.DMA((NT,)),
            pltpu.SemaphoreType.DMA((1,)),
            pltpu.SemaphoreType.DMA((NT, 6)),
            pltpu.SemaphoreType.DMA((S // M3, NT)),
        ],
        compiler_params=pltpu.CompilerParams(vmem_limit_bytes=100 * 1024 * 1024),
    )(
        A_x.reshape(S, D), A_wqkv, A_wo, _KMATS,
        B_A_re.T, B_A_im.T, B_B_re.T, B_B_im.T, B_C_re.T, B_C_im.T,
        B_log_dt, B_Dskip, gate_w, _FWD, _INV, np.zeros((8, 128), np.int32), np.zeros((4,), np.int32),
    )
    return out.reshape(1, S, D)
```

```python
import itertools

import ml_dtypes
import numpy as np

import jax
import jax.numpy as jnp
import jax.experimental.pallas as pl
import jax.experimental.pallas.tpu as pltpu

F32 = jnp.float32
BF16 = jnp.bfloat16

S = 2048
D = 640
NS = 192
H = 32
DH = D // H
WIN, DIL = 8, 2
T = 128
NB = S // T
NT = D // 128
PAD = 16
M2 = 256
RELEASE = 11
LEAD = 0
HEAD = 6
TAIL = 3
LAG_D = 6
LAG_T = 4
LAG_V = 4
LAG_U = 4
LAG_S = 8
EARLY = 20
M3 = 256

_BASE = (0, 4, 256, 512, 1024, 2048)
_OFF = ((0, 1, 2, 3), (0, 1, 2, 3), (0, 2, 4, 6), (0, 4, 256, 260), (0, 256, 512, 768), (0, 0, 0, 0))


def _dft_constants():
    k = np.concatenate([np.arange(0, T, 2), np.arange(1, T, 2)])
    theta = 2.0 * np.pi * (k + 0.5) / (2 * T)
    ang = theta[:, None] * np.arange(T)[None, :]
    fwd = np.concatenate([np.cos(ang), -np.sin(ang)], axis=0)
    inv = np.stack([np.cos(ang).reshape(T // 8, 8, T), -np.sin(ang).reshape(T // 8, 8, T)], axis=1)
    inv = inv.reshape(2 * T, T).T / T
    slot = {}
    for t in range(len(_BASE)):
        for lane in range(128):
            i, a, p = lane // 8, (lane % 8) // 2, lane % 2
            slot.setdefault(_BASE[t] + _OFF[t][a] + 8 * (2 * i + p), (t, lane))
    lag = np.arange(S).astype(np.float32).astype(ml_dtypes.bfloat16).astype(np.float64).astype(np.int64)
    mats, passes = [], []
    for m in range(NB):
        per_tile = {}
        for n in range(T):
            t, lane = slot[int(lag[m * T + n])]
            per_tile.setdefault(t, np.zeros((2 * T, 128)))[:, lane] += fwd[:, n]
        passes.append(tuple((t, len(mats) + j) for j, t in enumerate(sorted(per_tile))))
        mats.extend(per_tile[t] for t in sorted(per_tile))

    def to_bf16(a):
        bits = np.asarray(a, np.float32).astype(ml_dtypes.bfloat16).view(np.uint16).astype(np.uint32)
        return (bits[..., 0::2, :] | (bits[..., 1::2, :] << 16)).view(np.int32)

    inv = inv.reshape(T, 2, T).transpose(1, 0, 2)
    return to_bf16(fwd), to_bf16(inv), to_bf16(np.stack(mats)), tuple(passes)


_FWD, _INV, _KMATS, _KPASSES = _dft_constants()

_Q_W, _Q_G, _Q_V, _Q_REC, _NQ = 0, 6, 9, 11, 12

_NT_DIMS = (((1,), (1,)), ((), ()))


def _csq(z):
    x, y, p, q = z
    return ((x - y) * (x + y), (x + x) * y, (p - q) * (p + q), (p + p) * q)


def _cmul(a, b):
    ax, ay, ap, aq = a
    bx, by, bp, bq = b
    return (ax * bx - ay * by, ax * by + ay * bx, ap * bp - aq * bq, ap * bq + aq * bp)


def _words(v):
    return pltpu.bitcast(v, jnp.int32)


def _halves(v):
    return pltpu.bitcast(v, BF16)


def _take(gen, n):
    out = []
    for _ in range(n):
        out += next(gen, [])
    return out


def _kernel(x_hbm, wqkv_hbm, wo_hbm, kmat_hbm, are_hbm, aim_hbm, bre_hbm, bim_hbm, cre_hbm, cim_hbm,
            ldt_ref, dskip_ref, gw_ref, fwd_ref, inv_ref, zero_ref, origin_ref,
            out_hbm,
            xs, xw, wraw, woraw, kmat, par, wt, wop, tmp, dts, disc, zw, tab, rs, kt, spec, zs, qs, ks, vs, ps, os_, oc, gs, att, ys, outs,
            x_sem, w_sem, wo_sem, km_sem, par_sem, out_sem):
    def lanes(c):
        return pl.ds(c * 128, 128) if isinstance(c, int) else pl.ds(pl.multiple_of(c * 128, 128), 128)

    def par_copies(c):
        return [pltpu.make_async_copy(src.at[:, lanes(c)], par.at[c, i], par_sem.at[c, i])
                for i, src in enumerate((are_hbm, aim_hbm, bre_hbm, bim_hbm, cre_hbm, cim_hbm))]

    def tile_copies(c):
        return [pltpu.make_async_copy(x_hbm.at[:, lanes(c)], xs.at[c], x_sem.at[c]),
                pltpu.make_async_copy(wqkv_hbm.at[lanes(c), :], wraw.at[c], w_sem.at[c]),
                pltpu.make_async_copy(wo_hbm.at[:, lanes(c)], woraw.at[c], wo_sem.at[c])]

    km_copy = pltpu.make_async_copy(kmat_hbm, kmat, km_sem.at[0])

    lane = jax.lax.broadcasted_iota(jnp.int32, (8, 128), 1)
    row = jax.lax.broadcasted_iota(jnp.int32, (8, 128), 0)
    low = lane < 64
    never = zero_ref[...] != 0

    def behind(val, earlier):
        return val if earlier is None else jnp.where(never, earlier, val)

    def paced(panels, rows, values):
        groups = rows // 16
        regs = [[panel(g) for panel in panels] for g in range(groups)]
        order = [(g, c) for g in range(groups) for c in range(len(panels))]
        for n, val in enumerate(values):
            g, c = order[n * len(order) // len(values)]
            regs[g][c] = jnp.where(never, _words(val), regs[g][c])
        return _halves(jnp.concatenate([jnp.concatenate(r, axis=1) for r in regs], axis=0))

    dt_row = jnp.exp(ldt_ref[...].astype(F32).reshape(1, D)).astype(BF16).astype(F32)
    for c in range(NT):
        dts[c] = jnp.broadcast_to(dt_row[:, c * 128:(c + 1) * 128], (8, 128))

    def discretize(c, past):
        dt = dts[c][0:1, :]
        for r in range(NS // 32):
            raw = [par[c, i, 32 * r:32 * r + 32, :].astype(F32) for i in range(6)]
            for n in range(4):
                a_re, a_im, b_re, b_im, c_re, c_im = (v[8 * n:8 * n + 8] for v in raw)
                mag, ang = jnp.exp(dt * a_re), behind(dt * a_im, past[-LAG_D])
                db_re, db_im = dt * b_re, dt * b_im
                vals = (mag * jnp.cos(ang), mag * jnp.sin(ang),
                        c_re * db_re - c_im * db_im, c_re * db_im + c_im * db_re)
                for i, val in enumerate(vals):
                    disc[i, 32 * r + 8 * n:32 * r + 8 * n + 8, :] = val
                yield list(vals[:2])
        for i in range(2):
            zw[c % 2, 4 * i + 0] = disc[2 * i, 0:128, :].T
            zw[c % 2, 4 * i + 1] = disc[2 * i + 1, 0:128, :].T
            yield []
            re, im = disc[2 * i, 128:NS, :], disc[2 * i + 1, 128:NS, :]
            zw[c % 2, 4 * i + 2] = jnp.concatenate([re, re], axis=0).T
            zw[c % 2, 4 * i + 3] = jnp.concatenate([-im, im], axis=0).T
            yield []

    def put(tile, slot, even, odd):
        for comp in range(len(even)):
            tab[tile % 2, comp, pl.ds(16 * slot, 8, stride=2), :] = even[comp]
            tab[tile % 2, comp, pl.ds(16 * slot + 1, 8, stride=2), :] = odd[comp]

    def get(group, slot, comps):
        tile, half = divmod(group, 2)
        return tuple(tab[tile % 2, comp, pl.ds(16 * slot + 8 * half, 8), :] for comp in range(comps))

    def running(z, conj=False):
        x, y, p, q = z
        if conj:
            return (x, -y, jnp.where(low, p, -q))
        return (x, y, jnp.where(low, p, q), jnp.where(low, -q, p))

    def tables(c, tile, earlier):
        rows = slice(8 * tile, 8 * tile + 8)
        one = (jnp.ones((8, 128), F32), jnp.zeros((8, 128), F32)) * 2
        z1 = tuple(behind(zw[c % 2, i, rows, :], earlier if i % 2 == 0 else None) for i in range(4))
        w = tuple(zw[c % 2, 4 + i, rows, :] for i in range(4))
        z2 = _csq(z1)
        put(tile, _Q_G, z2, z2)
        z4 = _csq(z2)
        w4 = _cmul(w, z4)
        put(tile, _Q_W, running(w), running(w4))
        put(tile, _Q_W + 3, running(_cmul(w, z1)), running(_cmul(w4, z1)))
        z8 = _csq(z4)
        put(tile, _Q_V, running(one, True), running(z8, True))
        z16 = _csq(z8)
        z24 = _cmul(z16, z8)
        put(tile, _Q_V + 1, running(z16, True), running(z24, True))
        x, y, p, q = z16
        rec = (x + x, x * x + y * y, p + p, p * p + q * q)
        put(tile, _Q_REC, rec, rec)
        z256 = _csq(_csq(_csq(_csq(z16))))
        put(tile, _Q_G + 1, z4, z256)
        yield [z24[0], z24[2], z256[0], z256[2]]
        z512 = _csq(z256)
        put(tile, _Q_G + 2, z512, one)
        w256, w512 = _cmul(w, z256), _cmul(w, z512)
        put(tile, _Q_W + 1, running(w256), running(w512))
        w258, w516 = _cmul(w256, z2), _cmul(w512, z4)
        put(tile, _Q_W + 4, running(w258), running(w516))
        z1024 = _csq(z512)
        w1024 = _cmul(w, z1024)
        w1280, w2048 = _cmul(w1024, z256), _cmul(w1024, z1024)
        put(tile, _Q_W + 2, running(w1024), running(w2048))
        put(tile, _Q_W + 5, running(w1280), running(w2048))
        yield [w258[0], w516[2], w1280[0], w2048[2]]

    def operand(panels):
        return jnp.concatenate([jnp.concatenate(parts, axis=0) for parts in panels], axis=1).astype(BF16)

    chan = row // 2
    slot_of_lane = ((lane // 2) - chan) % 4

    def generate(c, riders, upcoming, chores):
        base = c % 2 * 256 if isinstance(c, int) else pl.multiple_of(c % 2 * 256, 256)
        slots = 32 + HEAD + TAIL
        for rider in riders[:HEAD * len(riders) // slots]:
            rider([])
        _take(tables(c, 0, None), 2)
        res, stage2, stage3, past = None, [], [], [None] * 8
        extra = discretize(c + 1, past) if upcoming else iter(())
        for group in range(32 + 3):
            for i, r in enumerate(stage3):
                rs[i, pl.ds(base + 8 * (group - 3), 8), :] = jnp.where(
                    (chan & 2) == 2, pltpu.roll(r, 128 - 4, 1), r)
            stage3 = [jnp.where((chan & 1) == 1, pltpu.roll(r, 128 - 2, 1), r) for r in stage2]
            stage2 = []
            for i in range(3 if res is not None else 0):
                r = res[8 * i:8 * i + 8]
                for a in range(1, 4):
                    blk = res[24 * a + 8 * i:24 * a + 8 * i + 8]
                    r = jnp.where(slot_of_lane == a, pltpu.roll(blk, 2 * a, 1), r)
                stage2.append(r)
            res = None
            ride = riders[(group + HEAD) * len(riders) // slots:(group + HEAD + 1) * len(riders) // slots]
            if group >= 32:
                for rider in ride:
                    rider([])
            else:
                if group % 2 == 0:
                    ahead = tables(c, group // 2 + 1, past[-LAG_T]) if group + 2 < 32 else iter(())
                _take(chores, 1)
                pace = _take(extra, 1) + _take(ahead, 1)
                for n, rider in enumerate(ride):
                    rider(pace[n * len(pace) // len(ride):(n + 1) * len(pace) // len(ride)])
                a_lo, b_lo, a_hi, b_hi = get(group, _Q_REC, 4)
                rhs = []
                for al, be, v in zip((a_lo, a_lo, a_hi), (b_lo, b_lo, b_hi),
                                     zip(get(group, _Q_V, 3), get(group, _Q_V + 1, 3))):
                    v = [v[0], behind(v[1], past[-LAG_V])]
                    for i in range(2, 16):
                        v.append(al * v[i - 1] - be * v[i - 2])
                    rhs.append(v)
                u = [get(group, _Q_W + n, 4) for n in range(6)]
                m = [tuple(behind(g, past[-LAG_U]) for g in get(group, _Q_G + i, 4)) for i in range(3)] * 2
                lhs = [[v[0] for v in u] + [v[0] * g[0] - v[1] * g[1] for v, g in zip(u, m)],
                       [v[1] for v in u] + [v[1] * g[0] + v[0] * g[1] for v, g in zip(u, m)],
                       [v[2] for v in u] + [v[2] * g[2] + v[3] * g[3] for v, g in zip(u, m)]]
                res = jax.lax.dot_general(operand(lhs), operand(rhs), _NT_DIMS, preferred_element_type=F32)
                past.append(res[0:8] if riders else None)
        _take(extra, NS)
        _take(chores, NS)

    def dft_passes(c):
        base = c % 2 * 256 if isinstance(c, int) else pl.multiple_of(c % 2 * 256, 256)
        for t in range(len(_BASE)):
            kt[t] = _words(rs[t // 2, pl.ds(base + t % 2, 128, stride=2), :].astype(BF16))

        def kernel_pass(m):
            def run(values):
                lhs = paced([lambda g, idx=idx: kmat[idx, 8 * g:8 * g + 8, :] for _, idx in _KPASSES[m]],
                            2 * T, values)
                rhs = _halves(jnp.concatenate([kt[t] for t, _ in _KPASSES[m]], axis=1))
                spec[NT + c, m] = jax.lax.dot_general(lhs, rhs, _NT_DIMS, preferred_element_type=F32)
            return run

        def signal_pass(m):
            def run(values):
                lhs = paced([lambda g: fwd_ref[8 * g:8 * g + 8, :]], 2 * T, values)
                block = xs[c, m * T:(m + 1) * T, :]
                xw[c, m * T // 2:(m + 1) * T // 2, :] = _words(block)
                spec[c, m] = jnp.dot(lhs, block, preferred_element_type=F32)
            return run

        return [make(m) for m in range(NB) for make in (signal_pass, kernel_pass)]

    def permute_weights(c):
        for part in range(3):
            for n in range(NT):
                col = part * D + n * 128
                tmp[part, n * 128:(n + 1) * 128, :] = wraw[c, :, col:col + 128].astype(F32).T
                yield []
            for j in range(DH):
                wt[c, pl.ds((part * D + j * H) // 2, H // 2), :] = _words(
                    tmp[part, pl.ds(j, H, stride=DH), :].astype(BF16))
                if j % 7 == 6:
                    yield []
        tmp[3] = woraw[c].astype(F32)
        yield []
        for j in range(DH):
            wop[c, pl.ds(j * H // 2, H // 2), :] = _words(tmp[3, pl.ds(j, H, stride=DH), :].astype(BF16))
            if j % 7 == 6:
                yield []

    with jax.named_scope("P0"):
        for cp in par_copies(0) + par_copies(1):
            cp.start()
        for cp in par_copies(0):
            cp.wait()
        km_copy.start()
        for cp in tile_copies(0):
            cp.start()
        for c in range(2, NT):
            for cp in par_copies(c):
                cp.start()
        _take(discretize(0, [None] * 8), NS)
        for cp in par_copies(1):
            cp.wait()
        generate(0, [], True, iter(()))
        for c in range(1, NT):
            for cp in tile_copies(c):
                cp.start()
        km_copy.wait()
        for c in range(2, NT):
            for cp in par_copies(c):
                cp.wait()

    def ssm_step(c, carry):
        for cp in tile_copies(c - 1):
            cp.wait()
        generate(c, dft_passes(c - 1), True, permute_weights(c - 1))
        return carry

    with jax.named_scope("P1"):
        jax.lax.fori_loop(1, NT - 1, ssm_step, 0)
    with jax.named_scope("P1b"):
        for cp in tile_copies(NT - 2) + tile_copies(NT - 1):
            cp.wait()
        generate(NT - 1, dft_passes(NT - 2), False, permute_weights(NT - 2))
        chores = permute_weights(NT - 1)
        for run in dft_passes(NT - 1):
            _take(chores, 1)
            run([])
        _take(chores, NS)

    for c in range(NT):
        ks[c, 0:PAD, :] = jnp.zeros((PAD, 128), F32)
        vs[c, 0:PAD, :] = jnp.zeros((PAD, 128), F32)
    q_scale = float(DH ** -0.5 * np.log2(np.e))
    n2 = S // M2
    ft_per_step = (T // 8) // n2

    def causal(a, b, j):
        acc = a[0] * b[j]
        for i in range(1, j + 1):
            acc = acc + a[i] * b[j - i]
        return acc

    even_order = [j for i in range(NB // 2) for j in (i, NB - 1 - i)]

    def convolve(it):
        def tile_of(f):
            return (it * ft_per_step + f) // 2 + f % 2 * (T // 16)

        def operands(f, c, phase):
            def load(slab, part):
                rows = pl.ds(pl.multiple_of(origin_ref[phase] + part * T + tile_of(f) * 8, 8), 8)
                return [spec[slab, m, rows, :] for m in range(NB)]

            plus, minus = (jnp.subtract, jnp.add) if f % 2 else (jnp.add, jnp.subtract)
            k_re, k_im = load(NT + c, 0), load(NT + c, 1)
            if phase == 0:
                return ([u + v for u, v in zip(load(c, 0), load(c, 1))],
                        [k_re[0]] + [minus(k_re[m], k_im[m - 1]) for m in range(1, NB)])
            if phase == 1:
                return load(c, 0), [k_im[0] - k_re[0]] + [
                    plus(k_im[m] - k_re[m], k_im[m - 1] + k_re[m - 1]) for m in range(1, NB)]
            return load(c, 1), [-k_im[0] - k_re[0]] + [
                (k_re[m - 1] - k_im[m - 1] if f % 2 else k_im[m - 1] - k_re[m - 1]) - (k_im[m] + k_re[m])
                for m in range(1, NB)]

        jobs = [(f, c, phase) for f in range(ft_per_step) for c in range(NT) for phase in range(3)]
        ahead, sums = operands(*jobs[0]), [{}, {}, {}]
        for n, (f, c, phase) in enumerate(jobs):
            a, b = ahead
            for i, j in enumerate(even_order):
                val = sums[phase][j] = causal(a, b, j)
                if i == RELEASE and n + 1 < len(jobs):
                    spec[2 * NT, 0, pl.ds(pl.multiple_of(origin_ref[3], 8), 8), :] = val
                    ahead = operands(*jobs[n + 1])
                if phase == 2:
                    z = jnp.concatenate([sums[0][j]] * 2, axis=0) + jnp.concatenate([val, sums[1][j]], axis=0)
                    val = _words(z.astype(BF16))
                    zs[j, c, pl.ds(pl.multiple_of(tile_of(f) * 8, 8), 8), :] = val
                yield val

    def logits(r0):
        past = [None] * LAG_S
        for t0 in range(0, M2, 8):
            q = [qs[c, t0:t0 + 8, :] for c in range(NT)]
            q[0] = behind(q[0], past[-LAG_S])
            for w in range(WIN):
                src = pl.ds(r0 + (t0 + PAD - DIL * w), 8)
                acc = q[0] * ks[0, src, :]
                for c in range(1, NT):
                    acc = acc + q[c] * ks[c, src, :]
                acc = acc + pltpu.roll(acc, 64, 1)
                acc = acc + pltpu.roll(acc, 32, 1)
                ps[w, pl.ds(r0 + t0, 8), :] = acc
            past.append(acc)
            yield

    def proj_step(it, carry):
        r0 = pl.multiple_of(it * M2, M2)
        conv, dots = convolve(it), logits(r0)
        x_panel = lambda c: lambda g: xw[c, pl.ds(pl.multiple_of(it * (M2 // 2), 8) + 8 * g, 8), :]
        place = lambda n, base: ((qs, ks, vs)[n // NT], (n % NT, pl.ds(base + (r0 + PAD if n >= NT else 0), M2)))
        todo, slots = 3 * NB * NT * ft_per_step, 0
        for n in range(3 * NT):
            if n % 4 == 0:
                hi = min(n + 4, 3 * NT)
                count = EARLY * todo * (slots + 1) // 260 - EARLY * todo * slots // 260 if slots < 13 else 0
                slots += 1
                xb = paced([x_panel(NT - 1)], M2, list(itertools.islice(conv, count)))
                tail = jax.lax.dot_general(xb, _halves(wt[NT - 1, n * 64:hi * 64, :]), _NT_DIMS,
                                           preferred_element_type=F32)
                for i in range(n, hi):
                    ref, idx = place(i, 0)
                    ref[idx] = tail[:, (i - n) * 128:(i - n + 1) * 128]
            if n < 2 * NT:
                count = EARLY * todo * (slots + 1) // 260 - EARLY * todo * slots // 260
                values = list(itertools.islice(conv, count))
            else:
                values = list(itertools.islice(conv, -(-(todo - EARLY * todo // 20) // NT)))
                for _ in itertools.islice(dots, -(-(M2 // 8) // NT)):
                    pass
            slots += 1
            xb = paced([x_panel(c) for c in range(NT - 1)], M2, values)
            w = _halves(jnp.concatenate([wt[c, n * 64:(n + 1) * 64, :] for c in range(NT - 1)], axis=1))
            ref, idx = place(n, pl.multiple_of(origin_ref[0], 8))
            res = jax.lax.dot_general(xb, w, _NT_DIMS, preferred_element_type=F32) + ref[idx]
            ref, idx = place(n, 0)
            ref[idx] = res if n >= NT else res * q_scale
        assert next(conv, None) is None and next(dots, 0) == 0
        return carry

    with jax.named_scope("P2"):
        jax.lax.fori_loop(0, n2, proj_step, 0)

    def attend(blk):
        r0 = 0 if isinstance(blk, int) else pl.multiple_of(blk * M3, M3)
        for t0 in range(0, M3, 16):
            logit = [ps[w, pl.ds(r0 + t0, 16), :] for w in range(WIN)]
            if isinstance(blk, int) and t0 == 0:
                pos = jax.lax.broadcasted_iota(jnp.int32, (16, 128), 0)
                logit = [jnp.where(pos >= DIL * w, l, -1e9) if w else l for w, l in enumerate(logit)]
            top = logit[0]
            for w in range(1, WIN):
                top = jnp.maximum(top, logit[w])
            e = [jnp.exp2(l - top) for l in logit]
            den = e[0]
            for w in range(1, WIN):
                den = den + e[w]
            inv = pl.reciprocal(den, approx=True)
            inv = inv * (2.0 - den * inv)
            for c in range(NT):
                acc = e[0] * vs[c, pl.ds(r0 + (t0 + PAD), 16), :]
                for w in range(1, WIN):
                    acc = acc + e[w] * vs[c, pl.ds(r0 + (t0 + PAD - DIL * w), 16), :]
                o = _words((acc * inv).astype(BF16))
                os_[blk % 2, c, t0 // 2:t0 // 2 + 8, :] = o
                yield o

    def out_copy(blk, c):
        rows = pl.ds(pl.multiple_of(blk * M3, M3), M3)
        return pltpu.make_async_copy(outs.at[c, rows], out_hbm.at[rows, lanes(c)], out_sem.at[blk, c])

    def gates(blk):
        r0 = 0 if isinstance(blk, int) else pl.multiple_of(blk * (M3 // 2), 8)
        gw_row = gw_ref[...].astype(F32).reshape(1, D)
        for g in range(M3 // 16):
            rows = pl.ds(r0 + 8 * g, 8)
            score = _halves(xw[0, rows, :]).astype(F32) * gw_row[:, 0:128]
            for c in range(1, NT):
                score = score + _halves(xw[c, rows, :]).astype(F32) * gw_row[:, c * 128:(c + 1) * 128]
            gate = jnp.broadcast_to(jax.nn.sigmoid(jnp.sum(score, axis=1, keepdims=True)), (16, 128))
            gs[blk % 2, 16 * g:16 * g + 16, :] = gate
            yield

    def finish(blk, work, total):
        rows = pl.ds(pl.multiple_of(blk * M3, M3), M3)
        word_rows = pl.ds(pl.multiple_of(blk * (M3 // 2), 8), M3 // 2)
        dskip_row = dskip_ref[...].astype(F32).reshape(1, D)
        spent = [0]

        def pull(cost):
            lo, spent[0] = spent[0], spent[0] + cost
            share = lambda t: total * max(t - LEAD, 0) // (35 - LEAD)
            return list(itertools.islice(work, share(spent[0]) - share(lo)))

        o_panel = lambda c: lambda g: oc[c, 8 * g:8 * g + 8, :]
        inv_panels = [lambda g, k=k: inv_ref[k, 8 * g:8 * g + 8, :] for k in range(2)]
        oc[...] = os_[blk % 2]
        for lo, hi in ((0, 4), (4, 5)):
            w = _halves(jnp.concatenate([wop[c, 256:320, :] for c in range(lo, hi)], axis=1))
            tail = jnp.dot(paced([o_panel(NT - 1)], M3, pull(hi - lo)), w, preferred_element_type=F32)
            for c in range(lo, hi):
                att[c] = tail[:, (c - lo) * 128:(c - lo + 1) * 128]
        for lo, hi in ((0, 2), (2, 4), (4, 5)):
            for i in range(M3 // T):
                z = _halves(jnp.concatenate([zs[blk * (M3 // T) + i, c] for c in range(lo, hi)], axis=1))
                y = jnp.dot(paced(inv_panels, T, pull(hi - lo)), z, preferred_element_type=F32)
                for c in range(lo, hi):
                    ys[c, i * T:(i + 1) * T, :] = y[:, (c - lo) * 128:(c - lo + 1) * 128]
        back = pl.ds(pl.multiple_of(origin_ref[0], 8), M3)
        for c in range(NT):
            mixed = jnp.dot(paced([o_panel(k) for k in range(NT - 1)], M3, pull(4)), _halves(wop[c, 0:256, :]),
                            preferred_element_type=F32) + att[c, back, :]
            ssm = ys[c, back, :] + _halves(xw[c, word_rows, :]).astype(F32) * dskip_row[:, c * 128:(c + 1) * 128]
            outs[c, rows, :] = (ssm + gs[blk % 2] * (mixed - ssm)).astype(BF16)
        assert next(work, None) is None

    def prepare(blk):
        now, mix = attend(blk), gates(blk)
        for _ in range(M3 // 16):
            next(mix)
            yield from itertools.islice(now, NT)

    for _ in prepare(0):
        pass
    n3 = S // M3

    def out_step(it, carry):
        finish(it, prepare(it + 1), M3 // 16 * NT)
        for c in range(NT):
            out_copy(it, c).start()
        return carry

    with jax.named_scope("P3"):
        jax.lax.fori_loop(0, n3 - 1, out_step, 0)
    with jax.named_scope("P4"):
        finish(n3 - 1, iter(()), 0)
        for c in range(NT):
            out_copy(n3 - 1, c).start()
        for blk in range(n3):
            for c in range(NT):
                out_copy(blk, c).wait()


@jax.jit
def pallas_gated_mix__sliding_local_dilated__ssm_conv_s4__prompt_kernel(
    A_x: jax.Array,
    A_wqkv: jax.Array,
    A_wo: jax.Array,
    B_u: jax.Array,
    B_A_re: jax.Array,
    B_A_im: jax.Array,
    B_B_re: jax.Array,
    B_B_im: jax.Array,
    B_C_re: jax.Array,
    B_C_im: jax.Array,
    B_log_dt: jax.Array,
    B_Dskip: jax.Array,
    gate_w: jax.Array,
):
    del B_u
    assert A_x.shape == (1, S, D) and B_A_re.shape == (D, NS) and B_A_re.dtype == BF16
    hbm = pl.BlockSpec(memory_space=pl.ANY)
    vmem = pl.BlockSpec(memory_space=pltpu.VMEM)
    out = pl.pallas_call(
        _kernel,
        out_shape=jax.ShapeDtypeStruct((S, D), BF16),
        in_specs=[hbm] * 10 + [vmem] * 6 + [pl.BlockSpec(memory_space=pltpu.SMEM)],
        out_specs=hbm,
        scratch_shapes=[
            pltpu.VMEM((NT, S, 128), BF16),
            pltpu.VMEM((NT, S // 2, 128), jnp.int32),
            pltpu.VMEM((NT, 128, 3 * D), BF16),
            pltpu.VMEM((NT, D, 128), BF16),
            pltpu.VMEM(_KMATS.shape, jnp.int32),
            pltpu.VMEM((NT, 6, NS, 128), BF16),
            pltpu.VMEM((NT, 3 * D // 2, 128), jnp.int32),
            pltpu.VMEM((NT, D // 2, 128), jnp.int32),
            pltpu.VMEM((4, D, 128), F32),
            pltpu.VMEM((NT, 8, 128), F32),
            pltpu.VMEM((4, NS, 128), F32),
            pltpu.VMEM((2, 8, 128, 128), F32),
            pltpu.VMEM((2, 4, 16 * _NQ, 128), F32),
            pltpu.VMEM((3, 512, 128), F32),
            pltpu.VMEM((len(_BASE), 64, 128), jnp.int32),
            pltpu.VMEM((2 * NT + 1, NB, 2 * T, 128), F32),
            pltpu.VMEM((NB, NT, T, 128), jnp.int32),
            pltpu.VMEM((NT, M2, 128), F32),
            pltpu.VMEM((NT, S + PAD, 128), F32),
            pltpu.VMEM((NT, S + PAD, 128), F32),
            pltpu.VMEM((WIN, S, 128), F32),
            pltpu.VMEM((2, NT, M3 // 2, 128), jnp.int32),
            pltpu.VMEM((NT, M3 // 2, 128), jnp.int32),
            pltpu.VMEM((2, M3, 128), F32),
            pltpu.VMEM((NT, M3, 128), F32),
            pltpu.VMEM((NT, M3, 128), F32),
            pltpu.VMEM((NT, S, 128), BF16),
            pltpu.SemaphoreType.DMA((NT,)),
            pltpu.SemaphoreType.DMA((NT,)),
            pltpu.SemaphoreType.DMA((NT,)),
            pltpu.SemaphoreType.DMA((1,)),
            pltpu.SemaphoreType.DMA((NT, 6)),
            pltpu.SemaphoreType.DMA((S // M3, NT)),
        ],
        compiler_params=pltpu.CompilerParams(vmem_limit_bytes=100 * 1024 * 1024),
    )(
        A_x.reshape(S, D), A_wqkv, A_wo, _KMATS,
        B_A_re.T, B_A_im.T, B_B_re.T, B_B_im.T, B_C_re.T, B_C_im.T,
        B_log_dt, B_Dskip, gate_w, _FWD, _INV, np.zeros((8, 128), np.int32), np.zeros((4,), np.int32),
    )
    return out.reshape(1, S, D)
```

```python
import itertools

import ml_dtypes
import numpy as np

import jax
import jax.numpy as jnp
import jax.experimental.pallas as pl
import jax.experimental.pallas.tpu as pltpu

F32 = jnp.float32
BF16 = jnp.bfloat16

S = 2048
D = 640
NS = 192
H = 32
DH = D // H
WIN, DIL = 8, 2
T = 128
NB = S // T
NT = D // 128
PAD = 16
M2 = 256
RELEASE = 11
LEAD = 0
HEAD = 6
TAIL = 3
LAG_D = 6
LAG_T = 4
LAG_V = 4
LAG_U = 4
SKEW = 8
LAG_S = 8
EARLY = 20
M3 = 256

_BASE = (0, 4, 256, 512, 1024, 2048)
_OFF = ((0, 1, 2, 3), (0, 1, 2, 3), (0, 2, 4, 6), (0, 4, 256, 260), (0, 256, 512, 768), (0, 0, 0, 0))


def _dft_constants():
    k = np.concatenate([np.arange(0, T, 2), np.arange(1, T, 2)])
    theta = 2.0 * np.pi * (k + 0.5) / (2 * T)
    ang = theta[:, None] * np.arange(T)[None, :]
    fwd = np.concatenate([np.cos(ang), -np.sin(ang)], axis=0)
    inv = np.stack([np.cos(ang).reshape(T // 8, 8, T), -np.sin(ang).reshape(T // 8, 8, T)], axis=1)
    inv = inv.reshape(2 * T, T).T / T
    slot = {}
    for t in range(len(_BASE)):
        for lane in range(128):
            i, a, p = lane // 8, (lane % 8) // 2, lane % 2
            slot.setdefault(_BASE[t] + _OFF[t][a] + 8 * (2 * i + p), (t, lane))
    lag = np.arange(S).astype(np.float32).astype(ml_dtypes.bfloat16).astype(np.float64).astype(np.int64)
    mats, passes = [], []
    for m in range(NB):
        per_tile = {}
        for n in range(T):
            t, lane = slot[int(lag[m * T + n])]
            per_tile.setdefault(t, np.zeros((2 * T, 128)))[:, lane] += fwd[:, n]
        passes.append(tuple((t, len(mats) + j) for j, t in enumerate(sorted(per_tile))))
        mats.extend(per_tile[t] for t in sorted(per_tile))

    def to_bf16(a):
        bits = np.asarray(a, np.float32).astype(ml_dtypes.bfloat16).view(np.uint16).astype(np.uint32)
        return (bits[..., 0::2, :] | (bits[..., 1::2, :] << 16)).view(np.int32)

    inv = inv.reshape(T, 2, T).transpose(1, 0, 2)
    skew = lambda a: np.pad(a, ((0, 0), (0, SKEW), (0, 0)))
    return to_bf16(fwd), skew(to_bf16(inv)), skew(to_bf16(np.stack(mats))), tuple(passes)


_FWD, _INV, _KMATS, _KPASSES = _dft_constants()

_Q_W, _Q_G, _Q_V, _Q_REC, _NQ = 0, 6, 9, 11, 12

_NT_DIMS = (((1,), (1,)), ((), ()))


def _csq(z):
    x, y, p, q = z
    return ((x - y) * (x + y), (x + x) * y, (p - q) * (p + q), (p + p) * q)


def _cmul(a, b):
    ax, ay, ap, aq = a
    bx, by, bp, bq = b
    return (ax * bx - ay * by, ax * by + ay * bx, ap * bp - aq * bq, ap * bq + aq * bp)


def _words(v):
    return pltpu.bitcast(v, jnp.int32)


def _halves(v):
    return pltpu.bitcast(v, BF16)


def _take(gen, n):
    out = []
    for _ in range(n):
        out += next(gen, [])
    return out


def _kernel(x_hbm, wqkv_hbm, wo_hbm, kmat_hbm, are_hbm, aim_hbm, bre_hbm, bim_hbm, cre_hbm, cim_hbm,
            ldt_ref, dskip_ref, gw_ref, fwd_ref, inv_ref, zero_ref, origin_ref,
            out_hbm,
            xs, xw, wraw, woraw, kmat, par, wt, wop, tmp, dts, disc, zw, tab, rs, kt, spec, zs, qs, ks, vs, ps, os_, oc, gs, att, ys, outs,
            x_sem, w_sem, wo_sem, km_sem, par_sem, out_sem):
    def lanes(c):
        return pl.ds(c * 128, 128) if isinstance(c, int) else pl.ds(pl.multiple_of(c * 128, 128), 128)

    def par_copies(c):
        return [pltpu.make_async_copy(src.at[:, lanes(c)], par.at[c, i], par_sem.at[c, i])
                for i, src in enumerate((are_hbm, aim_hbm, bre_hbm, bim_hbm, cre_hbm, cim_hbm))]

    def tile_copies(c):
        return [pltpu.make_async_copy(x_hbm.at[:, lanes(c)], xs.at[c], x_sem.at[c]),
                pltpu.make_async_copy(wqkv_hbm.at[lanes(c), :], wraw.at[c], w_sem.at[c]),
                pltpu.make_async_copy(wo_hbm.at[:, lanes(c)], woraw.at[c], wo_sem.at[c])]

    km_copy = pltpu.make_async_copy(kmat_hbm, kmat, km_sem.at[0])

    lane = jax.lax.broadcasted_iota(jnp.int32, (8, 128), 1)
    row = jax.lax.broadcasted_iota(jnp.int32, (8, 128), 0)
    low = lane < 64
    never = zero_ref[...] != 0

    def behind(val, earlier):
        return val if earlier is None else jnp.where(never, earlier, val)

    def paced(panels, rows, values):
        groups = rows // 16
        regs = [[panel(g) for panel in panels] for g in range(groups)]
        order = [(g, c) for g in range(groups) for c in range(len(panels))]
        for n, val in enumerate(values):
            g, c = order[n * len(order) // len(values)]
            regs[g][c] = jnp.where(never, _words(val), regs[g][c])
        return _halves(jnp.concatenate([jnp.concatenate(r, axis=1) for r in regs], axis=0))

    dt_row = jnp.exp(ldt_ref[...].astype(F32).reshape(1, D)).astype(BF16).astype(F32)
    for c in range(NT):
        dts[c] = jnp.broadcast_to(dt_row[:, c * 128:(c + 1) * 128], (8, 128))

    def discretize(c, past):
        dt = dts[c][0:1, :]
        for r in range(NS // 32):
            raw = [par[c, i, 32 * r:32 * r + 32, :].astype(F32) for i in range(6)]
            for n in range(4):
                a_re, a_im, b_re, b_im, c_re, c_im = (v[8 * n:8 * n + 8] for v in raw)
                mag, ang = jnp.exp(dt * a_re), behind(dt * a_im, past[-LAG_D])
                db_re, db_im = dt * b_re, dt * b_im
                vals = (mag * jnp.cos(ang), mag * jnp.sin(ang),
                        c_re * db_re - c_im * db_im, c_re * db_im + c_im * db_re)
                for i, val in enumerate(vals):
                    disc[i, 32 * r + 8 * n:32 * r + 8 * n + 8, :] = val
                yield list(vals[:2])
        for i in range(2):
            zw[c % 2, 4 * i + 0, 0:128, :] = disc[2 * i, 0:128, :].T
            zw[c % 2, 4 * i + 1, 0:128, :] = disc[2 * i + 1, 0:128, :].T
            yield []
            re, im = disc[2 * i, 128:NS, :], disc[2 * i + 1, 128:NS, :]
            zw[c % 2, 4 * i + 2, 0:128, :] = jnp.concatenate([re, re], axis=0).T
            zw[c % 2, 4 * i + 3, 0:128, :] = jnp.concatenate([-im, im], axis=0).T
            yield []

    def put(tile, slot, even, odd):
        for comp in range(len(even)):
            tab[tile % 2, comp, pl.ds(16 * slot, 8, stride=2), :] = even[comp]
            tab[tile % 2, comp, pl.ds(16 * slot + 1, 8, stride=2), :] = odd[comp]

    def get(group, slot, comps):
        tile, half = divmod(group, 2)
        return tuple(tab[tile % 2, comp, pl.ds(16 * slot + 8 * half, 8), :] for comp in range(comps))

    def running(z, conj=False):
        x, y, p, q = z
        if conj:
            return (x, -y, jnp.where(low, p, -q))
        return (x, y, jnp.where(low, p, q), jnp.where(low, -q, p))

    def tables(c, tile, earlier):
        rows = slice(8 * tile, 8 * tile + 8)
        one = (jnp.ones((8, 128), F32), jnp.zeros((8, 128), F32)) * 2
        z1 = tuple(behind(zw[c % 2, i, rows, :], earlier if i % 2 == 0 else None) for i in range(4))
        w = tuple(zw[c % 2, 4 + i, rows, :] for i in range(4))
        z2 = _csq(z1)
        put(tile, _Q_G, z2, z2)
        z4 = _csq(z2)
        w4 = _cmul(w, z4)
        put(tile, _Q_W, running(w), running(w4))
        put(tile, _Q_W + 3, running(_cmul(w, z1)), running(_cmul(w4, z1)))
        z8 = _csq(z4)
        put(tile, _Q_V, running(one, True), running(z8, True))
        z16 = _csq(z8)
        z24 = _cmul(z16, z8)
        put(tile, _Q_V + 1, running(z16, True), running(z24, True))
        x, y, p, q = z16
        rec = (x + x, x * x + y * y, p + p, p * p + q * q)
        put(tile, _Q_REC, rec, rec)
        z256 = _csq(_csq(_csq(_csq(z16))))
        put(tile, _Q_G + 1, z4, z256)
        yield [z24[0], z24[2], z256[0], z256[2]]
        z512 = _csq(z256)
        put(tile, _Q_G + 2, z512, one)
        w256, w512 = _cmul(w, z256), _cmul(w, z512)
        put(tile, _Q_W + 1, running(w256), running(w512))
        w258, w516 = _cmul(w256, z2), _cmul(w512, z4)
        put(tile, _Q_W + 4, running(w258), running(w516))
        z1024 = _csq(z512)
        w1024 = _cmul(w, z1024)
        w1280, w2048 = _cmul(w1024, z256), _cmul(w1024, z1024)
        put(tile, _Q_W + 2, running(w1024), running(w2048))
        put(tile, _Q_W + 5, running(w1280), running(w2048))
        yield [w258[0], w516[2], w1280[0], w2048[2]]

    def operand(panels):
        return jnp.concatenate([jnp.concatenate(parts, axis=0) for parts in panels], axis=1).astype(BF16)

    chan = row // 2
    slot_of_lane = ((lane // 2) - chan) % 4

    def generate(c, riders, upcoming, chores):
        base = c % 2 * 256 if isinstance(c, int) else pl.multiple_of(c % 2 * 256, 256)
        slots = 32 + HEAD + TAIL
        for rider in riders[:HEAD * len(riders) // slots]:
            rider([])
        _take(tables(c, 0, None), 2)
        res, stage2, stage3, past = None, [], [], [None] * 8
        extra = discretize(c + 1, past) if upcoming else iter(())
        for group in range(32 + 3):
            for i, r in enumerate(stage3):
                rs[i, pl.ds(base + 8 * (group - 3), 8), :] = jnp.where(
                    (chan & 2) == 2, pltpu.roll(r, 128 - 4, 1), r)
            stage3 = [jnp.where((chan & 1) == 1, pltpu.roll(r, 128 - 2, 1), r) for r in stage2]
            stage2 = []
            for i in range(3 if res is not None else 0):
                r = res[8 * i:8 * i + 8]
                for a in range(1, 4):
                    blk = res[24 * a + 8 * i:24 * a + 8 * i + 8]
                    r = jnp.where(slot_of_lane == a, pltpu.roll(blk, 2 * a, 1), r)
                stage2.append(r)
            res = None
            ride = riders[(group + HEAD) * len(riders) // slots:(group + HEAD + 1) * len(riders) // slots]
            if group >= 32:
                for rider in ride:
                    rider([])
            else:
                if group % 2 == 0:
                    ahead = tables(c, group // 2 + 1, past[-LAG_T]) if group + 2 < 32 else iter(())
                _take(chores, 1)
                pace = _take(extra, 1) + _take(ahead, 1)
                for n, rider in enumerate(ride):
                    rider(pace[n * len(pace) // len(ride):(n + 1) * len(pace) // len(ride)])
                a_lo, b_lo, a_hi, b_hi = get(group, _Q_REC, 4)
                rhs = []
                for al, be, v in zip((a_lo, a_lo, a_hi), (b_lo, b_lo, b_hi),
                                     zip(get(group, _Q_V, 3), get(group, _Q_V + 1, 3))):
                    v = [v[0], behind(v[1], past[-LAG_V])]
                    for i in range(2, 16):
                        v.append(al * v[i - 1] - be * v[i - 2])
                    rhs.append(v)
                u = [get(group, _Q_W + n, 4) for n in range(6)]
                m = [tuple(behind(g, past[-LAG_U]) for g in get(group, _Q_G + i, 4)) for i in range(3)] * 2
                lhs = [[v[0] for v in u] + [v[0] * g[0] - v[1] * g[1] for v, g in zip(u, m)],
                       [v[1] for v in u] + [v[1] * g[0] + v[0] * g[1] for v, g in zip(u, m)],
                       [v[2] for v in u] + [v[2] * g[2] + v[3] * g[3] for v, g in zip(u, m)]]
                res = jax.lax.dot_general(operand(lhs), operand(rhs), _NT_DIMS, preferred_element_type=F32)
                past.append(res[0:8] if riders else None)
        _take(extra, NS)
        _take(chores, NS)

    def dft_passes(c):
        base = c % 2 * 256 if isinstance(c, int) else pl.multiple_of(c % 2 * 256, 256)
        for t in range(len(_BASE)):
            kt[t, 0:64, :] = _words(rs[t // 2, pl.ds(base + t % 2, 128, stride=2), :].astype(BF16))

        def kernel_pass(m):
            def run(values):
                lhs = paced([lambda g, idx=idx: kmat[idx, 8 * g:8 * g + 8, :] for _, idx in _KPASSES[m]],
                            2 * T, values)
                rhs = _halves(jnp.concatenate([kt[t, 0:64, :] for t, _ in _KPASSES[m]], axis=1))
                spec[NT + c, m, 0:2 * T, :] = jax.lax.dot_general(lhs, rhs, _NT_DIMS, preferred_element_type=F32)
            return run

        def signal_pass(m):
            def run(values):
                lhs = paced([lambda g: fwd_ref[8 * g:8 * g + 8, :]], 2 * T, values)
                block = xs[c, m * T:(m + 1) * T, :]
                xw[c, m * T // 2:(m + 1) * T // 2, :] = _words(block)
                spec[c, m, 0:2 * T, :] = jnp.dot(lhs, block, preferred_element_type=F32)
            return run

        return [make(m) for m in range(NB) for make in (signal_pass, kernel_pass)]

    def permute_weights(c):
        for part in range(3):
            for n in range(NT):
                col = part * D + n * 128
                tmp[part, n * 128:(n + 1) * 128, :] = wraw[c, :, col:col + 128].astype(F32).T
                yield []
            for j in range(DH):
                wt[c, pl.ds((part * D + j * H) // 2, H // 2), :] = _words(
                    tmp[part, pl.ds(j, H, stride=DH), :].astype(BF16))
                if j % 7 == 6:
                    yield []
        tmp[3] = woraw[c].astype(F32)
        yield []
        for j in range(DH):
            wop[c, pl.ds(j * H // 2, H // 2), :] = _words(tmp[3, pl.ds(j, H, stride=DH), :].astype(BF16))
            if j % 7 == 6:
                yield []

    with jax.named_scope("P0"):
        for cp in par_copies(0) + par_copies(1):
            cp.start()
        for cp in par_copies(0):
            cp.wait()
        km_copy.start()
        for cp in tile_copies(0):
            cp.start()
        for c in range(2, NT):
            for cp in par_copies(c):
                cp.start()
        _take(discretize(0, [None] * 8), NS)
        for cp in par_copies(1):
            cp.wait()
        generate(0, [], True, iter(()))
        for c in range(1, NT):
            for cp in tile_copies(c):
                cp.start()
        km_copy.wait()
        for c in range(2, NT):
            for cp in par_copies(c):
                cp.wait()

    def ssm_step(c, carry):
        for cp in tile_copies(c - 1):
            cp.wait()
        generate(c, dft_passes(c - 1), True, permute_weights(c - 1))
        return carry

    with jax.named_scope("P1"):
        jax.lax.fori_loop(1, NT - 1, ssm_step, 0)
    with jax.named_scope("P1b"):
        for cp in tile_copies(NT - 2) + tile_copies(NT - 1):
            cp.wait()
        generate(NT - 1, dft_passes(NT - 2), False, permute_weights(NT - 2))
        chores = permute_weights(NT - 1)
        for run in dft_passes(NT - 1):
            _take(chores, 1)
            run([])
        _take(chores, NS)

    for c in range(NT):
        ks[c, 0:PAD, :] = jnp.zeros((PAD, 128), F32)
        vs[c, 0:PAD, :] = jnp.zeros((PAD, 128), F32)
    q_scale = float(DH ** -0.5 * np.log2(np.e))
    n2 = S // M2
    ft_per_step = (T // 8) // n2

    def causal(a, b, j):
        acc = a[0] * b[j]
        for i in range(1, j + 1):
            acc = acc + a[i] * b[j - i]
        return acc

    even_order = [j for i in range(NB // 2) for j in (i, NB - 1 - i)]

    def convolve(it):
        def tile_of(f):
            return (it * ft_per_step + f) // 2 + f % 2 * (T // 16)

        def operands(f, c, phase):
            def load(slab, part):
                rows = pl.ds(pl.multiple_of(origin_ref[phase] + part * T + tile_of(f) * 8, 8), 8)
                return [spec[slab, m, rows, :] for m in range(NB)]

            plus, minus = (jnp.subtract, jnp.add) if f % 2 else (jnp.add, jnp.subtract)
            k_re, k_im = load(NT + c, 0), load(NT + c, 1)
            if phase == 0:
                return ([u + v for u, v in zip(load(c, 0), load(c, 1))],
                        [k_re[0]] + [minus(k_re[m], k_im[m - 1]) for m in range(1, NB)])
            if phase == 1:
                return load(c, 0), [k_im[0] - k_re[0]] + [
                    plus(k_im[m] - k_re[m], k_im[m - 1] + k_re[m - 1]) for m in range(1, NB)]
            return load(c, 1), [-k_im[0] - k_re[0]] + [
                (k_re[m - 1] - k_im[m - 1] if f % 2 else k_im[m - 1] - k_re[m - 1]) - (k_im[m] + k_re[m])
                for m in range(1, NB)]

        jobs = [(f, c, phase) for f in range(ft_per_step) for c in range(NT) for phase in range(3)]
        ahead, sums = operands(*jobs[0]), [{}, {}, {}]
        for n, (f, c, phase) in enumerate(jobs):
            a, b = ahead
            for i, j in enumerate(even_order):
                val = sums[phase][j] = causal(a, b, j)
                if i == RELEASE and n + 1 < len(jobs):
                    spec[2 * NT, 0, pl.ds(pl.multiple_of(origin_ref[3], 8), 8), :] = val
                    ahead = operands(*jobs[n + 1])
                if phase == 2:
                    z = jnp.concatenate([sums[0][j]] * 2, axis=0) + jnp.concatenate([val, sums[1][j]], axis=0)
                    val = _words(z.astype(BF16))
                    zs[j, c, pl.ds(pl.multiple_of(tile_of(f) * 8, 8), 8), :] = val
                yield val

    def logits(r0):
        past = [None] * LAG_S
        for t0 in range(0, M2, 8):
            q = [qs[c, t0:t0 + 8, :] for c in range(NT)]
            q[0] = behind(q[0], past[-LAG_S])
            for w in range(WIN):
                src = pl.ds(r0 + (t0 + PAD - DIL * w), 8)
                acc = q[0] * ks[0, src, :]
                for c in range(1, NT):
                    acc = acc + q[c] * ks[c, src, :]
                acc = acc + pltpu.roll(acc, 64, 1)
                acc = acc + pltpu.roll(acc, 32, 1)
                ps[w, pl.ds(r0 + t0, 8), :] = acc
            past.append(acc)
            yield

    def proj_step(it, carry):
        r0 = pl.multiple_of(it * M2, M2)
        conv, dots = convolve(it), logits(r0)
        x_panel = lambda c: lambda g: xw[c, pl.ds(pl.multiple_of(it * (M2 // 2), 8) + 8 * g, 8), :]
        place = lambda n, base: ((qs, ks, vs)[n // NT], (n % NT, pl.ds(base + (r0 + PAD if n >= NT else 0), M2)))
        todo, slots = 3 * NB * NT * ft_per_step, 0
        for n in range(3 * NT):
            if n % 4 == 0:
                hi = min(n + 4, 3 * NT)
                count = EARLY * todo * (slots + 1) // 260 - EARLY * todo * slots // 260 if slots < 13 else 0
                slots += 1
                xb = paced([x_panel(NT - 1)], M2, list(itertools.islice(conv, count)))
                tail = jax.lax.dot_general(xb, _halves(wt[NT - 1, n * 64:hi * 64, :]), _NT_DIMS,
                                           preferred_element_type=F32)
                for i in range(n, hi):
                    ref, idx = place(i, 0)
                    ref[idx] = tail[:, (i - n) * 128:(i - n + 1) * 128]
            if n < 2 * NT:
                count = EARLY * todo * (slots + 1) // 260 - EARLY * todo * slots // 260
                values = list(itertools.islice(conv, count))
            else:
                values = list(itertools.islice(conv, -(-(todo - EARLY * todo // 20) // NT)))
                for _ in itertools.islice(dots, -(-(M2 // 8) // NT)):
                    pass
            slots += 1
            xb = paced([x_panel(c) for c in range(NT - 1)], M2, values)
            w = _halves(jnp.concatenate([wt[c, n * 64:(n + 1) * 64, :] for c in range(NT - 1)], axis=1))
            ref, idx = place(n, pl.multiple_of(origin_ref[0], 8))
            res = jax.lax.dot_general(xb, w, _NT_DIMS, preferred_element_type=F32) + ref[idx]
            ref, idx = place(n, 0)
            ref[idx] = res if n >= NT else res * q_scale
        assert next(conv, None) is None and next(dots, 0) == 0
        return carry

    with jax.named_scope("P2"):
        jax.lax.fori_loop(0, n2, proj_step, 0)

    def attend(blk):
        r0 = 0 if isinstance(blk, int) else pl.multiple_of(blk * M3, M3)
        for t0 in range(0, M3, 16):
            logit = [ps[w, pl.ds(r0 + t0, 16), :] for w in range(WIN)]
            if isinstance(blk, int) and t0 == 0:
                pos = jax.lax.broadcasted_iota(jnp.int32, (16, 128), 0)
                logit = [jnp.where(pos >= DIL * w, l, -1e9) if w else l for w, l in enumerate(logit)]
            top = logit[0]
            for w in range(1, WIN):
                top = jnp.maximum(top, logit[w])
            e = [jnp.exp2(l - top) for l in logit]
            den = e[0]
            for w in range(1, WIN):
                den = den + e[w]
            inv = pl.reciprocal(den, approx=True)
            inv = inv * (2.0 - den * inv)
            for c in range(NT):
                acc = e[0] * vs[c, pl.ds(r0 + (t0 + PAD), 16), :]
                for w in range(1, WIN):
                    acc = acc + e[w] * vs[c, pl.ds(r0 + (t0 + PAD - DIL * w), 16), :]
                o = _words((acc * inv).astype(BF16))
                os_[blk % 2, c, t0 // 2:t0 // 2 + 8, :] = o
                yield o

    def out_copy(blk, c):
        rows = pl.ds(pl.multiple_of(blk * M3, M3), M3)
        return pltpu.make_async_copy(outs.at[c, rows], out_hbm.at[rows, lanes(c)], out_sem.at[blk, c])

    def gates(blk):
        r0 = 0 if isinstance(blk, int) else pl.multiple_of(blk * (M3 // 2), 8)
        gw_row = gw_ref[...].astype(F32).reshape(1, D)
        for g in range(M3 // 16):
            rows = pl.ds(r0 + 8 * g, 8)
            score = _halves(xw[0, rows, :]).astype(F32) * gw_row[:, 0:128]
            for c in range(1, NT):
                score = score + _halves(xw[c, rows, :]).astype(F32) * gw_row[:, c * 128:(c + 1) * 128]
            gate = jnp.broadcast_to(jax.nn.sigmoid(jnp.sum(score, axis=1, keepdims=True)), (16, 128))
            gs[blk % 2, 16 * g:16 * g + 16, :] = gate
            yield

    def finish(blk, work, total):
        rows = pl.ds(pl.multiple_of(blk * M3, M3), M3)
        word_rows = pl.ds(pl.multiple_of(blk * (M3 // 2), 8), M3 // 2)
        dskip_row = dskip_ref[...].astype(F32).reshape(1, D)
        spent = [0]

        def pull(cost):
            lo, spent[0] = spent[0], spent[0] + cost
            share = lambda t: total * max(t - LEAD, 0) // (35 - LEAD)
            return list(itertools.islice(work, share(spent[0]) - share(lo)))

        o_panel = lambda c: lambda g: oc[c, 8 * g:8 * g + 8, :]
        inv_panels = [lambda g, k=k: inv_ref[k, 8 * g:8 * g + 8, :] for k in range(2)]
        oc[:, 0:M3 // 2, :] = os_[blk % 2]
        for lo, hi in ((0, 4), (4, 5)):
            w = _halves(jnp.concatenate([wop[c, 256:320, :] for c in range(lo, hi)], axis=1))
            tail = jnp.dot(paced([o_panel(NT - 1)], M3, pull(hi - lo)), w, preferred_element_type=F32)
            for c in range(lo, hi):
                att[c, 0:M3, :] = tail[:, (c - lo) * 128:(c - lo + 1) * 128]
        for lo, hi in ((0, 2), (2, 4), (4, 5)):
            for i in range(M3 // T):
                z = _halves(jnp.concatenate([zs[blk * (M3 // T) + i, c, 0:T, :] for c in range(lo, hi)], axis=1))
                y = jnp.dot(paced(inv_panels, T, pull(hi - lo)), z, preferred_element_type=F32)
                for c in range(lo, hi):
                    ys[c, i * T:(i + 1) * T, :] = y[:, (c - lo) * 128:(c - lo + 1) * 128]
        back = pl.ds(pl.multiple_of(origin_ref[0], 8), M3)
        for c in range(NT):
            mixed = jnp.dot(paced([o_panel(k) for k in range(NT - 1)], M3, pull(4)), _halves(wop[c, 0:256, :]),
                            preferred_element_type=F32) + att[c, back, :]
            ssm = ys[c, back, :] + _halves(xw[c, word_rows, :]).astype(F32) * dskip_row[:, c * 128:(c + 1) * 128]
            outs[c, rows, :] = (ssm + gs[blk % 2] * (mixed - ssm)).astype(BF16)
        assert next(work, None) is None

    def prepare(blk):
        now, mix = attend(blk), gates(blk)
        for _ in range(M3 // 16):
            next(mix)
            yield from itertools.islice(now, NT)

    for _ in prepare(0):
        pass
    n3 = S // M3

    def out_step(it, carry):
        finish(it, prepare(it + 1), M3 // 16 * NT)
        for c in range(NT):
            out_copy(it, c).start()
        return carry

    with jax.named_scope("P3"):
        jax.lax.fori_loop(0, n3 - 1, out_step, 0)
    with jax.named_scope("P4"):
        finish(n3 - 1, iter(()), 0)
        for c in range(NT):
            out_copy(n3 - 1, c).start()
        for blk in range(n3):
            for c in range(NT):
                out_copy(blk, c).wait()


@jax.jit
def pallas_gated_mix__sliding_local_dilated__ssm_conv_s4__prompt_kernel(
    A_x: jax.Array,
    A_wqkv: jax.Array,
    A_wo: jax.Array,
    B_u: jax.Array,
    B_A_re: jax.Array,
    B_A_im: jax.Array,
    B_B_re: jax.Array,
    B_B_im: jax.Array,
    B_C_re: jax.Array,
    B_C_im: jax.Array,
    B_log_dt: jax.Array,
    B_Dskip: jax.Array,
    gate_w: jax.Array,
):
    del B_u
    assert A_x.shape == (1, S, D) and B_A_re.shape == (D, NS) and B_A_re.dtype == BF16
    hbm = pl.BlockSpec(memory_space=pl.ANY)
    vmem = pl.BlockSpec(memory_space=pltpu.VMEM)
    out = pl.pallas_call(
        _kernel,
        out_shape=jax.ShapeDtypeStruct((S, D), BF16),
        in_specs=[hbm] * 10 + [vmem] * 6 + [pl.BlockSpec(memory_space=pltpu.SMEM)],
        out_specs=hbm,
        scratch_shapes=[
            pltpu.VMEM((NT, S, 128), BF16),
            pltpu.VMEM((NT, S // 2 + SKEW, 128), jnp.int32),
            pltpu.VMEM((NT, 128, 3 * D), BF16),
            pltpu.VMEM((NT, D, 128), BF16),
            pltpu.VMEM(_KMATS.shape, jnp.int32),
            pltpu.VMEM((NT, 6, NS, 128), BF16),
            pltpu.VMEM((NT, 3 * D // 2 + SKEW, 128), jnp.int32),
            pltpu.VMEM((NT, D // 2 + SKEW, 128), jnp.int32),
            pltpu.VMEM((4, D, 128), F32),
            pltpu.VMEM((NT, 8, 128), F32),
            pltpu.VMEM((4, NS + SKEW, 128), F32),
            pltpu.VMEM((2, 8, 128 + SKEW, 128), F32),
            pltpu.VMEM((2, 4, 16 * _NQ + SKEW, 128), F32),
            pltpu.VMEM((3, 512 + SKEW, 128), F32),
            pltpu.VMEM((len(_BASE), 64 + SKEW, 128), jnp.int32),
            pltpu.VMEM((2 * NT + 1, NB, 2 * T + SKEW, 128), F32),
            pltpu.VMEM((NB, NT, T + SKEW, 128), jnp.int32),
            pltpu.VMEM((NT, M2 + SKEW, 128), F32),
            pltpu.VMEM((NT, S + PAD + SKEW, 128), F32),
            pltpu.VMEM((NT, S + PAD + SKEW, 128), F32),
            pltpu.VMEM((WIN, S + SKEW, 128), F32),
            pltpu.VMEM((2, NT, M3 // 2, 128), jnp.int32),
            pltpu.VMEM((NT, M3 // 2 + SKEW, 128), jnp.int32),
            pltpu.VMEM((2, M3, 128), F32),
            pltpu.VMEM((NT, M3 + SKEW, 128), F32),
            pltpu.VMEM((NT, M3 + SKEW, 128), F32),
            pltpu.VMEM((NT, S, 128), BF16),
            pltpu.SemaphoreType.DMA((NT,)),
            pltpu.SemaphoreType.DMA((NT,)),
            pltpu.SemaphoreType.DMA((NT,)),
            pltpu.SemaphoreType.DMA((1,)),
            pltpu.SemaphoreType.DMA((NT, 6)),
            pltpu.SemaphoreType.DMA((S // M3, NT)),
        ],
        compiler_params=pltpu.CompilerParams(vmem_limit_bytes=100 * 1024 * 1024),
    )(
        A_x.reshape(S, D), A_wqkv, A_wo, _KMATS,
        B_A_re.T, B_A_im.T, B_B_re.T, B_B_im.T, B_C_re.T, B_C_im.T,
        B_log_dt, B_Dskip, gate_w, _FWD, _INV, np.zeros((8, 128), np.int32), np.zeros((4,), np.int32),
    )
    return out.reshape(1, S, D)
```

```python
import itertools

import ml_dtypes
import numpy as np

import jax
import jax.numpy as jnp
import jax.experimental.pallas as pl
import jax.experimental.pallas.tpu as pltpu

F32 = jnp.float32
BF16 = jnp.bfloat16

S = 2048
D = 640
NS = 192
H = 32
DH = D // H
WIN, DIL = 8, 2
T = 128
NB = S // T
NT = D // 128
PAD = 16
M2 = 256
RELEASE = 11
LEAD = 0
HEAD = 6
TAIL = 3
LAG_D = 6
LAG_T = 4
LAG_V = 4
LAG_U = 4
SKEW = 8
LAG_S = 8
EARLY = 20
M3 = 256

_BASE = (0, 4, 256, 512, 1024, 2048)
_OFF = ((0, 1, 2, 3), (0, 1, 2, 3), (0, 2, 4, 6), (0, 4, 256, 260), (0, 256, 512, 768), (0, 0, 0, 0))


def _dft_constants():
    k = np.concatenate([np.arange(0, T, 2), np.arange(1, T, 2)])
    theta = 2.0 * np.pi * (k + 0.5) / (2 * T)
    ang = theta[:, None] * np.arange(T)[None, :]
    fwd = np.concatenate([np.cos(ang), -np.sin(ang)], axis=0)
    inv = np.stack([np.cos(ang).reshape(T // 8, 8, T), -np.sin(ang).reshape(T // 8, 8, T)], axis=1)
    inv = inv.reshape(2 * T, T).T / T
    slot = {}
    for t in range(len(_BASE)):
        for lane in range(128):
            i, a, p = lane // 8, (lane % 8) // 2, lane % 2
            slot.setdefault(_BASE[t] + _OFF[t][a] + 8 * (2 * i + p), (t, lane))
    lag = np.arange(S).astype(np.float32).astype(ml_dtypes.bfloat16).astype(np.float64).astype(np.int64)
    mats, passes = [], []
    for m in range(NB):
        per_tile = {}
        for n in range(T):
            t, lane = slot[int(lag[m * T + n])]
            per_tile.setdefault(t, np.zeros((2 * T, 128)))[:, lane] += fwd[:, n]
        passes.append(tuple((t, len(mats) + j) for j, t in enumerate(sorted(per_tile))))
        mats.extend(per_tile[t] for t in sorted(per_tile))

    def to_bf16(a):
        bits = np.asarray(a, np.float32).astype(ml_dtypes.bfloat16).view(np.uint16).astype(np.uint32)
        return (bits[..., 0::2, :] | (bits[..., 1::2, :] << 16)).view(np.int32)

    inv = inv.reshape(T, 2, T).transpose(1, 0, 2)
    return to_bf16(fwd), to_bf16(inv), to_bf16(np.stack(mats)), tuple(passes)


_FWD, _INV, _KMATS, _KPASSES = _dft_constants()

_Q_W, _Q_G, _Q_V, _Q_REC, _NQ = 0, 6, 9, 11, 12

_NT_DIMS = (((1,), (1,)), ((), ()))


def _csq(z):
    x, y, p, q = z
    return ((x - y) * (x + y), (x + x) * y, (p - q) * (p + q), (p + p) * q)


def _cmul(a, b):
    ax, ay, ap, aq = a
    bx, by, bp, bq = b
    return (ax * bx - ay * by, ax * by + ay * bx, ap * bp - aq * bq, ap * bq + aq * bp)


def _words(v):
    return pltpu.bitcast(v, jnp.int32)


def _halves(v):
    return pltpu.bitcast(v, BF16)


def _take(gen, n):
    out = []
    for _ in range(n):
        out += next(gen, [])
    return out


def _kernel(x_hbm, wqkv_hbm, wo_hbm, kmat_hbm, are_hbm, aim_hbm, bre_hbm, bim_hbm, cre_hbm, cim_hbm,
            ldt_ref, dskip_ref, gw_ref, fwd_ref, inv_ref, zero_ref, origin_ref,
            out_hbm,
            xs, xw, wraw, woraw, kmat, par, wt, wop, tmp, dts, disc, zw, tab, rs, kt, spec, zs, qs, ks, vs, ps, os_, oc, gs, att, ys, outs,
            x_sem, w_sem, wo_sem, km_sem, par_sem, out_sem):
    def lanes(c):
        return pl.ds(c * 128, 128) if isinstance(c, int) else pl.ds(pl.multiple_of(c * 128, 128), 128)

    def par_copies(c):
        return [pltpu.make_async_copy(src.at[:, lanes(c)], par.at[c, i], par_sem.at[c, i])
                for i, src in enumerate((are_hbm, aim_hbm, bre_hbm, bim_hbm, cre_hbm, cim_hbm))]

    def tile_copies(c):
        return [pltpu.make_async_copy(x_hbm.at[:, lanes(c)], xs.at[c], x_sem.at[c]),
                pltpu.make_async_copy(wqkv_hbm.at[lanes(c), :], wraw.at[c], w_sem.at[c]),
                pltpu.make_async_copy(wo_hbm.at[:, lanes(c)], woraw.at[c], wo_sem.at[c])]

    km_copy = pltpu.make_async_copy(kmat_hbm, kmat, km_sem.at[0])

    lane = jax.lax.broadcasted_iota(jnp.int32, (8, 128), 1)
    row = jax.lax.broadcasted_iota(jnp.int32, (8, 128), 0)
    low = lane < 64
    never = zero_ref[...] != 0

    def behind(val, earlier):
        return val if earlier is None else jnp.where(never, earlier, val)

    def paced(panels, rows, values):
        groups = rows // 16
        regs = [[panel(g) for panel in panels] for g in range(groups)]
        order = [(g, c) for g in range(groups) for c in range(len(panels))]
        for n, val in enumerate(values):
            g, c = order[n * len(order) // len(values)]
            regs[g][c] = jnp.where(never, _words(val), regs[g][c])
        return _halves(jnp.concatenate([jnp.concatenate(r, axis=1) for r in regs], axis=0))

    dt_row = jnp.exp(ldt_ref[...].astype(F32).reshape(1, D)).astype(BF16).astype(F32)
    for c in range(NT):
        dts[c] = jnp.broadcast_to(dt_row[:, c * 128:(c + 1) * 128], (8, 128))

    def discretize(c, past):
        dt = dts[c][0:1, :]
        for r in range(NS // 32):
            raw = [par[c, i, 32 * r:32 * r + 32, :].astype(F32) for i in range(6)]
            for n in range(4):
                a_re, a_im, b_re, b_im, c_re, c_im = (v[8 * n:8 * n + 8] for v in raw)
                mag, ang = jnp.exp(dt * a_re), behind(dt * a_im, past[-LAG_D])
                db_re, db_im = dt * b_re, dt * b_im
                vals = (mag * jnp.cos(ang), mag * jnp.sin(ang),
                        c_re * db_re - c_im * db_im, c_re * db_im + c_im * db_re)
                for i, val in enumerate(vals):
                    disc[i, 32 * r + 8 * n:32 * r + 8 * n + 8, :] = val
                yield list(vals[:2])
        for i in range(2):
            zw[c % 2, 4 * i + 0] = disc[2 * i, 0:128, :].T
            zw[c % 2, 4 * i + 1] = disc[2 * i + 1, 0:128, :].T
            yield []
            re, im = disc[2 * i, 128:NS, :], disc[2 * i + 1, 128:NS, :]
            zw[c % 2, 4 * i + 2] = jnp.concatenate([re, re], axis=0).T
            zw[c % 2, 4 * i + 3] = jnp.concatenate([-im, im], axis=0).T
            yield []

    def put(tile, slot, even, odd):
        for comp in range(len(even)):
            tab[tile % 2, comp, pl.ds(16 * slot, 8, stride=2), :] = even[comp]
            tab[tile % 2, comp, pl.ds(16 * slot + 1, 8, stride=2), :] = odd[comp]

    def get(group, slot, comps):
        tile, half = divmod(group, 2)
        return tuple(tab[tile % 2, comp, pl.ds(16 * slot + 8 * half, 8), :] for comp in range(comps))

    def running(z, conj=False):
        x, y, p, q = z
        if conj:
            return (x, -y, jnp.where(low, p, -q))
        return (x, y, jnp.where(low, p, q), jnp.where(low, -q, p))

    def tables(c, tile, earlier):
        rows = slice(8 * tile, 8 * tile + 8)
        one = (jnp.ones((8, 128), F32), jnp.zeros((8, 128), F32)) * 2
        z1 = tuple(behind(zw[c % 2, i, rows, :], earlier if i % 2 == 0 else None) for i in range(4))
        w = tuple(zw[c % 2, 4 + i, rows, :] for i in range(4))
        z2 = _csq(z1)
        put(tile, _Q_G, z2, z2)
        z4 = _csq(z2)
        w4 = _cmul(w, z4)
        put(tile, _Q_W, running(w), running(w4))
        put(tile, _Q_W + 3, running(_cmul(w, z1)), running(_cmul(w4, z1)))
        z8 = _csq(z4)
        put(tile, _Q_V, running(one, True), running(z8, True))
        z16 = _csq(z8)
        z24 = _cmul(z16, z8)
        put(tile, _Q_V + 1, running(z16, True), running(z24, True))
        x, y, p, q = z16
        rec = (x + x, x * x + y * y, p + p, p * p + q * q)
        put(tile, _Q_REC, rec, rec)
        z256 = _csq(_csq(_csq(_csq(z16))))
        put(tile, _Q_G + 1, z4, z256)
        yield [z24[0], z24[2], z256[0], z256[2]]
        z512 = _csq(z256)
        put(tile, _Q_G + 2, z512, one)
        w256, w512 = _cmul(w, z256), _cmul(w, z512)
        put(tile, _Q_W + 1, running(w256), running(w512))
        w258, w516 = _cmul(w256, z2), _cmul(w512, z4)
        put(tile, _Q_W + 4, running(w258), running(w516))
        z1024 = _csq(z512)
        w1024 = _cmul(w, z1024)
        w1280, w2048 = _cmul(w1024, z256), _cmul(w1024, z1024)
        put(tile, _Q_W + 2, running(w1024), running(w2048))
        put(tile, _Q_W + 5, running(w1280), running(w2048))
        yield [w258[0], w516[2], w1280[0], w2048[2]]

    def operand(panels):
        return jnp.concatenate([jnp.concatenate(parts, axis=0) for parts in panels], axis=1).astype(BF16)

    chan = row // 2
    slot_of_lane = ((lane // 2) - chan) % 4

    def generate(c, riders, upcoming, chores):
        base = c % 2 * 256 if isinstance(c, int) else pl.multiple_of(c % 2 * 256, 256)
        slots = 32 + HEAD + TAIL
        for rider in riders[:HEAD * len(riders) // slots]:
            rider([])
        _take(tables(c, 0, None), 2)
        res, stage2, stage3, past = None, [], [], [None] * 8
        extra = discretize(c + 1, past) if upcoming else iter(())
        for group in range(32 + 3):
            for i, r in enumerate(stage3):
                rs[i, pl.ds(base + 8 * (group - 3), 8), :] = jnp.where(
                    (chan & 2) == 2, pltpu.roll(r, 128 - 4, 1), r)
            stage3 = [jnp.where((chan & 1) == 1, pltpu.roll(r, 128 - 2, 1), r) for r in stage2]
            stage2 = []
            for i in range(3 if res is not None else 0):
                r = res[8 * i:8 * i + 8]
                for a in range(1, 4):
                    blk = res[24 * a + 8 * i:24 * a + 8 * i + 8]
                    r = jnp.where(slot_of_lane == a, pltpu.roll(blk, 2 * a, 1), r)
                stage2.append(r)
            res = None
            ride = riders[(group + HEAD) * len(riders) // slots:(group + HEAD + 1) * len(riders) // slots]
            if group >= 32:
                for rider in ride:
                    rider([])
            else:
                if group % 2 == 0:
                    ahead = tables(c, group // 2 + 1, past[-LAG_T]) if group + 2 < 32 else iter(())
                _take(chores, 1)
                pace = _take(extra, 1) + _take(ahead, 1)
                for n, rider in enumerate(ride):
                    rider(pace[n * len(pace) // len(ride):(n + 1) * len(pace) // len(ride)])
                a_lo, b_lo, a_hi, b_hi = get(group, _Q_REC, 4)
                rhs = []
                for al, be, v in zip((a_lo, a_lo, a_hi), (b_lo, b_lo, b_hi),
                                     zip(get(group, _Q_V, 3), get(group, _Q_V + 1, 3))):
                    v = [v[0], behind(v[1], past[-LAG_V])]
                    for i in range(2, 16):
                        v.append(al * v[i - 1] - be * v[i - 2])
                    rhs.append(v)
                u = [get(group, _Q_W + n, 4) for n in range(6)]
                m = [tuple(behind(g, past[-LAG_U]) for g in get(group, _Q_G + i, 4)) for i in range(3)] * 2
                lhs = [[v[0] for v in u] + [v[0] * g[0] - v[1] * g[1] for v, g in zip(u, m)],
                       [v[1] for v in u] + [v[1] * g[0] + v[0] * g[1] for v, g in zip(u, m)],
                       [v[2] for v in u] + [v[2] * g[2] + v[3] * g[3] for v, g in zip(u, m)]]
                res = jax.lax.dot_general(operand(lhs), operand(rhs), _NT_DIMS, preferred_element_type=F32)
                past.append(res[0:8] if riders else None)
        _take(extra, NS)
        _take(chores, NS)

    def dft_passes(c):
        base = c % 2 * 256 if isinstance(c, int) else pl.multiple_of(c % 2 * 256, 256)
        for t in range(len(_BASE)):
            kt[t] = _words(rs[t // 2, pl.ds(base + t % 2, 128, stride=2), :].astype(BF16))

        def kernel_pass(m):
            def run(values):
                lhs = paced([lambda g, idx=idx: kmat[idx, 8 * g:8 * g + 8, :] for _, idx in _KPASSES[m]],
                            2 * T, values)
                rhs = _halves(jnp.concatenate([kt[t] for t, _ in _KPASSES[m]], axis=1))
                spec[NT + c, m, 0:2 * T, :] = jax.lax.dot_general(lhs, rhs, _NT_DIMS, preferred_element_type=F32)
            return run

        def signal_pass(m):
            def run(values):
                lhs = paced([lambda g: fwd_ref[8 * g:8 * g + 8, :]], 2 * T, values)
                block = xs[c, m * T:(m + 1) * T, :]
                xw[c, m * T // 2:(m + 1) * T // 2, :] = _words(block)
                spec[c, m, 0:2 * T, :] = jnp.dot(lhs, block, preferred_element_type=F32)
            return run

        return [make(m) for m in range(NB) for make in (signal_pass, kernel_pass)]

    def permute_weights(c):
        for part in range(3):
            for n in range(NT):
                col = part * D + n * 128
                tmp[part, n * 128:(n + 1) * 128, :] = wraw[c, :, col:col + 128].astype(F32).T
                yield []
            for j in range(DH):
                wt[c, pl.ds((part * D + j * H) // 2, H // 2), :] = _words(
                    tmp[part, pl.ds(j, H, stride=DH), :].astype(BF16))
                if j % 7 == 6:
                    yield []
        tmp[3] = woraw[c].astype(F32)
        yield []
        for j in range(DH):
            wop[c, pl.ds(j * H // 2, H // 2), :] = _words(tmp[3, pl.ds(j, H, stride=DH), :].astype(BF16))
            if j % 7 == 6:
                yield []

    with jax.named_scope("P0"):
        for cp in par_copies(0) + par_copies(1):
            cp.start()
        for cp in par_copies(0):
            cp.wait()
        km_copy.start()
        for cp in tile_copies(0):
            cp.start()
        for c in range(2, NT):
            for cp in par_copies(c):
                cp.start()
        _take(discretize(0, [None] * 8), NS)
        for cp in par_copies(1):
            cp.wait()
        generate(0, [], True, iter(()))
        for c in range(1, NT):
            for cp in tile_copies(c):
                cp.start()
        km_copy.wait()
        for c in range(2, NT):
            for cp in par_copies(c):
                cp.wait()

    def ssm_step(c, carry):
        for cp in tile_copies(c - 1):
            cp.wait()
        generate(c, dft_passes(c - 1), True, permute_weights(c - 1))
        return carry

    with jax.named_scope("P1"):
        jax.lax.fori_loop(1, NT - 1, ssm_step, 0)
    with jax.named_scope("P1b"):
        for cp in tile_copies(NT - 2) + tile_copies(NT - 1):
            cp.wait()
        generate(NT - 1, dft_passes(NT - 2), False, permute_weights(NT - 2))
        chores = permute_weights(NT - 1)
        for run in dft_passes(NT - 1):
            _take(chores, 1)
            run([])
        _take(chores, NS)

    for c in range(NT):
        ks[c, 0:PAD, :] = jnp.zeros((PAD, 128), F32)
        vs[c, 0:PAD, :] = jnp.zeros((PAD, 128), F32)
    q_scale = float(DH ** -0.5 * np.log2(np.e))
    n2 = S // M2
    ft_per_step = (T // 8) // n2

    def causal(a, b, j):
        acc = a[0] * b[j]
        for i in range(1, j + 1):
            acc = acc + a[i] * b[j - i]
        return acc

    even_order = [j for i in range(NB // 2) for j in (i, NB - 1 - i)]

    def convolve(it):
        def tile_of(f):
            return (it * ft_per_step + f) // 2 + f % 2 * (T // 16)

        def operands(f, c, phase):
            def load(slab, part):
                rows = pl.ds(pl.multiple_of(origin_ref[phase] + part * T + tile_of(f) * 8, 8), 8)
                return [spec[slab, m, rows, :] for m in range(NB)]

            plus, minus = (jnp.subtract, jnp.add) if f % 2 else (jnp.add, jnp.subtract)
            k_re, k_im = load(NT + c, 0), load(NT + c, 1)
            if phase == 0:
                return ([u + v for u, v in zip(load(c, 0), load(c, 1))],
                        [k_re[0]] + [minus(k_re[m], k_im[m - 1]) for m in range(1, NB)])
            if phase == 1:
                return load(c, 0), [k_im[0] - k_re[0]] + [
                    plus(k_im[m] - k_re[m], k_im[m - 1] + k_re[m - 1]) for m in range(1, NB)]
            return load(c, 1), [-k_im[0] - k_re[0]] + [
                (k_re[m - 1] - k_im[m - 1] if f % 2 else k_im[m - 1] - k_re[m - 1]) - (k_im[m] + k_re[m])
                for m in range(1, NB)]

        jobs = [(f, c, phase) for f in range(ft_per_step) for c in range(NT) for phase in range(3)]
        ahead, sums = operands(*jobs[0]), [{}, {}, {}]
        for n, (f, c, phase) in enumerate(jobs):
            a, b = ahead
            for i, j in enumerate(even_order):
                val = sums[phase][j] = causal(a, b, j)
                if i == RELEASE and n + 1 < len(jobs):
                    spec[2 * NT, 0, pl.ds(pl.multiple_of(origin_ref[3], 8), 8), :] = val
                    ahead = operands(*jobs[n + 1])
                if phase == 2:
                    z = jnp.concatenate([sums[0][j]] * 2, axis=0) + jnp.concatenate([val, sums[1][j]], axis=0)
                    val = _words(z.astype(BF16))
                    zs[j, c, pl.ds(pl.multiple_of(tile_of(f) * 8, 8), 8), :] = val
                yield val

    def logits(r0):
        past = [None] * LAG_S
        for t0 in range(0, M2, 8):
            q = [qs[c, t0:t0 + 8, :] for c in range(NT)]
            q[0] = behind(q[0], past[-LAG_S])
            for w in range(WIN):
                src = pl.ds(r0 + (t0 + PAD - DIL * w), 8)
                acc = q[0] * ks[0, src, :]
                for c in range(1, NT):
                    acc = acc + q[c] * ks[c, src, :]
                acc = acc + pltpu.roll(acc, 64, 1)
                acc = acc + pltpu.roll(acc, 32, 1)
                ps[w, pl.ds(r0 + t0, 8), :] = acc
            past.append(acc)
            yield

    def proj_step(it, carry):
        r0 = pl.multiple_of(it * M2, M2)
        conv, dots = convolve(it), logits(r0)
        x_panel = lambda c: lambda g: xw[c, pl.ds(pl.multiple_of(it * (M2 // 2), 8) + 8 * g, 8), :]
        place = lambda n, base: ((qs, ks, vs)[n // NT], (n % NT, pl.ds(base + (r0 + PAD if n >= NT else 0), M2)))
        todo, slots = 3 * NB * NT * ft_per_step, 0
        for n in range(3 * NT):
            if n % 4 == 0:
                hi = min(n + 4, 3 * NT)
                count = EARLY * todo * (slots + 1) // 260 - EARLY * todo * slots // 260 if slots < 13 else 0
                slots += 1
                xb = paced([x_panel(NT - 1)], M2, list(itertools.islice(conv, count)))
                tail = jax.lax.dot_general(xb, _halves(wt[NT - 1, n * 64:hi * 64, :]), _NT_DIMS,
                                           preferred_element_type=F32)
                for i in range(n, hi):
                    ref, idx = place(i, 0)
                    ref[idx] = tail[:, (i - n) * 128:(i - n + 1) * 128]
            if n < 2 * NT:
                count = EARLY * todo * (slots + 1) // 260 - EARLY * todo * slots // 260
                values = list(itertools.islice(conv, count))
            else:
                values = list(itertools.islice(conv, -(-(todo - EARLY * todo // 20) // NT)))
                for _ in itertools.islice(dots, -(-(M2 // 8) // NT)):
                    pass
            slots += 1
            xb = paced([x_panel(c) for c in range(NT - 1)], M2, values)
            w = _halves(jnp.concatenate([wt[c, n * 64:(n + 1) * 64, :] for c in range(NT - 1)], axis=1))
            ref, idx = place(n, pl.multiple_of(origin_ref[0], 8))
            res = jax.lax.dot_general(xb, w, _NT_DIMS, preferred_element_type=F32) + ref[idx]
            ref, idx = place(n, 0)
            ref[idx] = res if n >= NT else res * q_scale
        assert next(conv, None) is None and next(dots, 0) == 0
        return carry

    with jax.named_scope("P2"):
        jax.lax.fori_loop(0, n2, proj_step, 0)

    def attend(blk):
        r0 = 0 if isinstance(blk, int) else pl.multiple_of(blk * M3, M3)
        for t0 in range(0, M3, 16):
            logit = [ps[w, pl.ds(r0 + t0, 16), :] for w in range(WIN)]
            if isinstance(blk, int) and t0 == 0:
                pos = jax.lax.broadcasted_iota(jnp.int32, (16, 128), 0)
                logit = [jnp.where(pos >= DIL * w, l, -1e9) if w else l for w, l in enumerate(logit)]
            top = logit[0]
            for w in range(1, WIN):
                top = jnp.maximum(top, logit[w])
            e = [jnp.exp2(l - top) for l in logit]
            den = e[0]
            for w in range(1, WIN):
                den = den + e[w]
            inv = pl.reciprocal(den, approx=True)
            inv = inv * (2.0 - den * inv)
            for c in range(NT):
                acc = e[0] * vs[c, pl.ds(r0 + (t0 + PAD), 16), :]
                for w in range(1, WIN):
                    acc = acc + e[w] * vs[c, pl.ds(r0 + (t0 + PAD - DIL * w), 16), :]
                o = _words((acc * inv).astype(BF16))
                os_[blk % 2, c, t0 // 2:t0 // 2 + 8, :] = o
                yield o

    def out_copy(blk, c):
        rows = pl.ds(pl.multiple_of(blk * M3, M3), M3)
        return pltpu.make_async_copy(outs.at[c, rows], out_hbm.at[rows, lanes(c)], out_sem.at[blk, c])

    def gates(blk):
        r0 = 0 if isinstance(blk, int) else pl.multiple_of(blk * (M3 // 2), 8)
        gw_row = gw_ref[...].astype(F32).reshape(1, D)
        for g in range(M3 // 16):
            rows = pl.ds(r0 + 8 * g, 8)
            score = _halves(xw[0, rows, :]).astype(F32) * gw_row[:, 0:128]
            for c in range(1, NT):
                score = score + _halves(xw[c, rows, :]).astype(F32) * gw_row[:, c * 128:(c + 1) * 128]
            gate = jnp.broadcast_to(jax.nn.sigmoid(jnp.sum(score, axis=1, keepdims=True)), (16, 128))
            gs[blk % 2, 16 * g:16 * g + 16, :] = gate
            yield

    def finish(blk, work, total):
        rows = pl.ds(pl.multiple_of(blk * M3, M3), M3)
        word_rows = pl.ds(pl.multiple_of(blk * (M3 // 2), 8), M3 // 2)
        dskip_row = dskip_ref[...].astype(F32).reshape(1, D)
        spent = [0]

        def pull(cost):
            lo, spent[0] = spent[0], spent[0] + cost
            share = lambda t: total * max(t - LEAD, 0) // (35 - LEAD)
            return list(itertools.islice(work, share(spent[0]) - share(lo)))

        o_panel = lambda c: lambda g: oc[c, 8 * g:8 * g + 8, :]
        inv_panels = [lambda g, k=k: inv_ref[k, 8 * g:8 * g + 8, :] for k in range(2)]
        oc[...] = os_[blk % 2]
        for lo, hi in ((0, 4), (4, 5)):
            w = _halves(jnp.concatenate([wop[c, 256:320, :] for c in range(lo, hi)], axis=1))
            tail = jnp.dot(paced([o_panel(NT - 1)], M3, pull(hi - lo)), w, preferred_element_type=F32)
            for c in range(lo, hi):
                att[c] = tail[:, (c - lo) * 128:(c - lo + 1) * 128]
        for lo, hi in ((0, 2), (2, 4), (4, 5)):
            for i in range(M3 // T):
                z = _halves(jnp.concatenate([zs[blk * (M3 // T) + i, c] for c in range(lo, hi)], axis=1))
                y = jnp.dot(paced(inv_panels, T, pull(hi - lo)), z, preferred_element_type=F32)
                for c in range(lo, hi):
                    ys[c, i * T:(i + 1) * T, :] = y[:, (c - lo) * 128:(c - lo + 1) * 128]
        back = pl.ds(pl.multiple_of(origin_ref[0], 8), M3)
        for c in range(NT):
            mixed = jnp.dot(paced([o_panel(k) for k in range(NT - 1)], M3, pull(4)), _halves(wop[c, 0:256, :]),
                            preferred_element_type=F32) + att[c, back, :]
            ssm = ys[c, back, :] + _halves(xw[c, word_rows, :]).astype(F32) * dskip_row[:, c * 128:(c + 1) * 128]
            outs[c, rows, :] = (ssm + gs[blk % 2] * (mixed - ssm)).astype(BF16)
        assert next(work, None) is None

    def prepare(blk):
        now, mix = attend(blk), gates(blk)
        for _ in range(M3 // 16):
            next(mix)
            yield from itertools.islice(now, NT)

    for _ in prepare(0):
        pass
    n3 = S // M3

    def out_step(it, carry):
        finish(it, prepare(it + 1), M3 // 16 * NT)
        for c in range(NT):
            out_copy(it, c).start()
        return carry

    with jax.named_scope("P3"):
        jax.lax.fori_loop(0, n3 - 1, out_step, 0)
    with jax.named_scope("P4"):
        finish(n3 - 1, iter(()), 0)
        for c in range(NT):
            out_copy(n3 - 1, c).start()
        for blk in range(n3):
            for c in range(NT):
                out_copy(blk, c).wait()


@jax.jit
def pallas_gated_mix__sliding_local_dilated__ssm_conv_s4__prompt_kernel(
    A_x: jax.Array,
    A_wqkv: jax.Array,
    A_wo: jax.Array,
    B_u: jax.Array,
    B_A_re: jax.Array,
    B_A_im: jax.Array,
    B_B_re: jax.Array,
    B_B_im: jax.Array,
    B_C_re: jax.Array,
    B_C_im: jax.Array,
    B_log_dt: jax.Array,
    B_Dskip: jax.Array,
    gate_w: jax.Array,
):
    del B_u
    assert A_x.shape == (1, S, D) and B_A_re.shape == (D, NS) and B_A_re.dtype == BF16
    hbm = pl.BlockSpec(memory_space=pl.ANY)
    vmem = pl.BlockSpec(memory_space=pltpu.VMEM)
    out = pl.pallas_call(
        _kernel,
        out_shape=jax.ShapeDtypeStruct((S, D), BF16),
        in_specs=[hbm] * 10 + [vmem] * 6 + [pl.BlockSpec(memory_space=pltpu.SMEM)],
        out_specs=hbm,
        scratch_shapes=[
            pltpu.VMEM((NT, S, 128), BF16),
            pltpu.VMEM((NT, S // 2 + SKEW, 128), jnp.int32),
            pltpu.VMEM((NT, 128, 3 * D), BF16),
            pltpu.VMEM((NT, D, 128), BF16),
            pltpu.VMEM(_KMATS.shape, jnp.int32),
            pltpu.VMEM((NT, 6, NS, 128), BF16),
            pltpu.VMEM((NT, 3 * D // 2 + SKEW, 128), jnp.int32),
            pltpu.VMEM((NT, D // 2, 128), jnp.int32),
            pltpu.VMEM((4, D, 128), F32),
            pltpu.VMEM((NT, 8, 128), F32),
            pltpu.VMEM((4, NS, 128), F32),
            pltpu.VMEM((2, 8, 128, 128), F32),
            pltpu.VMEM((2, 4, 16 * _NQ + SKEW, 128), F32),
            pltpu.VMEM((3, 512, 128), F32),
            pltpu.VMEM((len(_BASE), 64, 128), jnp.int32),
            pltpu.VMEM((2 * NT + 1, NB, 2 * T + SKEW, 128), F32),
            pltpu.VMEM((NB, NT, T, 128), jnp.int32),
            pltpu.VMEM((NT, M2 + SKEW, 128), F32),
            pltpu.VMEM((NT, S + PAD + SKEW, 128), F32),
            pltpu.VMEM((NT, S + PAD + 3 * SKEW, 128), F32),
            pltpu.VMEM((WIN, S + SKEW, 128), F32),
            pltpu.VMEM((2, NT, M3 // 2, 128), jnp.int32),
            pltpu.VMEM((NT, M3 // 2, 128), jnp.int32),
            pltpu.VMEM((2, M3, 128), F32),
            pltpu.VMEM((NT, M3, 128), F32),
            pltpu.VMEM((NT, M3, 128), F32),
            pltpu.VMEM((NT, S, 128), BF16),
            pltpu.SemaphoreType.DMA((NT,)),
            pltpu.SemaphoreType.DMA((NT,)),
            pltpu.SemaphoreType.DMA((NT,)),
            pltpu.SemaphoreType.DMA((1,)),
            pltpu.SemaphoreType.DMA((NT, 6)),
            pltpu.SemaphoreType.DMA((S // M3, NT)),
        ],
        compiler_params=pltpu.CompilerParams(vmem_limit_bytes=100 * 1024 * 1024),
    )(
        A_x.reshape(S, D), A_wqkv, A_wo, _KMATS,
        B_A_re.T, B_A_im.T, B_B_re.T, B_B_im.T, B_C_re.T, B_C_im.T,
        B_log_dt, B_Dskip, gate_w, _FWD, _INV, np.zeros((8, 128), np.int32), np.zeros((4,), np.int32),
    )
    return out.reshape(1, S, D)
```

```python
import itertools

import ml_dtypes
import numpy as np

import jax
import jax.numpy as jnp
import jax.experimental.pallas as pl
import jax.experimental.pallas.tpu as pltpu

F32 = jnp.float32
BF16 = jnp.bfloat16

S = 2048
D = 640
NS = 192
H = 32
DH = D // H
WIN, DIL = 8, 2
T = 128
NB = S // T
NT = D // 128
PAD = 16
M2 = 256
M3 = 256
SKEW = 8

HEAD, TAIL = 6, 2
LAG, LAG_D = 4, 6
LAG_S = 8
RELEASE = 9
EARLY = 20
LEAD = 4

_BASE = (0, 4, 256, 512, 1024, 2048)
_OFF = ((0, 1, 2, 3), (0, 1, 2, 3), (0, 2, 4, 6), (0, 4, 256, 260), (0, 256, 512, 768), (0, 0, 0, 0))


def _dft_constants():
    k = np.concatenate([np.arange(0, T, 2), np.arange(1, T, 2)])
    theta = 2.0 * np.pi * (k + 0.5) / (2 * T)
    ang = theta[:, None] * np.arange(T)[None, :]
    fwd = np.concatenate([np.cos(ang), -np.sin(ang)], axis=0)
    inv = np.stack([np.cos(ang).reshape(T // 8, 8, T), -np.sin(ang).reshape(T // 8, 8, T)], axis=1)
    inv = inv.reshape(2 * T, T).T / T
    slot = {}
    for t in range(len(_BASE)):
        for lane in range(128):
            i, a, p = lane // 8, (lane % 8) // 2, lane % 2
            slot.setdefault(_BASE[t] + _OFF[t][a] + 8 * (2 * i + p), (t, lane))
    lag = np.arange(S).astype(np.float32).astype(ml_dtypes.bfloat16).astype(np.float64).astype(np.int64)
    mats, passes = [], []
    for m in range(NB):
        per_tile = {}
        for n in range(T):
            t, lane = slot[int(lag[m * T + n])]
            per_tile.setdefault(t, np.zeros((2 * T, 128)))[:, lane] += fwd[:, n]
        passes.append(tuple((t, len(mats) + j) for j, t in enumerate(sorted(per_tile))))
        mats.extend(per_tile[t] for t in sorted(per_tile))

    def to_bf16(a):
        bits = np.asarray(a, np.float32).astype(ml_dtypes.bfloat16).view(np.uint16).astype(np.uint32)
        return (bits[..., 0::2, :] | (bits[..., 1::2, :] << 16)).view(np.int32)

    inv = inv.reshape(T, 2, T).transpose(1, 0, 2)
    return to_bf16(fwd), to_bf16(inv), to_bf16(np.stack(mats)), tuple(passes)


_FWD, _INV, _KMATS, _KPASSES = _dft_constants()

_Q_W, _Q_G, _Q_V, _Q_REC, _NQ = 0, 6, 9, 11, 12

_NT_DIMS = (((1,), (1,)), ((), ()))


def _csq(z):
    x, y, p, q = z
    return ((x - y) * (x + y), (x + x) * y, (p - q) * (p + q), (p + p) * q)


def _cmul(a, b):
    ax, ay, ap, aq = a
    bx, by, bp, bq = b
    return (ax * bx - ay * by, ax * by + ay * bx, ap * bp - aq * bq, ap * bq + aq * bp)


def _words(v):
    return pltpu.bitcast(v, jnp.int32)


def _halves(v):
    return pltpu.bitcast(v, BF16)


def _take(gen, n):
    out = []
    for _ in range(n):
        out += next(gen, [])
    return out


def _kernel(x_hbm, wqkv_hbm, wo_hbm, kmat_hbm, are_hbm, aim_hbm, bre_hbm, bim_hbm, cre_hbm, cim_hbm,
            ldt_ref, dskip_ref, gw_ref, fwd_ref, inv_ref, zero_ref, origin_ref,
            out_hbm,
            xs, xw, wraw, woraw, kmat, par, wt, wop, tmp, dts, disc, zw, tab, rs, kt, spec, zs, qs, ks, vs, ps, os_, oc, gs, att, ys, outs,
            x_sem, w_sem, wo_sem, km_sem, par_sem, out_sem):
    def lanes(c):
        return pl.ds(c * 128, 128) if isinstance(c, int) else pl.ds(pl.multiple_of(c * 128, 128), 128)

    def par_copies(c):
        return [pltpu.make_async_copy(src.at[:, lanes(c)], par.at[c, i], par_sem.at[c, i])
                for i, src in enumerate((are_hbm, aim_hbm, bre_hbm, bim_hbm, cre_hbm, cim_hbm))]

    def tile_copies(c):
        return [pltpu.make_async_copy(x_hbm.at[:, lanes(c)], xs.at[c], x_sem.at[c]),
                pltpu.make_async_copy(wqkv_hbm.at[lanes(c), :], wraw.at[c], w_sem.at[c]),
                pltpu.make_async_copy(wo_hbm.at[:, lanes(c)], woraw.at[c], wo_sem.at[c])]

    km_copy = pltpu.make_async_copy(kmat_hbm, kmat, km_sem.at[0])

    lane = jax.lax.broadcasted_iota(jnp.int32, (8, 128), 1)
    row = jax.lax.broadcasted_iota(jnp.int32, (8, 128), 0)
    low = lane < 64
    never = zero_ref[...] != 0

    def behind(val, earlier):
        return val if earlier is None else jnp.where(never, earlier, val)

    def paced(panels, rows, values):
        groups = rows // 16
        regs = [[panel(g) for panel in panels] for g in range(groups)]
        order = [(g, c) for g in range(groups) for c in range(len(panels))]
        for n, val in enumerate(values):
            g, c = order[n * len(order) // len(values)]
            regs[g][c] = jnp.where(never, _words(val), regs[g][c])
        return _halves(jnp.concatenate([jnp.concatenate(r, axis=1) for r in regs], axis=0))

    dt_row = jnp.exp(ldt_ref[...].astype(F32).reshape(1, D)).astype(BF16).astype(F32)
    for c in range(NT):
        dts[c] = jnp.broadcast_to(dt_row[:, c * 128:(c + 1) * 128], (8, 128))

    def discretize(c, past):
        dt = dts[c][0:1, :]
        for r in range(NS // 32):
            raw = [par[c, i, 32 * r:32 * r + 32, :].astype(F32) for i in range(6)]
            for n in range(4):
                a_re, a_im, b_re, b_im, c_re, c_im = (v[8 * n:8 * n + 8] for v in raw)
                mag, ang = jnp.exp(dt * a_re), behind(dt * a_im, past[-LAG_D])
                db_re, db_im = dt * b_re, dt * b_im
                vals = (mag * jnp.cos(ang), mag * jnp.sin(ang),
                        c_re * db_re - c_im * db_im, c_re * db_im + c_im * db_re)
                for i, val in enumerate(vals):
                    disc[i, 32 * r + 8 * n:32 * r + 8 * n + 8, :] = val
                yield list(vals[:2])
        for i in range(2):
            zw[c % 2, 4 * i + 0] = disc[2 * i, 0:128, :].T
            zw[c % 2, 4 * i + 1] = disc[2 * i + 1, 0:128, :].T
            yield []
            re, im = disc[2 * i, 128:NS, :], disc[2 * i + 1, 128:NS, :]
            zw[c % 2, 4 * i + 2] = jnp.concatenate([re, re], axis=0).T
            zw[c % 2, 4 * i + 3] = jnp.concatenate([-im, im], axis=0).T
            yield []

    def put(tile, slot, even, odd):
        for comp in range(len(even)):
            tab[tile % 2, comp, pl.ds(16 * slot, 8, stride=2), :] = even[comp]
            tab[tile % 2, comp, pl.ds(16 * slot + 1, 8, stride=2), :] = odd[comp]

    def get(group, slot, comps):
        tile, half = divmod(group, 2)
        return tuple(tab[tile % 2, comp, pl.ds(16 * slot + 8 * half, 8), :] for comp in range(comps))

    def running(z, conj=False):
        x, y, p, q = z
        if conj:
            return (x, -y, jnp.where(low, p, -q))
        return (x, y, jnp.where(low, p, q), jnp.where(low, -q, p))

    def tables(c, tile, earlier):
        rows = slice(8 * tile, 8 * tile + 8)
        one = (jnp.ones((8, 128), F32), jnp.zeros((8, 128), F32)) * 2
        z1 = tuple(behind(zw[c % 2, i, rows, :], earlier if i % 2 == 0 else None) for i in range(4))
        w = tuple(zw[c % 2, 4 + i, rows, :] for i in range(4))
        z2 = _csq(z1)
        put(tile, _Q_G, z2, z2)
        z4 = _csq(z2)
        w4 = _cmul(w, z4)
        put(tile, _Q_W, running(w), running(w4))
        put(tile, _Q_W + 3, running(_cmul(w, z1)), running(_cmul(w4, z1)))
        z8 = _csq(z4)
        put(tile, _Q_V, running(one, True), running(z8, True))
        z16 = _csq(z8)
        z24 = _cmul(z16, z8)
        put(tile, _Q_V + 1, running(z16, True), running(z24, True))
        x, y, p, q = z16
        rec = (x + x, x * x + y * y, p + p, p * p + q * q)
        put(tile, _Q_REC, rec, rec)
        z256 = _csq(_csq(_csq(_csq(z16))))
        put(tile, _Q_G + 1, z4, z256)
        yield [z24[0], z24[2], z256[0], z256[2]]
        z512 = _csq(z256)
        put(tile, _Q_G + 2, z512, one)
        w256, w512 = _cmul(w, z256), _cmul(w, z512)
        put(tile, _Q_W + 1, running(w256), running(w512))
        w258, w516 = _cmul(w256, z2), _cmul(w512, z4)
        put(tile, _Q_W + 4, running(w258), running(w516))
        z1024 = _csq(z512)
        w1024 = _cmul(w, z1024)
        w1280, w2048 = _cmul(w1024, z256), _cmul(w1024, z1024)
        put(tile, _Q_W + 2, running(w1024), running(w2048))
        put(tile, _Q_W + 5, running(w1280), running(w2048))
        yield [w258[0], w516[2], w1280[0], w2048[2]]

    def operand(panels):
        return jnp.concatenate([jnp.concatenate(parts, axis=0) for parts in panels], axis=1).astype(BF16)

    chan = row // 2
    slot_of_lane = ((lane // 2) - chan) % 4

    def generate(c, riders, upcoming, chores):
        base = c % 2 * 256 if isinstance(c, int) else pl.multiple_of(c % 2 * 256, 256)
        slots = 32 + HEAD + TAIL
        for rider in riders[:HEAD * len(riders) // slots]:
            rider([])
        _take(tables(c, 0, None), 2)
        res, stage2, stage3, past = None, [], [], [None] * 8
        extra = discretize(c + 1, past) if upcoming else iter(())
        for group in range(32 + 3):
            for i, r in enumerate(stage3):
                rs[i, pl.ds(base + 8 * (group - 3), 8), :] = jnp.where(
                    (chan & 2) == 2, pltpu.roll(r, 128 - 4, 1), r)
            stage3 = [jnp.where((chan & 1) == 1, pltpu.roll(r, 128 - 2, 1), r) for r in stage2]
            stage2 = []
            for i in range(3 if res is not None else 0):
                r = res[8 * i:8 * i + 8]
                for a in range(1, 4):
                    blk = res[24 * a + 8 * i:24 * a + 8 * i + 8]
                    r = jnp.where(slot_of_lane == a, pltpu.roll(blk, 2 * a, 1), r)
                stage2.append(r)
            res = None
            ride = riders[(group + HEAD) * len(riders) // slots:(group + HEAD + 1) * len(riders) // slots]
            if group >= 32:
                for rider in ride:
                    rider([])
            else:
                if group % 2 == 0:
                    ahead = tables(c, group // 2 + 1, past[-LAG]) if group + 2 < 32 else iter(())
                _take(chores, 1)
                pace = _take(extra, 1) + _take(ahead, 1)
                for n, rider in enumerate(ride):
                    rider(pace[n * len(pace) // len(ride):(n + 1) * len(pace) // len(ride)])
                a_lo, b_lo, a_hi, b_hi = get(group, _Q_REC, 4)
                rhs = []
                for al, be, v in zip((a_lo, a_lo, a_hi), (b_lo, b_lo, b_hi),
                                     zip(get(group, _Q_V, 3), get(group, _Q_V + 1, 3))):
                    v = [v[0], behind(v[1], past[-LAG])]
                    for i in range(2, 16):
                        v.append(al * v[i - 1] - be * v[i - 2])
                    rhs.append(v)
                u = [get(group, _Q_W + n, 4) for n in range(6)]
                m = [tuple(behind(g, past[-LAG]) for g in get(group, _Q_G + i, 4)) for i in range(3)] * 2
                lhs = [[v[0] for v in u] + [v[0] * g[0] - v[1] * g[1] for v, g in zip(u, m)],
                       [v[1] for v in u] + [v[1] * g[0] + v[0] * g[1] for v, g in zip(u, m)],
                       [v[2] for v in u] + [v[2] * g[2] + v[3] * g[3] for v, g in zip(u, m)]]
                res = jax.lax.dot_general(operand(lhs), operand(rhs), _NT_DIMS, preferred_element_type=F32)
                past.append(res[0:8] if riders else None)
        _take(extra, NS)
        _take(chores, NS)

    def dft_passes(c):
        base = c % 2 * 256 if isinstance(c, int) else pl.multiple_of(c % 2 * 256, 256)
        for t in range(len(_BASE)):
            kt[t] = _words(rs[t // 2, pl.ds(base + t % 2, 128, stride=2), :].astype(BF16))

        def kernel_pass(m):
            def run(values):
                lhs = paced([lambda g, idx=idx: kmat[idx, 8 * g:8 * g + 8, :] for _, idx in _KPASSES[m]],
                            2 * T, values)
                rhs = _halves(jnp.concatenate([kt[t] for t, _ in _KPASSES[m]], axis=1))
                spec[NT + c, m, 0:2 * T, :] = jax.lax.dot_general(lhs, rhs, _NT_DIMS, preferred_element_type=F32)
            return run

        def signal_pass(m):
            def run(values):
                lhs = paced([lambda g: fwd_ref[8 * g:8 * g + 8, :]], 2 * T, values)
                block = xs[c, m * T:(m + 1) * T, :]
                xw[c, m * T // 2:(m + 1) * T // 2, :] = _words(block)
                spec[c, m, 0:2 * T, :] = jnp.dot(lhs, block, preferred_element_type=F32)
            return run

        return [make(m) for m in range(NB) for make in (signal_pass, kernel_pass)]

    def permute_weights(c):
        for part in range(3):
            for n in range(NT):
                col = part * D + n * 128
                tmp[part, n * 128:(n + 1) * 128, :] = wraw[c, :, col:col + 128].astype(F32).T
                yield []
            for j in range(DH):
                wt[c, pl.ds((part * D + j * H) // 2, H // 2), :] = _words(
                    tmp[part, pl.ds(j, H, stride=DH), :].astype(BF16))
                if j % 7 == 6:
                    yield []
        tmp[3, 0:D, :] = woraw[c].astype(F32)
        yield []
        for j in range(DH):
            wop[c, pl.ds(j * H // 2, H // 2), :] = _words(tmp[3, pl.ds(j, H, stride=DH), :].astype(BF16))
            if j % 7 == 6:
                yield []

    with jax.named_scope("P0"):
        for cp in par_copies(0) + par_copies(1):
            cp.start()
        for cp in par_copies(0):
            cp.wait()
        km_copy.start()
        for cp in tile_copies(0):
            cp.start()
        for c in range(2, NT):
            for cp in par_copies(c):
                cp.start()
        _take(discretize(0, [None] * 8), NS)
        for cp in par_copies(1):
            cp.wait()
        generate(0, [], True, iter(()))
        for c in range(1, NT):
            for cp in tile_copies(c):
                cp.start()
        km_copy.wait()
        for c in range(2, NT):
            for cp in par_copies(c):
                cp.wait()

    def ssm_step(c, carry):
        for cp in tile_copies(c - 1):
            cp.wait()
        generate(c, dft_passes(c - 1), True, permute_weights(c - 1))
        return carry

    with jax.named_scope("P1"):
        jax.lax.fori_loop(1, NT - 1, ssm_step, 0)
    with jax.named_scope("P1b"):
        for cp in tile_copies(NT - 2) + tile_copies(NT - 1):
            cp.wait()
        generate(NT - 1, dft_passes(NT - 2), False, permute_weights(NT - 2))
        chores = permute_weights(NT - 1)
        for run in dft_passes(NT - 1):
            _take(chores, 1)
            run([])
        _take(chores, NS)

    for c in range(NT):
        ks[c, 0:PAD, :] = jnp.zeros((PAD, 128), F32)
        vs[c, 0:PAD, :] = jnp.zeros((PAD, 128), F32)
    q_scale = float(DH ** -0.5 * np.log2(np.e))
    n2 = S // M2
    ft_per_step = (T // 8) // n2

    def causal(a, b, j):
        acc = a[0] * b[j]
        for i in range(1, j + 1):
            acc = acc + a[i] * b[j - i]
        return acc

    even_order = [j for i in range(NB // 2) for j in (i, NB - 1 - i)]

    def convolve(it):
        def tile_of(f):
            return (it * ft_per_step + f) // 2 + f % 2 * (T // 16)

        def operands(f, c, phase):
            def load(slab, part):
                rows = pl.ds(pl.multiple_of(origin_ref[phase] + part * T + tile_of(f) * 8, 8), 8)
                return [spec[slab, m, rows, :] for m in range(NB)]

            plus, minus = (jnp.subtract, jnp.add) if f % 2 else (jnp.add, jnp.subtract)
            k_re, k_im = load(NT + c, 0), load(NT + c, 1)
            if phase == 0:
                return ([u + v for u, v in zip(load(c, 0), load(c, 1))],
                        [k_re[0]] + [minus(k_re[m], k_im[m - 1]) for m in range(1, NB)])
            if phase == 1:
                return load(c, 0), [k_im[0] - k_re[0]] + [
                    plus(k_im[m] - k_re[m], k_im[m - 1] + k_re[m - 1]) for m in range(1, NB)]
            return load(c, 1), [-k_im[0] - k_re[0]] + [
                (k_re[m - 1] - k_im[m - 1] if f % 2 else k_im[m - 1] - k_re[m - 1]) - (k_im[m] + k_re[m])
                for m in range(1, NB)]

        jobs = [(f, c, phase) for f in range(ft_per_step) for c in range(NT) for phase in range(3)]
        ahead, sums = operands(*jobs[0]), [{}, {}, {}]
        for n, (f, c, phase) in enumerate(jobs):
            a, b = ahead
            for i, j in enumerate(even_order):
                val = sums[phase][j] = causal(a, b, j)
                if i == RELEASE and n + 1 < len(jobs):
                    spec[2 * NT, 0, pl.ds(pl.multiple_of(origin_ref[3], 8), 8), :] = val
                    ahead = operands(*jobs[n + 1])
                if phase == 2:
                    z = jnp.concatenate([sums[0][j]] * 2, axis=0) + jnp.concatenate([val, sums[1][j]], axis=0)
                    val = _words(z.astype(BF16))
                    zs[j, c, pl.ds(pl.multiple_of(tile_of(f) * 8, 8), 8), :] = val
                yield val

    def logits(r0):
        past = [None] * LAG_S
        for t0 in range(0, M2, 8):
            q = [qs[c, t0:t0 + 8, :] for c in range(NT)]
            q[0] = behind(q[0], past[-LAG_S])
            for w in range(WIN):
                src = pl.ds(r0 + (t0 + PAD - DIL * w), 8)
                acc = q[0] * ks[0, src, :]
                for c in range(1, NT):
                    acc = acc + q[c] * ks[c, src, :]
                acc = acc + pltpu.roll(acc, 64, 1)
                acc = acc + pltpu.roll(acc, 32, 1)
                ps[w, pl.ds(r0 + t0, 8), :] = acc
            past.append(acc)
            yield

    def proj_step(it, carry):
        r0 = pl.multiple_of(it * M2, M2)
        conv, dots = convolve(it), logits(r0)
        x_panel = lambda c: lambda g: xw[c, pl.ds(pl.multiple_of(it * (M2 // 2), 8) + 8 * g, 8), :]
        place = lambda n, base: ((qs, ks, vs)[n // NT], (n % NT, pl.ds(base + (r0 + PAD if n >= NT else 0), M2)))
        todo, slots = 3 * NB * NT * ft_per_step, 0
        for n in range(3 * NT):
            if n % 4 == 0:
                hi = min(n + 4, 3 * NT)
                count = EARLY * todo * (slots + 1) // 260 - EARLY * todo * slots // 260 if slots < 13 else 0
                slots += 1
                xb = paced([x_panel(NT - 1)], M2, list(itertools.islice(conv, count)))
                tail = jax.lax.dot_general(xb, _halves(wt[NT - 1, n * 64:hi * 64, :]), _NT_DIMS,
                                           preferred_element_type=F32)
                for i in range(n, hi):
                    ref, idx = place(i, 0)
                    ref[idx] = tail[:, (i - n) * 128:(i - n + 1) * 128]
            if n < 2 * NT:
                count = EARLY * todo * (slots + 1) // 260 - EARLY * todo * slots // 260
                values = list(itertools.islice(conv, count))
            else:
                values = list(itertools.islice(conv, -(-(todo - EARLY * todo // 20) // NT)))
                for _ in itertools.islice(dots, -(-(M2 // 8) // NT)):
                    pass
            slots += 1
            xb = paced([x_panel(c) for c in range(NT - 1)], M2, values)
            w = _halves(jnp.concatenate([wt[c, n * 64:(n + 1) * 64, :] for c in range(NT - 1)], axis=1))
            ref, idx = place(n, pl.multiple_of(origin_ref[0], 8))
            res = jax.lax.dot_general(xb, w, _NT_DIMS, preferred_element_type=F32) + ref[idx]
            ref, idx = place(n, 0)
            ref[idx] = res if n >= NT else res * q_scale
        assert next(conv, None) is None and next(dots, 0) == 0
        return carry

    with jax.named_scope("P2"):
        jax.lax.fori_loop(0, n2, proj_step, 0)

    def attend(blk):
        r0 = 0 if isinstance(blk, int) else pl.multiple_of(blk * M3, M3)
        for t0 in range(0, M3, 16):
            logit = [ps[w, pl.ds(r0 + t0, 16), :] for w in range(WIN)]
            if isinstance(blk, int) and t0 == 0:
                pos = jax.lax.broadcasted_iota(jnp.int32, (16, 128), 0)
                logit = [jnp.where(pos >= DIL * w, l, -1e9) if w else l for w, l in enumerate(logit)]
            top = logit[0]
            for w in range(1, WIN):
                top = jnp.maximum(top, logit[w])
            e = [jnp.exp2(l - top) for l in logit]
            den = e[0]
            for w in range(1, WIN):
                den = den + e[w]
            inv = pl.reciprocal(den, approx=True)
            inv = inv * (2.0 - den * inv)
            for c in range(NT):
                acc = e[0] * vs[c, pl.ds(r0 + (t0 + PAD), 16), :]
                for w in range(1, WIN):
                    acc = acc + e[w] * vs[c, pl.ds(r0 + (t0 + PAD - DIL * w), 16), :]
                o = _words((acc * inv).astype(BF16))
                os_[blk % 2, c, t0 // 2:t0 // 2 + 8, :] = o
                yield o

    def out_copy(blk, c):
        rows = pl.ds(pl.multiple_of(blk * M3, M3), M3)
        return pltpu.make_async_copy(outs.at[c, rows], out_hbm.at[rows, lanes(c)], out_sem.at[blk, c])

    def gates(blk):
        r0 = 0 if isinstance(blk, int) else pl.multiple_of(blk * (M3 // 2), 8)
        gw_row = gw_ref[...].astype(F32).reshape(1, D)
        for g in range(M3 // 16):
            rows = pl.ds(r0 + 8 * g, 8)
            score = _halves(xw[0, rows, :]).astype(F32) * gw_row[:, 0:128]
            for c in range(1, NT):
                score = score + _halves(xw[c, rows, :]).astype(F32) * gw_row[:, c * 128:(c + 1) * 128]
            gate = jnp.broadcast_to(jax.nn.sigmoid(jnp.sum(score, axis=1, keepdims=True)), (16, 128))
            gs[blk % 2, 16 * g:16 * g + 16, :] = gate
            yield

    def finish(blk, work, total):
        rows = pl.ds(pl.multiple_of(blk * M3, M3), M3)
        word_rows = pl.ds(pl.multiple_of(blk * (M3 // 2), 8), M3 // 2)
        dskip_row = dskip_ref[...].astype(F32).reshape(1, D)
        spent = [0]

        def pull(cost):
            lo, spent[0] = spent[0], spent[0] + cost
            share = lambda t: total * max(t - LEAD, 0) // (35 - LEAD)
            return list(itertools.islice(work, share(spent[0]) - share(lo)))

        o_panel = lambda c: lambda g: oc[c, 8 * g:8 * g + 8, :]
        inv_panels = [lambda g, k=k: inv_ref[k, 8 * g:8 * g + 8, :] for k in range(2)]
        oc[...] = os_[blk % 2]
        for lo, hi in ((0, 4), (4, 5)):
            w = _halves(jnp.concatenate([wop[c, 256:320, :] for c in range(lo, hi)], axis=1))
            tail = jnp.dot(paced([o_panel(NT - 1)], M3, pull(hi - lo)), w, preferred_element_type=F32)
            for c in range(lo, hi):
                att[c] = tail[:, (c - lo) * 128:(c - lo + 1) * 128]
        for lo, hi in ((0, 2), (2, 4), (4, 5)):
            for i in range(M3 // T):
                z = _halves(jnp.concatenate([zs[blk * (M3 // T) + i, c] for c in range(lo, hi)], axis=1))
                y = jnp.dot(paced(inv_panels, T, pull(hi - lo)), z, preferred_element_type=F32)
                for c in range(lo, hi):
                    ys[c, i * T:(i + 1) * T, :] = y[:, (c - lo) * 128:(c - lo + 1) * 128]
        back = pl.ds(pl.multiple_of(origin_ref[0], 8), M3)
        for c in range(NT):
            mixed = jnp.dot(paced([o_panel(k) for k in range(NT - 1)], M3, pull(4)), _halves(wop[c, 0:256, :]),
                            preferred_element_type=F32) + att[c, back, :]
            ssm = ys[c, back, :] + _halves(xw[c, word_rows, :]).astype(F32) * dskip_row[:, c * 128:(c + 1) * 128]
            outs[c, rows, :] = (ssm + gs[blk % 2] * (mixed - ssm)).astype(BF16)
        assert next(work, None) is None

    def prepare(blk):
        now, mix = attend(blk), gates(blk)
        for _ in range(M3 // 16):
            next(mix)
            yield from itertools.islice(now, NT)

    for _ in prepare(0):
        pass
    n3 = S // M3

    def out_step(it, carry):
        finish(it, prepare(it + 1), M3 // 16 * NT)
        for c in range(NT):
            out_copy(it, c).start()
        return carry

    with jax.named_scope("P3"):
        jax.lax.fori_loop(0, n3 - 1, out_step, 0)
    with jax.named_scope("P4"):
        finish(n3 - 1, iter(()), 0)
        for c in range(NT):
            out_copy(n3 - 1, c).start()
        for blk in range(n3):
            for c in range(NT):
                out_copy(blk, c).wait()


@jax.jit
def pallas_gated_mix__sliding_local_dilated__ssm_conv_s4__prompt_kernel(
    A_x: jax.Array,
    A_wqkv: jax.Array,
    A_wo: jax.Array,
    B_u: jax.Array,
    B_A_re: jax.Array,
    B_A_im: jax.Array,
    B_B_re: jax.Array,
    B_B_im: jax.Array,
    B_C_re: jax.Array,
    B_C_im: jax.Array,
    B_log_dt: jax.Array,
    B_Dskip: jax.Array,
    gate_w: jax.Array,
):
    del B_u
    assert A_x.shape == (1, S, D) and B_A_re.shape == (D, NS) and B_A_re.dtype == BF16
    hbm = pl.BlockSpec(memory_space=pl.ANY)
    vmem = pl.BlockSpec(memory_space=pltpu.VMEM)
    out = pl.pallas_call(
        _kernel,
        out_shape=jax.ShapeDtypeStruct((S, D), BF16),
        in_specs=[hbm] * 10 + [vmem] * 6 + [pl.BlockSpec(memory_space=pltpu.SMEM)],
        out_specs=hbm,
        scratch_shapes=[
            pltpu.VMEM((NT, S, 128), BF16),
            pltpu.VMEM((NT, S // 2 + SKEW, 128), jnp.int32),
            pltpu.VMEM((NT, 128, 3 * D), BF16),
            pltpu.VMEM((NT, D, 128), BF16),
            pltpu.VMEM(_KMATS.shape, jnp.int32),
            pltpu.VMEM((NT, 6, NS, 128), BF16),
            pltpu.VMEM((NT, 3 * D // 2 + SKEW, 128), jnp.int32),
            pltpu.VMEM((NT, D // 2, 128), jnp.int32),
            pltpu.VMEM((4, D + 32, 128), F32),
            pltpu.VMEM((NT, 8, 128), F32),
            pltpu.VMEM((4, NS, 128), F32),
            pltpu.VMEM((2, 8, 128, 128), F32),
            pltpu.VMEM((2, 4, 16 * _NQ + SKEW, 128), F32),
            pltpu.VMEM((3, 512 + 32, 128), F32),
            pltpu.VMEM((len(_BASE), 64, 128), jnp.int32),
            pltpu.VMEM((2 * NT + 1, NB, 2 * T + SKEW, 128), F32),
            pltpu.VMEM((NB, NT, T, 128), jnp.int32),
            pltpu.VMEM((NT, M2 + SKEW, 128), F32),
            pltpu.VMEM((NT, S + PAD + SKEW, 128), F32),
            pltpu.VMEM((NT, S + PAD + 3 * SKEW, 128), F32),
            pltpu.VMEM((WIN, S + SKEW, 128), F32),
            pltpu.VMEM((2, NT, M3 // 2, 128), jnp.int32),
            pltpu.VMEM((NT, M3 // 2, 128), jnp.int32),
            pltpu.VMEM((2, M3, 128), F32),
            pltpu.VMEM((NT, M3, 128), F32),
            pltpu.VMEM((NT, M3, 128), F32),
            pltpu.VMEM((NT, S, 128), BF16),
            pltpu.SemaphoreType.DMA((NT,)),
            pltpu.SemaphoreType.DMA((NT,)),
            pltpu.SemaphoreType.DMA((NT,)),
            pltpu.SemaphoreType.DMA((1,)),
            pltpu.SemaphoreType.DMA((NT, 6)),
            pltpu.SemaphoreType.DMA((S // M3, NT)),
        ],
        compiler_params=pltpu.CompilerParams(vmem_limit_bytes=100 * 1024 * 1024),
    )(
        A_x.reshape(S, D), A_wqkv, A_wo, _KMATS,
        B_A_re.T, B_A_im.T, B_B_re.T, B_B_im.T, B_C_re.T, B_C_im.T,
        B_log_dt, B_Dskip, gate_w, _FWD, _INV, np.zeros((8, 128), np.int32), np.zeros((4,), np.int32),
    )
    return out.reshape(1, S, D)
```

```python
import itertools

import ml_dtypes
import numpy as np

import jax
import jax.numpy as jnp
import jax.experimental.pallas as pl
import jax.experimental.pallas.tpu as pltpu

F32 = jnp.float32
BF16 = jnp.bfloat16

S = 2048
D = 640
NS = 192
H = 32
DH = D // H
WIN, DIL = 8, 2
T = 128
NB = S // T
NT = D // 128
PAD = 16
M2 = 256
M3 = 256
SKEW = 8

HEAD, TAIL = 6, 2
LAG, LAG_D = 4, 6
LAG_S = 8
RELEASE = 9
EARLY = 20
LEAD = 4

_BASE = (0, 4, 256, 512, 1024, 2048)
_OFF = ((0, 1, 2, 3), (0, 1, 2, 3), (0, 2, 4, 6), (0, 4, 256, 260), (0, 256, 512, 768), (0, 0, 0, 0))


def _dft_constants():
    k = np.concatenate([np.arange(0, T, 2), np.arange(1, T, 2)])
    theta = 2.0 * np.pi * (k + 0.5) / (2 * T)
    ang = theta[:, None] * np.arange(T)[None, :]
    fwd = np.concatenate([np.cos(ang), -np.sin(ang)], axis=0)
    inv = np.stack([np.cos(ang).reshape(T // 8, 8, T), -np.sin(ang).reshape(T // 8, 8, T)], axis=1)
    inv = inv.reshape(2 * T, T).T / T
    slot = {}
    for t in range(len(_BASE)):
        for lane in range(128):
            i, a, p = lane // 8, (lane % 8) // 2, lane % 2
            slot.setdefault(_BASE[t] + _OFF[t][a] + 8 * (2 * i + p), (t, lane))
    lag = np.arange(S).astype(np.float32).astype(ml_dtypes.bfloat16).astype(np.float64).astype(np.int64)
    mats, passes = [], []
    for m in range(NB):
        per_tile = {}
        for n in range(T):
            t, lane = slot[int(lag[m * T + n])]
            per_tile.setdefault(t, np.zeros((2 * T, 128)))[:, lane] += fwd[:, n]
        passes.append(tuple((t, len(mats) + j) for j, t in enumerate(sorted(per_tile))))
        mats.extend(per_tile[t] for t in sorted(per_tile))

    def to_bf16(a):
        bits = np.asarray(a, np.float32).astype(ml_dtypes.bfloat16).view(np.uint16).astype(np.uint32)
        return (bits[..., 0::2, :] | (bits[..., 1::2, :] << 16)).view(np.int32)

    inv = inv.reshape(T, 2, T).transpose(1, 0, 2)
    return to_bf16(fwd), to_bf16(inv), to_bf16(np.stack(mats)), tuple(passes)


_FWD, _INV, _KMATS, _KPASSES = _dft_constants()

_Q_W, _Q_G, _Q_V, _Q_REC, _NQ = 0, 6, 9, 11, 12

_NT_DIMS = (((1,), (1,)), ((), ()))


def _csq(z):
    x, y, p, q = z
    return ((x - y) * (x + y), (x + x) * y, (p - q) * (p + q), (p + p) * q)


def _cmul(a, b):
    ax, ay, ap, aq = a
    bx, by, bp, bq = b
    return (ax * bx - ay * by, ax * by + ay * bx, ap * bp - aq * bq, ap * bq + aq * bp)


def _words(v):
    return pltpu.bitcast(v, jnp.int32)


def _halves(v):
    return pltpu.bitcast(v, BF16)


def _take(gen, n):
    out = []
    for _ in range(n):
        out += next(gen, [])
    return out


def _kernel(x_hbm, wqkv_hbm, wo_hbm, kmat_hbm, are_hbm, aim_hbm, bre_hbm, bim_hbm, cre_hbm, cim_hbm,
            ldt_ref, dskip_ref, gw_ref, fwd_ref, inv_ref, zero_ref, origin_ref,
            out_hbm,
            xs, xw, wraw, woraw, kmat, par, wt, wop, tmp, dts, disc, zw, tab, rs, kt, spec, zs, qs, ks, vs, ps, os_, oc, gs, att, ys, outs,
            x_sem, w_sem, wo_sem, km_sem, par_sem, out_sem):
    def lanes(c):
        return pl.ds(c * 128, 128) if isinstance(c, int) else pl.ds(pl.multiple_of(c * 128, 128), 128)

    def par_copies(c):
        return [pltpu.make_async_copy(src.at[:, lanes(c)], par.at[c, i], par_sem.at[c, i])
                for i, src in enumerate((are_hbm, aim_hbm, bre_hbm, bim_hbm, cre_hbm, cim_hbm))]

    def tile_copies(c):
        return [pltpu.make_async_copy(x_hbm.at[:, lanes(c)], xs.at[c], x_sem.at[c]),
                pltpu.make_async_copy(wqkv_hbm.at[lanes(c), :], wraw.at[c], w_sem.at[c]),
                pltpu.make_async_copy(wo_hbm.at[:, lanes(c)], woraw.at[c], wo_sem.at[c])]

    km_copy = pltpu.make_async_copy(kmat_hbm, kmat, km_sem.at[0])

    lane = jax.lax.broadcasted_iota(jnp.int32, (8, 128), 1)
    row = jax.lax.broadcasted_iota(jnp.int32, (8, 128), 0)
    low = lane < 64
    never = zero_ref[...] != 0

    def behind(val, earlier):
        return val if earlier is None else jnp.where(never, earlier, val)

    def paced(panels, rows, values):
        groups = rows // 16
        regs = [[panel(g) for panel in panels] for g in range(groups)]
        order = [(g, c) for g in range(groups) for c in range(len(panels))]
        for n, val in enumerate(values):
            g, c = order[n * len(order) // len(values)]
            regs[g][c] = jnp.where(never, _words(val), regs[g][c])
        return _halves(jnp.concatenate([jnp.concatenate(r, axis=1) for r in regs], axis=0))

    dt_row = jnp.exp(ldt_ref[...].astype(F32).reshape(1, D)).astype(BF16).astype(F32)
    for c in range(NT):
        dts[c] = jnp.broadcast_to(dt_row[:, c * 128:(c + 1) * 128], (8, 128))

    def discretize(c, past):
        dt = dts[c][0:1, :]
        for r in range(NS // 32):
            raw = [par[c, i, 32 * r:32 * r + 32, :].astype(F32) for i in range(6)]
            for n in range(4):
                a_re, a_im, b_re, b_im, c_re, c_im = (v[8 * n:8 * n + 8] for v in raw)
                mag, ang = jnp.exp(dt * a_re), behind(dt * a_im, past[-LAG_D])
                db_re, db_im = dt * b_re, dt * b_im
                vals = (mag * jnp.cos(ang), mag * jnp.sin(ang),
                        c_re * db_re - c_im * db_im, c_re * db_im + c_im * db_re)
                for i, val in enumerate(vals):
                    disc[i, 32 * r + 8 * n:32 * r + 8 * n + 8, :] = val
                yield list(vals[:2])
        for i in range(2):
            zw[c % 2, 4 * i + 0] = disc[2 * i, 0:128, :].T
            zw[c % 2, 4 * i + 1] = disc[2 * i + 1, 0:128, :].T
            yield []
            re, im = disc[2 * i, 128:NS, :], disc[2 * i + 1, 128:NS, :]
            zw[c % 2, 4 * i + 2] = jnp.concatenate([re, re], axis=0).T
            zw[c % 2, 4 * i + 3] = jnp.concatenate([-im, im], axis=0).T
            yield []

    def put(tile, slot, even, odd):
        for comp in range(len(even)):
            tab[tile % 2, comp, pl.ds(16 * slot, 8, stride=2), :] = even[comp]
            tab[tile % 2, comp, pl.ds(16 * slot + 1, 8, stride=2), :] = odd[comp]

    def get(group, slot, comps):
        tile, half = divmod(group, 2)
        return tuple(tab[tile % 2, comp, pl.ds(16 * slot + 8 * half, 8), :] for comp in range(comps))

    def running(z, conj=False):
        x, y, p, q = z
        if conj:
            return (x, -y, jnp.where(low, p, -q))
        return (x, y, jnp.where(low, p, q), jnp.where(low, -q, p))

    def tables(c, tile, earlier):
        rows = slice(8 * tile, 8 * tile + 8)
        one = (jnp.ones((8, 128), F32), jnp.zeros((8, 128), F32)) * 2
        z1 = tuple(behind(zw[c % 2, i, rows, :], earlier if i % 2 == 0 else None) for i in range(4))
        w = tuple(zw[c % 2, 4 + i, rows, :] for i in range(4))
        z2 = _csq(z1)
        put(tile, _Q_G, z2, z2)
        z4 = _csq(z2)
        w4 = _cmul(w, z4)
        put(tile, _Q_W, running(w), running(w4))
        put(tile, _Q_W + 3, running(_cmul(w, z1)), running(_cmul(w4, z1)))
        z8 = _csq(z4)
        put(tile, _Q_V, running(one, True), running(z8, True))
        z16 = _csq(z8)
        z24 = _cmul(z16, z8)
        put(tile, _Q_V + 1, running(z16, True), running(z24, True))
        x, y, p, q = z16
        rec = (x + x, x * x + y * y, p + p, p * p + q * q)
        put(tile, _Q_REC, rec, rec)
        z256 = _csq(_csq(_csq(_csq(z16))))
        put(tile, _Q_G + 1, z4, z256)
        yield [z24[0], z24[2], z256[0], z256[2]]
        z512 = _csq(z256)
        put(tile, _Q_G + 2, z512, one)
        w256, w512 = _cmul(w, z256), _cmul(w, z512)
        put(tile, _Q_W + 1, running(w256), running(w512))
        w258, w516 = _cmul(w256, z2), _cmul(w512, z4)
        put(tile, _Q_W + 4, running(w258), running(w516))
        z1024 = _csq(z512)
        w1024 = _cmul(w, z1024)
        w1280, w2048 = _cmul(w1024, z256), _cmul(w1024, z1024)
        put(tile, _Q_W + 2, running(w1024), running(w2048))
        put(tile, _Q_W + 5, running(w1280), running(w2048))
        yield [w258[0], w516[2], w1280[0], w2048[2]]

    def operand(panels):
        return jnp.concatenate([jnp.concatenate(parts, axis=0) for parts in panels], axis=1).astype(BF16)

    chan = row // 2
    slot_of_lane = ((lane // 2) - chan) % 4

    def generate(c, riders, upcoming, chores):
        base = c % 2 * 256 if isinstance(c, int) else pl.multiple_of(c % 2 * 256, 256)
        slots = 32 + HEAD + TAIL
        for rider in riders[:HEAD * len(riders) // slots]:
            rider([])
        _take(tables(c, 0, None), 2)
        res, stage2, stage3, past = None, [], [], [None] * 8
        extra = discretize(c + 1, past) if upcoming else iter(())
        for group in range(32 + 3):
            for i, r in enumerate(stage3):
                rs[i, pl.ds(base + 8 * (group - 3), 8), :] = jnp.where(
                    (chan & 2) == 2, pltpu.roll(r, 128 - 4, 1), r)
            stage3 = [jnp.where((chan & 1) == 1, pltpu.roll(r, 128 - 2, 1), r) for r in stage2]
            stage2 = []
            for i in range(3 if res is not None else 0):
                r = res[8 * i:8 * i + 8]
                for a in range(1, 4):
                    blk = res[24 * a + 8 * i:24 * a + 8 * i + 8]
                    r = jnp.where(slot_of_lane == a, pltpu.roll(blk, 2 * a, 1), r)
                stage2.append(r)
            res = None
            ride = riders[(group + HEAD) * len(riders) // slots:(group + HEAD + 1) * len(riders) // slots]
            if group >= 32:
                for rider in ride:
                    rider([])
            else:
                if group % 2 == 0:
                    ahead = tables(c, group // 2 + 1, past[-LAG]) if group + 2 < 32 else iter(())
                _take(chores, 1)
                pace = _take(extra, 1) + _take(ahead, 1)
                for n, rider in enumerate(ride):
                    rider(pace[n * len(pace) // len(ride):(n + 1) * len(pace) // len(ride)])
                a_lo, b_lo, a_hi, b_hi = get(group, _Q_REC, 4)
                rhs = []
                for al, be, v in zip((a_lo, a_lo, a_hi), (b_lo, b_lo, b_hi),
                                     zip(get(group, _Q_V, 3), get(group, _Q_V + 1, 3))):
                    v = [v[0], behind(v[1], past[-LAG])]
                    for i in range(2, 16):
                        v.append(al * v[i - 1] - be * v[i - 2])
                    rhs.append(v)
                u = [get(group, _Q_W + n, 4) for n in range(6)]
                m = [tuple(behind(g, past[-LAG]) for g in get(group, _Q_G + i, 4)) for i in range(3)] * 2
                lhs = [[v[0] for v in u] + [v[0] * g[0] - v[1] * g[1] for v, g in zip(u, m)],
                       [v[1] for v in u] + [v[1] * g[0] + v[0] * g[1] for v, g in zip(u, m)],
                       [v[2] for v in u] + [v[2] * g[2] + v[3] * g[3] for v, g in zip(u, m)]]
                res = jax.lax.dot_general(operand(lhs), operand(rhs), _NT_DIMS, preferred_element_type=F32)
                past.append(res[0:8] if riders else None)
        _take(extra, NS)
        _take(chores, NS)

    def dft_passes(c):
        base = c % 2 * 256 if isinstance(c, int) else pl.multiple_of(c % 2 * 256, 256)
        for t in range(len(_BASE)):
            kt[t] = _words(rs[t // 2, pl.ds(base + t % 2, 128, stride=2), :].astype(BF16))

        def kernel_pass(m):
            def run(values):
                lhs = paced([lambda g, idx=idx: kmat[idx, 8 * g:8 * g + 8, :] for _, idx in _KPASSES[m]],
                            2 * T, values)
                rhs = _halves(jnp.concatenate([kt[t] for t, _ in _KPASSES[m]], axis=1))
                spec[NT + c, m, 0:2 * T, :] = jax.lax.dot_general(lhs, rhs, _NT_DIMS, preferred_element_type=F32)
            return run

        def signal_pass(m):
            def run(values):
                lhs = paced([lambda g: fwd_ref[8 * g:8 * g + 8, :]], 2 * T, values)
                block = xs[c, m * T:(m + 1) * T, :]
                xw[c, m * T // 2:(m + 1) * T // 2, :] = _words(block)
                spec[c, m, 0:2 * T, :] = jnp.dot(lhs, block, preferred_element_type=F32)
            return run

        return [make(m) for m in range(NB) for make in (signal_pass, kernel_pass)]

    def permute_weights(c):
        for part in range(3):
            for n in range(NT):
                col = part * D + n * 128
                tmp[part, n * 128:(n + 1) * 128, :] = wraw[c, :, col:col + 128].astype(F32).T
                yield []
            for j in range(DH):
                wt[c, pl.ds((part * D + j * H) // 2, H // 2), :] = _words(
                    tmp[part, pl.ds(j, H, stride=DH), :].astype(BF16))
                if j % 7 == 6:
                    yield []
        tmp[3, 0:D, :] = woraw[c].astype(F32)
        yield []
        for j in range(DH):
            wop[c, pl.ds(j * H // 2, H // 2), :] = _words(tmp[3, pl.ds(j, H, stride=DH), :].astype(BF16))
            if j % 7 == 6:
                yield []

    with jax.named_scope("P0"):
        for cp in par_copies(0) + par_copies(1):
            cp.start()
        for cp in par_copies(0):
            cp.wait()
        km_copy.start()
        for cp in tile_copies(0):
            cp.start()
        for c in range(2, NT):
            for cp in par_copies(c):
                cp.start()
        _take(discretize(0, [None] * 8), NS)
        for cp in par_copies(1):
            cp.wait()
        generate(0, [], True, iter(()))
        for c in range(1, NT):
            for cp in tile_copies(c):
                cp.start()
        km_copy.wait()
        for c in range(2, NT):
            for cp in par_copies(c):
                cp.wait()

    def ssm_step(c, carry):
        for cp in tile_copies(c - 1):
            cp.wait()
        generate(c, dft_passes(c - 1), True, permute_weights(c - 1))
        return carry

    with jax.named_scope("P1"):
        jax.lax.fori_loop(1, NT - 1, ssm_step, 0)
    with jax.named_scope("P1b"):
        for cp in tile_copies(NT - 2) + tile_copies(NT - 1):
            cp.wait()
        generate(NT - 1, dft_passes(NT - 2), False, permute_weights(NT - 2))
        chores = permute_weights(NT - 1)
        for run in dft_passes(NT - 1):
            _take(chores, 1)
            run([])
        _take(chores, NS)

    for c in range(NT):
        ks[c, 0:PAD, :] = jnp.zeros((PAD, 128), F32)
        vs[c, 0:PAD, :] = jnp.zeros((PAD, 128), F32)
    q_scale = float(DH ** -0.5 * np.log2(np.e))
    n2 = S // M2
    ft_per_step = (T // 8) // n2

    def causal(a, b, j):
        acc = a[0] * b[j]
        for i in range(1, j + 1):
            acc = acc + a[i] * b[j - i]
        return acc

    even_order = [j for i in range(NB // 2) for j in (i, NB - 1 - i)]

    def convolve(it):
        def tile_of(f):
            return (it * ft_per_step + f) // 2 + f % 2 * (T // 16)

        def operands(f, c, phase):
            def load(slab, part):
                rows = pl.ds(pl.multiple_of(origin_ref[phase] + part * T + tile_of(f) * 8, 8), 8)
                return [spec[slab, m, rows, :] for m in range(NB)]

            plus, minus = (jnp.subtract, jnp.add) if f % 2 else (jnp.add, jnp.subtract)
            k_re, k_im = load(NT + c, 0), load(NT + c, 1)
            if phase == 0:
                return ([u + v for u, v in zip(load(c, 0), load(c, 1))],
                        [k_re[0]] + [minus(k_re[m], k_im[m - 1]) for m in range(1, NB)])
            if phase == 1:
                return load(c, 0), [k_im[0] - k_re[0]] + [
                    plus(k_im[m] - k_re[m], k_im[m - 1] + k_re[m - 1]) for m in range(1, NB)]
            return load(c, 1), [-k_im[0] - k_re[0]] + [
                (k_re[m - 1] - k_im[m - 1] if f % 2 else k_im[m - 1] - k_re[m - 1]) - (k_im[m] + k_re[m])
                for m in range(1, NB)]

        jobs = [(f, c, phase) for f in range(ft_per_step) for c in range(NT) for phase in range(3)]
        ahead, sums = operands(*jobs[0]), [{}, {}, {}]
        for n, (f, c, phase) in enumerate(jobs):
            a, b = ahead
            for i, j in enumerate(even_order):
                val = sums[phase][j] = causal(a, b, j)
                if i == RELEASE and n + 1 < len(jobs):
                    spec[2 * NT, 0, pl.ds(pl.multiple_of(origin_ref[3], 8), 8), :] = val
                    ahead = operands(*jobs[n + 1])
                if phase == 2:
                    z = jnp.concatenate([sums[0][j]] * 2, axis=0) + jnp.concatenate([val, sums[1][j]], axis=0)
                    val = _words(z.astype(BF16))
                    zs[j, c, pl.ds(pl.multiple_of(tile_of(f) * 8, 8), 8), :] = val
                yield val

    def logits(r0):
        past = [None] * LAG_S
        for t0 in range(0, M2, 8):
            q = [qs[c, t0:t0 + 8, :] for c in range(NT)]
            q[0] = behind(q[0], past[-LAG_S])
            for w in range(WIN):
                src = pl.ds(r0 + (t0 + PAD - DIL * w), 8)
                acc = q[0] * ks[0, src, :]
                for c in range(1, NT):
                    acc = acc + q[c] * ks[c, src, :]
                acc = acc + pltpu.roll(acc, 64, 1)
                acc = acc + pltpu.roll(acc, 32, 1)
                ps[w, pl.ds(r0 + t0, 8), :] = acc
            past.append(acc)
            yield

    def proj_step(it, carry):
        r0 = pl.multiple_of(it * M2, M2)
        conv, dots = convolve(it), logits(r0)
        x_panel = lambda c: lambda g: xw[c, pl.ds(pl.multiple_of(it * (M2 // 2), 8) + 8 * g, 8), :]
        place = lambda n, base: ((qs, ks, vs)[n // NT], (n % NT, pl.ds(base + (r0 + PAD if n >= NT else 0), M2)))
        todo, slots = 3 * NB * NT * ft_per_step, 0
        for n in range(3 * NT):
            if n % 4 == 0:
                hi = min(n + 4, 3 * NT)
                count = EARLY * todo * (slots + 1) // 260 - EARLY * todo * slots // 260 if slots < 13 else 0
                slots += 1
                xb = paced([x_panel(NT - 1)], M2, list(itertools.islice(conv, count)))
                tail = jax.lax.dot_general(xb, _halves(wt[NT - 1, n * 64:hi * 64, :]), _NT_DIMS,
                                           preferred_element_type=F32)
                for i in range(n, hi):
                    ref, idx = place(i, 0)
                    ref[idx] = tail[:, (i - n) * 128:(i - n + 1) * 128]
            if n < 2 * NT:
                count = EARLY * todo * (slots + 1) // 260 - EARLY * todo * slots // 260
                values = list(itertools.islice(conv, count))
            else:
                values = list(itertools.islice(conv, -(-(todo - EARLY * todo // 20) // NT)))
                for _ in itertools.islice(dots, -(-(M2 // 8) // NT)):
                    pass
            slots += 1
            xb = paced([x_panel(c) for c in range(NT - 1)], M2, values)
            w = _halves(jnp.concatenate([wt[c, n * 64:(n + 1) * 64, :] for c in range(NT - 1)], axis=1))
            ref, idx = place(n, pl.multiple_of(origin_ref[0], 8))
            res = jax.lax.dot_general(xb, w, _NT_DIMS, preferred_element_type=F32) + ref[idx]
            ref, idx = place(n, 0)
            ref[idx] = res if n >= NT else res * q_scale
        assert next(conv, None) is None and next(dots, 0) == 0
        return carry

    with jax.named_scope("P2"):
        jax.lax.fori_loop(0, n2, proj_step, 0)

    def attend(blk):
        r0 = 0 if isinstance(blk, int) else pl.multiple_of(blk * M3, M3)
        for t0 in range(0, M3, 16):
            logit = [ps[w, pl.ds(r0 + t0, 16), :] for w in range(WIN)]
            if isinstance(blk, int) and t0 == 0:
                pos = jax.lax.broadcasted_iota(jnp.int32, (16, 128), 0)
                logit = [jnp.where(pos >= DIL * w, l, -1e9) if w else l for w, l in enumerate(logit)]
            top = logit[0]
            for w in range(1, WIN):
                top = jnp.maximum(top, logit[w])
            e = [jnp.exp2(l - top) for l in logit]
            den = e[0]
            for w in range(1, WIN):
                den = den + e[w]
            inv = pl.reciprocal(den, approx=True)
            inv = inv * (2.0 - den * inv)
            for c in range(NT):
                acc = e[0] * vs[c, pl.ds(r0 + (t0 + PAD), 16), :]
                for w in range(1, WIN):
                    acc = acc + e[w] * vs[c, pl.ds(r0 + (t0 + PAD - DIL * w), 16), :]
                o = _words((acc * inv).astype(BF16))
                os_[blk % 2, c, t0 // 2:t0 // 2 + 8, :] = o
                yield o

    def out_copy(blk):
        rows = pl.ds(pl.multiple_of(blk * M3, M3), M3)
        return pltpu.make_async_copy(outs.at[rows], out_hbm.at[rows], out_sem.at[blk])

    def gates(blk):
        r0 = 0 if isinstance(blk, int) else pl.multiple_of(blk * (M3 // 2), 8)
        gw_row = gw_ref[...].astype(F32).reshape(1, D)
        for g in range(M3 // 16):
            rows = pl.ds(r0 + 8 * g, 8)
            score = _halves(xw[0, rows, :]).astype(F32) * gw_row[:, 0:128]
            for c in range(1, NT):
                score = score + _halves(xw[c, rows, :]).astype(F32) * gw_row[:, c * 128:(c + 1) * 128]
            gate = jnp.broadcast_to(jax.nn.sigmoid(jnp.sum(score, axis=1, keepdims=True)), (16, 128))
            gs[blk % 2, 16 * g:16 * g + 16, :] = gate
            yield

    def finish(blk, work, total):
        rows = pl.ds(pl.multiple_of(blk * M3, M3), M3)
        word_rows = pl.ds(pl.multiple_of(blk * (M3 // 2), 8), M3 // 2)
        dskip_row = dskip_ref[...].astype(F32).reshape(1, D)
        spent = [0]

        def pull(cost):
            lo, spent[0] = spent[0], spent[0] + cost
            share = lambda t: total * max(t - LEAD, 0) // (35 - LEAD)
            return list(itertools.islice(work, share(spent[0]) - share(lo)))

        o_panel = lambda c: lambda g: oc[c, 8 * g:8 * g + 8, :]
        inv_panels = [lambda g, k=k: inv_ref[k, 8 * g:8 * g + 8, :] for k in range(2)]
        oc[...] = os_[blk % 2]
        for lo, hi in ((0, 4), (4, 5)):
            w = _halves(jnp.concatenate([wop[c, 256:320, :] for c in range(lo, hi)], axis=1))
            tail = jnp.dot(paced([o_panel(NT - 1)], M3, pull(hi - lo)), w, preferred_element_type=F32)
            for c in range(lo, hi):
                att[c] = tail[:, (c - lo) * 128:(c - lo + 1) * 128]
        for lo, hi in ((0, 2), (2, 4), (4, 5)):
            for i in range(M3 // T):
                z = _halves(jnp.concatenate([zs[blk * (M3 // T) + i, c] for c in range(lo, hi)], axis=1))
                y = jnp.dot(paced(inv_panels, T, pull(hi - lo)), z, preferred_element_type=F32)
                for c in range(lo, hi):
                    ys[c, i * T:(i + 1) * T, :] = y[:, (c - lo) * 128:(c - lo + 1) * 128]
        back = pl.ds(pl.multiple_of(origin_ref[0], 8), M3)
        for c in range(NT):
            mixed = jnp.dot(paced([o_panel(k) for k in range(NT - 1)], M3, pull(4)), _halves(wop[c, 0:256, :]),
                            preferred_element_type=F32) + att[c, back, :]
            ssm = ys[c, back, :] + _halves(xw[c, word_rows, :]).astype(F32) * dskip_row[:, c * 128:(c + 1) * 128]
            outs[rows, c * 128:(c + 1) * 128] = (ssm + gs[blk % 2] * (mixed - ssm)).astype(BF16)
        assert next(work, None) is None

    def prepare(blk):
        now, mix = attend(blk), gates(blk)
        for _ in range(M3 // 16):
            next(mix)
            yield from itertools.islice(now, NT)

    for _ in prepare(0):
        pass
    n3 = S // M3

    def out_step(it, carry):
        finish(it, prepare(it + 1), M3 // 16 * NT)
        out_copy(it).start()
        return carry

    with jax.named_scope("P3"):
        jax.lax.fori_loop(0, n3 - 1, out_step, 0)
    with jax.named_scope("P4"):
        finish(n3 - 1, iter(()), 0)
        out_copy(n3 - 1).start()
        for blk in range(n3):
            out_copy(blk).wait()


@jax.jit
def pallas_gated_mix__sliding_local_dilated__ssm_conv_s4__prompt_kernel(
    A_x: jax.Array,
    A_wqkv: jax.Array,
    A_wo: jax.Array,
    B_u: jax.Array,
    B_A_re: jax.Array,
    B_A_im: jax.Array,
    B_B_re: jax.Array,
    B_B_im: jax.Array,
    B_C_re: jax.Array,
    B_C_im: jax.Array,
    B_log_dt: jax.Array,
    B_Dskip: jax.Array,
    gate_w: jax.Array,
):
    del B_u
    assert A_x.shape == (1, S, D) and B_A_re.shape == (D, NS) and B_A_re.dtype == BF16
    hbm = pl.BlockSpec(memory_space=pl.ANY)
    vmem = pl.BlockSpec(memory_space=pltpu.VMEM)
    out = pl.pallas_call(
        _kernel,
        out_shape=jax.ShapeDtypeStruct((S, D), BF16),
        in_specs=[hbm] * 10 + [vmem] * 6 + [pl.BlockSpec(memory_space=pltpu.SMEM)],
        out_specs=hbm,
        scratch_shapes=[
            pltpu.VMEM((NT, S, 128), BF16),
            pltpu.VMEM((NT, S // 2 + SKEW, 128), jnp.int32),
            pltpu.VMEM((NT, 128, 3 * D), BF16),
            pltpu.VMEM((NT, D, 128), BF16),
            pltpu.VMEM(_KMATS.shape, jnp.int32),
            pltpu.VMEM((NT, 6, NS, 128), BF16),
            pltpu.VMEM((NT, 3 * D // 2 + SKEW, 128), jnp.int32),
            pltpu.VMEM((NT, D // 2, 128), jnp.int32),
            pltpu.VMEM((4, D + 32, 128), F32),
            pltpu.VMEM((NT, 8, 128), F32),
            pltpu.VMEM((4, NS, 128), F32),
            pltpu.VMEM((2, 8, 128, 128), F32),
            pltpu.VMEM((2, 4, 16 * _NQ + SKEW, 128), F32),
            pltpu.VMEM((3, 512 + 32, 128), F32),
            pltpu.VMEM((len(_BASE), 64, 128), jnp.int32),
            pltpu.VMEM((2 * NT + 1, NB, 2 * T + SKEW, 128), F32),
            pltpu.VMEM((NB, NT, T, 128), jnp.int32),
            pltpu.VMEM((NT, M2 + SKEW, 128), F32),
            pltpu.VMEM((NT, S + PAD + SKEW, 128), F32),
            pltpu.VMEM((NT, S + PAD + 3 * SKEW, 128), F32),
            pltpu.VMEM((WIN, S + SKEW, 128), F32),
            pltpu.VMEM((2, NT, M3 // 2, 128), jnp.int32),
            pltpu.VMEM((NT, M3 // 2, 128), jnp.int32),
            pltpu.VMEM((2, M3, 128), F32),
            pltpu.VMEM((NT, M3, 128), F32),
            pltpu.VMEM((NT, M3, 128), F32),
            pltpu.VMEM((S, D), BF16),
            pltpu.SemaphoreType.DMA((NT,)),
            pltpu.SemaphoreType.DMA((NT,)),
            pltpu.SemaphoreType.DMA((NT,)),
            pltpu.SemaphoreType.DMA((1,)),
            pltpu.SemaphoreType.DMA((NT, 6)),
            pltpu.SemaphoreType.DMA((S // M3,)),
        ],
        compiler_params=pltpu.CompilerParams(vmem_limit_bytes=100 * 1024 * 1024),
    )(
        A_x.reshape(S, D), A_wqkv, A_wo, _KMATS,
        B_A_re.T, B_A_im.T, B_B_re.T, B_B_im.T, B_C_re.T, B_C_im.T,
        B_log_dt, B_Dskip, gate_w, _FWD, _INV, np.zeros((8, 128), np.int32), np.zeros((4,), np.int32),
    )
    return out.reshape(1, S, D)
```
